```python
import jax
import jax.numpy as jnp

def _softmax(x, axis=-1):
    return jax.nn.softmax(x, axis=axis)

def _gelu(x):
    return jax.nn.gelu(x, approximate=True)

def _silu(x):
    return jax.nn.silu(x)

def _sigmoid(x):
    return jax.nn.sigmoid(x)

def _layernorm(x, axis=-1, eps=1e-05):
    m = jnp.mean(x, axis=axis, keepdims=True)
    v = jnp.var(x, axis=axis, keepdims=True)
    return (x - m) / jnp.sqrt(v + eps)

def _scatter_add(tgt, idx, src, axis=0):
    return tgt.at[idx].add(src)

def _segment_sum(src, seg, n):
    return jax.ops.segment_sum(src, seg, n)

class _Rng:

    def __init__(self, key):
        self._k = key

    def _next(self):
        self._k, sub = jax.random.split(self._k)
        return sub

    def normal(self, shape):
        return jax.random.normal(self._next(), shape, dtype=jnp.bfloat16)

    def randint(self, lo, hi, shape):
        return jax.random.randint(self._next(), shape, lo, hi, dtype=jnp.int32)

    def uniform(self, shape, lo=0.0, hi=1.0):
        return jax.random.uniform(self._next(), shape, jnp.bfloat16, lo, hi)

    def permutation(self, n):
        return jax.random.permutation(self._next(), n)
kernel_name = 'adaLN_cond__sliding_local_dilated__glu_gated_bilinear__prompt'

def setup_inputs():
    _rng = _Rng(jax.random.key(int.from_bytes(__import__("os").urandom(4), "little")))
    _w = lambda a: (lambda t: t.astype(jnp.bfloat16) if jnp.issubdtype(t.dtype, jnp.floating) else t)(jnp.asarray(a))

    def _A_setup():
        B, S, D = (1, 2048, 576)
        return {'x': _w((lambda *s: _rng.normal(s) * 0.05)(B, S, D)), 'wqkv': _w((lambda *s: _rng.normal(s) * 0.05)(D, 3 * D)), 'wo': _w((lambda *s: _rng.normal(s) * 0.05)(D, D))}
    _A_in = _A_setup()

    def _B_setup():
        B, S, D, F = (1, 2048, 576, 4608)
        return {'x': _w((lambda *s: _rng.normal(s) * 0.05)(B, S, D)), 'w_gate': _w((lambda *s: _rng.normal(s) * 0.05)(D, F) * D ** (-0.5)), 'w_up': _w((lambda *s: _rng.normal(s) * 0.05)(D, F) * D ** (-0.5)), 'w_down': _w((lambda *s: _rng.normal(s) * 0.05)(F, D) * F ** (-0.5))}
    _B_in = _B_setup()
    return {'A_x': _A_in['x'], 'A_wqkv': _A_in['wqkv'], 'A_wo': _A_in['wo'], 'B_x': _B_in['x'], 'B_w_gate': _B_in['w_gate'], 'B_w_up': _B_in['w_up'], 'B_w_down': _B_in['w_down'], 'c': _w((lambda *s: _rng.normal(s) * 0.05)(1, 576)), 'w_mod': _w((lambda *s: _rng.normal(s) * 0.05)(576, 6 * 576) * 576 ** (-0.5))}

def reference(A_x, A_wqkv, A_wo, B_x, B_w_gate, B_w_up, B_w_down, c, w_mod):

    def _A_ref(x, wqkv, wo):
        B, S, D = x.shape
        H = 32
        Dh = D // H
        W, dil = (8, 2)
        qkv = (lambda x, *d: x.transpose(*d))((x @ wqkv).reshape(B, S, 3, H, Dh), 2, 0, 3, 1, 4)
        q, k, v = (qkv[0], qkv[1], qkv[2])
        scale = Dh ** (-0.5)
        pos = jnp.arange(S)
        off = jnp.arange(W) * dil
        idx = pos[:, None] - off[None, :]
        mask = idx >= 0
        idx_c = jnp.where(mask, idx, 0).reshape(-1)
        kg = k[:, :, idx_c, :].reshape(B, H, S, W, Dh)
        vg = v[:, :, idx_c, :].reshape(B, H, S, W, Dh)
        logits = jnp.einsum('bhsd,bhswd->bhsw', q, kg) * scale
        logits = jnp.where(mask[None, None, :, :], logits, -1000000000.0)
        attn = _softmax(logits, axis=-1)
        o = jnp.einsum('bhsw,bhswd->bhsd', attn, vg)
        return (lambda x, *d: x.transpose(*d))(o, 0, 2, 1, 3).reshape(B, S, D) @ wo

    def _B_ref(x, w_gate, w_up, w_down):
        g = jnp.einsum('bsd,df->bsf', x, w_gate)
        u = jnp.einsum('bsd,df->bsf', x, w_up)
        h = g * u
        return jnp.einsum('bsf,fd->bsd', h, w_down)
    x = A_x
    mod = (_silu(c) @ w_mod).reshape(c.shape[0], 6, 1, -1)
    sa, ca, ga, sb, cb, gb = (mod[:, 0].copy(), mod[:, 1].copy(), mod[:, 2].copy(), mod[:, 3].copy(), mod[:, 4].copy(), mod[:, 5].copy())
    h = _layernorm(x, axis=-1) * (1 + ca) + sa
    x = x + ga * _A_ref(h, A_wqkv, A_wo)
    h = _layernorm(x, axis=-1) * (1 + cb) + sb
    x = x + gb * _B_ref(h, B_w_gate, B_w_up, B_w_down)
    return x
```

```python
import functools

import jax
import jax.numpy as jnp
from jax import lax
import jax.experimental.pallas as pl
import jax.experimental.pallas.tpu as pltpu

S, D, H, DH, W, DIL, F = 2048, 576, 32, 18, 8, 2, 4608
HALO = 16
NT = 5
EPS = 1e-5
BF, F32 = jnp.bfloat16, jnp.float32
NT_DIMS = (((1,), (1,)), ((), ()))


def _tw(j):
    return min(128, D - 128 * j)


def make(blocks=(512, 512, 512, 512), FC=512, R=16, flags=None, sched=None, name="k1"):
    assert sum(blocks) == S
    TMX = max(blocks)
    starts = [sum(blocks[:i]) for i in range(len(blocks))]
    nb = len(blocks)
    nF = F // FC

    def kernel(c_ref, xT_hbm, wqkv_hbm, wo_hbm, wg_hbm, wu_hbm, wdT_hbm, wmod_hbm, outT_hbm,
               xT, wqkv, wo, wg, wu, wdT, wmod, tmpT, wpT, woT, modT,
               qbuf, kbuf, vbuf, hbuf, obuf, x1a, x1b, h2a, h2b, accT, outT, sems):
        x1s, h2s = (x1a, x1b), (h2a, h2b)
        sem_i = [0]

        def copy(src, dst):
            cp = pltpu.make_async_copy(src, dst, sems.at[sem_i[0]])
            sem_i[0] += 1
            cp.start()
            return cp

        cp_wqkv = copy(wqkv_hbm, wqkv)
        cp_x0 = copy(xT_hbm.at[:, pl.ds(0, blocks[0])], xT.at[:, pl.ds(0, blocks[0])])
        cp_m0 = copy(wmod_hbm.at[:, pl.ds(0, 2 * D)], wmod.at[:, pl.ds(0, 2 * D)])
        cp_wo = copy(wo_hbm, wo)
        cp_m1 = copy(wmod_hbm.at[:, pl.ds(2 * D, 4 * D)], wmod.at[:, pl.ds(2 * D, 4 * D)])
        cp_x1 = copy(xT_hbm.at[:, pl.ds(blocks[0], S - blocks[0])], xT.at[:, pl.ds(blocks[0], S - blocks[0])])
        cp_f = []
        for j in range(nF):
            cs = pl.ds(j * FC, FC)
            cp_f.append((copy(wg_hbm.at[:, cs], wg.at[:, cs]), copy(wu_hbm.at[:, cs], wu.at[:, cs]),
                         copy(wdT_hbm.at[:, cs], wdT.at[:, cs])))

        def prep_wqkv():
            for cb in range(14):
                cw = min(128, 3 * D - cb * 128)
                t = wqkv[:, cb * 128:cb * 128 + cw].astype(F32).T
                for j in range(NT):
                    tmpT[j, cb * 128:cb * 128 + cw, 0:_tw(j)] = t[:, j * 128:j * 128 + _tw(j)]
            for part in range(3):
                for d in range(DH):
                    if part == 0:
                        r0 = d * H
                    elif part == 1:
                        r0 = 640 + d * H if d < 16 else D + (d - 16) * H
                    else:
                        r0 = 1152 + d * H
                    v = tmpT[:, pl.ds(part * D + d, H, stride=DH), :].astype(BF)
                    for j in range(NT):
                        wpT[r0:r0 + H, j * 128:j * 128 + _tw(j)] = v[j][:, 0:_tw(j)]
            wpT[3 * D:3 * D + 64, :] = jnp.zeros((64, D), BF)

        def prep_wo():
            for j in range(NT):
                tmpT[j, 0:D, 0:_tw(j)] = wo[:, j * 128:j * 128 + _tw(j)].astype(F32)
            for j in range(NT):
                p = jnp.concatenate([tmpT[j, pl.ds(d, H, stride=DH), :] for d in range(DH)], axis=0)
                woT[j * 128:j * 128 + _tw(j), :] = p[:, 0:_tw(j)].T.astype(BF)

        def prep_mod(c0, n, one_lo, one_hi):
            cf = c_ref[...].astype(F32)
            sc = (cf * jax.nn.sigmoid(cf)).astype(BF)
            m = jnp.dot(jnp.broadcast_to(sc, (16, D)), wmod[:, c0:c0 + n], preferred_element_type=F32)[0:8]
            col = lax.broadcasted_iota(jnp.int32, m.shape, 1)
            m = jnp.where((col >= one_lo) & (col < one_hi), m + 1.0, m)
            for t in range(n // 128):
                mt = jnp.broadcast_to(m[0:1, t * 128:(t + 1) * 128], (128, 128))
                modT[c0 + t * 128:c0 + (t + 1) * 128, :] = mt.T

        def ln_mod(xf, shift_row, scale_row):
            mean = jnp.sum(xf, axis=0, keepdims=True) * (1.0 / D)
            xc = xf - mean
            var = jnp.sum(xc * xc, axis=0, keepdims=True) * (1.0 / D)
            y = xc * lax.rsqrt(var + EPS)
            return y * modT[scale_row:scale_row + D, :] + modT[shift_row:shift_row + D, :]

        lane = lax.broadcasted_iota(jnp.int32, (1, 128), 1)

        def stage_a(i):
            s0, tm = starts[i], blocks[i]
            x1, h2 = x1s[i % 2], h2s[i % 2]
            for t in range(tm // 128):
                xf = xT[:, s0 + t * 128:s0 + (t + 1) * 128].astype(F32)
                hbuf[t * 128:(t + 1) * 128, :] = ln_mod(xf, 0, D).T.astype(BF)
            yield
            h = hbuf[0:tm, :]
            res = lax.dot_general(h, wpT[0:640, :], NT_DIMS, preferred_element_type=F32)
            scale = DH ** -0.5
            for j in range(4):
                qbuf[j, 0:tm, :] = res[:, j * 128:(j + 1) * 128] * scale
            xt = res[:, 512:640]
            qbuf[4, 0:tm, :] = jnp.where(lane < 64, xt * scale, 0.0)
            kbuf[4, HALO + s0:HALO + s0 + tm, :] = jnp.where(lane < 64, pltpu.roll(xt, 64, 1), 0.0)
            yield
            res = lax.dot_general(h, wpT[640:1152, :], NT_DIMS, preferred_element_type=F32)
            for j in range(4):
                kbuf[j, HALO + s0:HALO + s0 + tm, :] = res[:, j * 128:(j + 1) * 128]
            res = lax.dot_general(h, wpT[1152:1792, :], NT_DIMS, preferred_element_type=F32)
            for j in range(NT):
                vbuf[j, HALO + s0:HALO + s0 + tm, :] = res[:, j * 128:(j + 1) * 128]
            if i == 0:
                for j in range(NT):
                    kbuf[j, 0:HALO, :] = jnp.broadcast_to(kbuf[j, HALO:HALO + 1, :], (HALO, 128))
                    vbuf[j, 0:HALO, :] = jnp.broadcast_to(vbuf[j, HALO:HALO + 1, :], (HALO, 128))
            yield
            ngrp = tm // R
            for gi in range(ngrp):
                r0 = gi * R
                q = qbuf[:, r0:r0 + R, :]
                ls = []
                for w in range(W):
                    a = HALO + s0 + r0 - DIL * w
                    p = jnp.sum(q * kbuf[:, a:a + R, :], axis=0)
                    p = p + pltpu.roll(p, 64, 1)
                    p = p + pltpu.roll(p, 32, 1)
                    if s0 + r0 < DIL * w:
                        row = lax.broadcasted_iota(jnp.int32, (R, 128), 0) + (s0 + r0)
                        p = jnp.where(row >= DIL * w, p, -1e9)
                    ls.append(p)
                m = functools.reduce(jnp.maximum, ls)
                es = [jnp.exp(l - m) for l in ls]
                den = functools.reduce(jnp.add, es)
                acc = None
                for w in range(W):
                    a = HALO + s0 + r0 - DIL * w
                    t = es[w][None] * vbuf[:, a:a + R, :]
                    acc = t if acc is None else acc + t
                o = (acc * (1.0 / den)[None]).astype(BF)
                for j in range(NT):
                    obuf[r0:r0 + R, j * 128:j * 128 + _tw(j)] = o[j][:, 0:_tw(j)]
                if (gi + 1) % (ngrp // 4) == 0:
                    yield
            if i == 0:
                cp_wo.wait()
                prep_wo()
                cp_m1.wait()
                prep_mod(2 * D, 4 * D, 2 * D, 3 * D)
            aT = lax.dot_general(woT[...], obuf[0:tm, :], NT_DIMS, preferred_element_type=F32)
            for t in range(tm // 128):
                xf = xT[:, s0 + t * 128:s0 + (t + 1) * 128].astype(F32)
                x1[:, t * 128:(t + 1) * 128] = xf + modT[2 * D:3 * D, :] * aT[:, t * 128:(t + 1) * 128]
            yield
            for t in range(tm // 128):
                h2[t * 128:(t + 1) * 128, :] = ln_mod(x1[:, t * 128:(t + 1) * 128], 3 * D, 4 * D).T.astype(BF)
            yield

        out_cps = []

        def stage_b(i, other):
            s0, tm = starts[i], blocks[i]
            x1, h2 = x1s[i % 2], h2s[i % 2]
            h = h2[0:tm, :]
            for j in range(nF):
                if i == 0:
                    for cp in cp_f[j]:
                        cp.wait()
                c0 = j * FC
                g = jnp.dot(h, wg[:, c0:c0 + FC], preferred_element_type=F32)
                u = jnp.dot(h, wu[:, c0:c0 + FC], preferred_element_type=F32)
                hh = (g * u).astype(BF)
                part = lax.dot_general(wdT[:, c0:c0 + FC], hh, NT_DIMS, preferred_element_type=F32)
                if j == 0:
                    accT[:, 0:tm] = part
                else:
                    accT[:, 0:tm] += part
                if other is not None:
                    n_adv = ((j + 1) * 9) // nF - (j * 9) // nF
                    for _ in range(n_adv):
                        next(other, None)
            if other is not None:
                for _ in other:
                    pass
            for t in range(tm // 128):
                sl = slice(t * 128, (t + 1) * 128)
                outT[:, s0 + t * 128:s0 + (t + 1) * 128] = (x1[:, sl] + modT[5 * D:6 * D, :] * accT[:, sl]).astype(BF)
            out_cps.append(copy(outT.at[:, pl.ds(s0, tm)], outT_hbm.at[:, pl.ds(s0, tm)]))

        cp_wqkv.wait()
        prep_wqkv()
        cp_m0.wait()
        prep_mod(0, 2 * D, D, 2 * D)
        cp_x0.wait()
        for _ in stage_a(0):
            pass
        cp_x1.wait()
        for i in range(nb):
            stage_b(i, stage_a(i + 1) if i + 1 < nb else None)
        for cp in out_cps:
            cp.wait()

    n_sems = 6 + 3 * nF + nb
    hbm = pl.BlockSpec(memory_space=pltpu.HBM)

    def fn(A_x, A_wqkv, A_wo, B_x, B_w_gate, B_w_up, B_w_down, c, w_mod):
        del B_x
        outT = pl.pallas_call(
            kernel,
            in_specs=[pl.BlockSpec(memory_space=pltpu.VMEM)] + [hbm] * 7,
            out_specs=hbm,
            out_shape=jax.ShapeDtypeStruct((D, S), BF),
            scratch_shapes=[
                pltpu.VMEM((D, S), BF), pltpu.VMEM((D, 3 * D), BF), pltpu.VMEM((D, D), BF),
                pltpu.VMEM((D, F), BF), pltpu.VMEM((D, F), BF), pltpu.VMEM((D, F), BF),
                pltpu.VMEM((D, 6 * D), BF),
                pltpu.VMEM((NT, 1792, 128), F32), pltpu.VMEM((1792, D), BF), pltpu.VMEM((D, D), BF),
                pltpu.VMEM((6 * D, 128), F32),
                pltpu.VMEM((NT, TMX, 128), F32), pltpu.VMEM((NT, HALO + S, 128), F32),
                pltpu.VMEM((NT, HALO + S, 128), F32),
                pltpu.VMEM((TMX, D), BF), pltpu.VMEM((TMX, D), BF),
                pltpu.VMEM((D, TMX), F32), pltpu.VMEM((D, TMX), F32),
                pltpu.VMEM((TMX, D), BF), pltpu.VMEM((TMX, D), BF),
                pltpu.VMEM((D, TMX), F32), pltpu.VMEM((D, S), BF),
                pltpu.SemaphoreType.DMA((n_sems,)),
            ],
            compiler_params=pltpu.CompilerParams(vmem_limit_bytes=110 * 2**20, flags=flags),
            name=name,
        )(c, A_x[0].T, A_wqkv, A_wo, B_w_gate, B_w_up, B_w_down.T, w_mod)
        return outT.T[None]

    return fn


@jax.jit
def pallas_adaLN_cond__sliding_local_dilated__glu_gated_bilinear__prompt_kernel(
    A_x: jax.Array,
    A_wqkv: jax.Array,
    A_wo: jax.Array,
    B_x: jax.Array,
    B_w_gate: jax.Array,
    B_w_up: jax.Array,
    B_w_down: jax.Array,
    c: jax.Array,
    w_mod: jax.Array,
):
    return make()(A_x, A_wqkv, A_wo, B_x, B_w_gate, B_w_up, B_w_down, c, w_mod)
```

```python
import contextlib
import functools

import jax
import jax.numpy as jnp
from jax import lax
import jax.experimental.pallas as pl
import jax.experimental.pallas.tpu as pltpu

S, D, H, DH, W, DIL, F = 2048, 576, 32, 18, 8, 2, 4608
HALO = 16
NT = 5
DHALF = D // 2
EPS = 1e-5
BF, F32 = jnp.bfloat16, jnp.float32
NT_DIMS = (((1,), (1,)), ((), ()))


def _tw(j):
    return min(128, D - 128 * j)


def _dot(a, b):
    return jnp.dot(a, b, preferred_element_type=F32)


def _dot_nt(a, b):
    return lax.dot_general(a, b, NT_DIMS, preferred_element_type=F32)


def make(TM=512, FC=384, R=16, chain=1, chain0=2, waits=None, chain_ln=False, swp=False, nb_run=None, flags=None, name="k2",
         scopes=False, wo_at=None, qkv_at=None):
    nb = S // TM
    T = TM // 2
    nP = F // (2 * FC)
    nb_run = nb if nb_run is None else nb_run
    wo_at = (2 * nP) // 3 if wo_at is None else wo_at
    qkv_at = 0 if qkv_at is None else qkv_at
    waits = {1: [1], 2: list(range(2, nP))} if waits is None else waits

    def kernel(c_ref, xT_hbm, wqkv_hbm, wo_hbm, wg_hbm, wu_hbm, wdT_hbm, wmod_hbm, outT_hbm,
               xT, wqkv, wo, wg, wu, wdT, wmod, tmpT, wpT, woT, modT, wg5, wu5, wd5,
               qbuf, kbuf, vbuf, hbuf, obuf, x1, a7, hr, acc7, outT, sems):
        sc = jax.named_scope if scopes else (lambda n: contextlib.nullcontext())
        sem_i = [0]

        def copy(src, dst):
            cp = pltpu.make_async_copy(src, dst, sems.at[sem_i[0]])
            sem_i[0] += 1
            cp.start()
            return cp

        def copy_cols(src, dst, c0, n):
            return copy(src.at[:, pl.ds(c0, n)], dst.at[:, pl.ds(c0, n)])

        cp_wqkv = copy(wqkv_hbm, wqkv)
        cp_m0 = copy_cols(wmod_hbm, wmod, 0, 2 * D)
        cp_x0 = copy_cols(xT_hbm, xT, 0, 2 * TM)
        cp_wo = copy(wo_hbm, wo)
        cp_m1 = copy_cols(wmod_hbm, wmod, 2 * D, 4 * D)
        cp_f = []
        for p in range(nP):
            cp_f.append([copy_cols(s, d, 2 * p * FC, 2 * FC) for s, d in ((wg_hbm, wg), (wu_hbm, wu), (wdT_hbm, wdT))])
            if p == 0:
                cp_x1 = copy_cols(xT_hbm, xT, 2 * TM, S - 2 * TM)

        cbits = pltpu.bitcast(jnp.broadcast_to(c_ref[:, 0:128].astype(F32), (8, 128)), jnp.int32)
        keep = ((cbits * cbits) & 2) == 0

        def after(x, prev):
            k = jnp.broadcast_to(keep[0:1], x.shape[-2:])
            return jnp.where(k, x, prev)

        def prep_wqkv():
            for cb in range(14):
                cw = min(128, 3 * D - cb * 128)
                t = wqkv[:, cb * 128:cb * 128 + cw].astype(F32).T
                for j in range(NT):
                    tmpT[j, cb * 128:cb * 128 + cw, 0:_tw(j)] = t[:, j * 128:j * 128 + _tw(j)]
            for part in range(3):
                for d in range(DH):
                    if part == 0:
                        r0 = d * H
                    elif part == 1:
                        r0 = 640 + d * H if d < 16 else D + (d - 16) * H
                    else:
                        r0 = 1152 + d * H
                    v = tmpT[:, pl.ds(part * D + d, H, stride=DH), :].astype(BF)
                    for j in range(NT):
                        wpT[r0:r0 + H, j * 128:j * 128 + _tw(j)] = v[j][:, 0:_tw(j)]
            wpT[3 * D:3 * D + 64, :] = jnp.zeros((64, D), BF)

        def prep_wo():
            for j in range(NT):
                tmpT[j, 0:D, 0:_tw(j)] = wo[:, j * 128:j * 128 + _tw(j)].astype(F32)
            for j in range(NT):
                p = jnp.concatenate([tmpT[j, pl.ds(d, H, stride=DH), :] for d in range(DH)], axis=0)
                woT[j * 128:j * 128 + _tw(j), :] = p[:, 0:_tw(j)].T.astype(BF)

        def prep_mod(c0, n, one_lo, one_hi):
            cf = c_ref[...].astype(F32)
            sc_ = (cf * jax.nn.sigmoid(cf)).astype(BF)
            m = _dot(jnp.broadcast_to(sc_, (16, D)), wmod[:, c0:c0 + n])[0:8]
            col = lax.broadcasted_iota(jnp.int32, m.shape, 1)
            m = jnp.where((col >= one_lo) & (col < one_hi), m + 1.0, m)
            for t in range(n // 128):
                mt = jnp.broadcast_to(m[0:1, t * 128:(t + 1) * 128], (128, 128))
                modT[c0 + t * 128:c0 + (t + 1) * 128, :] = mt.T

        def ln_mod(xf, shift_row, scale_row):
            mean = jnp.sum(xf, axis=0, keepdims=True) * (1.0 / D)
            xc = xf - mean
            var = jnp.sum(xc * xc, axis=0, keepdims=True) * (1.0 / D)
            y = xc * lax.rsqrt(var + EPS)
            return y * modT[scale_row:scale_row + D, :] + modT[shift_row:shift_row + D, :]

        lane = lax.broadcasted_iota(jnp.int32, (1, 128), 1)

        def ln1(i):
            prev = None
            for t in range(TM // 128):
                r = i * TM + t * 128
                xf = xT[:, r:r + 128].astype(F32)
                if chain_ln and prev is not None:
                    xf = after(xf, prev)
                prev = ln_mod(xf, 0, D)
                hbuf[r:r + 128, :] = prev.T.astype(BF)

        def qkv_q(i):
            s0 = i * TM
            res = _dot_nt(hbuf[s0:s0 + TM, :], wpT[0:640, :])
            scale = DH ** -0.5
            for j in range(4):
                qbuf[j, s0:s0 + TM, :] = res[:, j * 128:(j + 1) * 128] * scale
            xt = res[:, 512:640]
            qbuf[4, s0:s0 + TM, :] = jnp.where(lane < 64, xt * scale, 0.0)
            kbuf[4, HALO + s0:HALO + s0 + TM, :] = jnp.where(lane < 64, pltpu.roll(xt, 64, 1), 0.0)

        def qkv_k(i):
            s0 = i * TM
            res = _dot_nt(hbuf[s0:s0 + TM, :], wpT[640:1152, :])
            for j in range(4):
                kbuf[j, HALO + s0:HALO + s0 + TM, :] = res[:, j * 128:(j + 1) * 128]

        def qkv_v(i):
            s0 = i * TM
            res = _dot_nt(hbuf[s0:s0 + TM, :], wpT[1152:1792, :])
            for j in range(NT):
                vbuf[j, HALO + s0:HALO + s0 + TM, :] = res[:, j * 128:(j + 1) * 128]
            if i == 0:
                for j in range(NT):
                    kbuf[j, 0:HALO, :] = jnp.broadcast_to(kbuf[j, HALO:HALO + 1, :], (HALO, 128))
                    vbuf[j, 0:HALO, :] = jnp.broadcast_to(vbuf[j, HALO:HALO + 1, :], (HALO, 128))

        def attention(i, chained):
            done = []
            for gi in range(TM // R):
                r0 = i * TM + gi * R
                q = qbuf[:, r0:r0 + R, :]
                if chained and gi >= chained:
                    q = after(q, done[gi - chained])
                ls = []
                for w in range(W):
                    a = HALO + r0 - DIL * w
                    p = jnp.sum(q * kbuf[:, a:a + R, :], axis=0)
                    p = p + pltpu.roll(p, 64, 1)
                    p = p + pltpu.roll(p, 32, 1)
                    if r0 < DIL * w:
                        row = lax.broadcasted_iota(jnp.int32, (R, 128), 0) + r0
                        p = jnp.where(row >= DIL * w, p, -1e9)
                    ls.append(p)
                m = functools.reduce(jnp.maximum, ls)
                es = [jnp.exp(l - m) for l in ls]
                den = functools.reduce(jnp.add, es)
                acc = None
                for w in range(W):
                    a = HALO + r0 - DIL * w
                    t = es[w][None] * vbuf[:, a:a + R, :]
                    acc = t if acc is None else acc + t
                done.append(acc * (1.0 / den)[None])
                o = done[-1].astype(BF)
                for j in range(NT):
                    obuf[r0:r0 + R, j * 128:j * 128 + _tw(j)] = o[j][:, 0:_tw(j)]

        def wo_proj(i):
            s0 = i * TM
            aT = _dot_nt(woT[...], obuf[s0:s0 + TM, :])
            for t in range(TM // 128):
                sl = slice(s0 + t * 128, s0 + (t + 1) * 128)
                x1[:, sl] = xT[:, sl].astype(F32) + modT[2 * D:3 * D, :] * aT[:, t * 128:(t + 1) * 128]

        def ln2(i):
            s0 = i * TM
            prev = None
            for t in range(T // 128):
                hs = []
                for half in range(2):
                    r = s0 + half * T + t * 128
                    xf = x1[:, r:r + 128]
                    if chain_ln and prev is not None:
                        xf = after(xf, prev)
                    prev = ln_mod(xf, 3 * D, 4 * D)
                    h = prev.T
                    hr[i, half * T + t * 128:half * T + (t + 1) * 128, :] = h[:, 512:D].astype(BF)
                    hs.append(h)
                a11, a12, a21, a22 = hs[0][:, 0:256], hs[0][:, 256:512], hs[1][:, 0:256], hs[1][:, 256:512]
                for n, v in enumerate((a11 + a22, a21 + a22, a11, a22, a11 + a12, a21 - a11, a12 - a22)):
                    a7[i, n, t * 128:(t + 1) * 128, :] = v.astype(BF)

        def summed(i, dst, n, o, x_ref, xi, y_ref, yi, sign):
            if i > 0:
                return dst[n, :, o]
            x, y = x_ref[xi].astype(F32), y_ref[yi].astype(F32)
            v = (x + y if sign > 0 else x - y).astype(BF)
            dst[n, :, o] = v
            return v

        def gate_up(i, p):
            a, b, o = slice(2 * p * FC, (2 * p + 1) * FC), slice((2 * p + 1) * FC, (2 * p + 2) * FC), slice(p * FC, (p + 1) * FC)
            lo, hi = slice(0, 256), slice(256, 512)
            cs = []
            for w, w5 in ((wg, wg5), (wu, wu5)):
                l = _dot(hr[i], w[512:D, 2 * p * FC:(2 * p + 2) * FC])
                m2 = _dot(a7[i, 1], w[lo, a])
                m5 = _dot(a7[i, 4], w[hi, b])
                m1 = _dot(a7[i, 0], summed(i, w5, 0, o, w, (lo, a), w, (hi, b), 1))
                m3 = _dot(a7[i, 2], summed(i, w5, 1, o, w, (lo, b), w, (hi, b), -1))
                m4 = _dot(a7[i, 3], summed(i, w5, 2, o, w, (hi, a), w, (lo, a), -1))
                m6 = _dot(a7[i, 5], summed(i, w5, 3, o, w, (lo, a), w, (lo, b), 1))
                m7 = _dot(a7[i, 6], summed(i, w5, 4, o, w, (hi, a), w, (hi, b), 1))
                cs.append((l[:T, :FC] - m5 + m1 + m4 + m7, l[:T, FC:] + m5 + m3,
                           l[T:, :FC] + m2 + m4, l[T:, FC:] - m2 + m1 + m3 + m6))
            b11, b21, b12, b22 = [g * u for g, u in zip(*cs)]
            return [v.astype(BF) for v in (b11 + b22, b11, b12 - b22, b21 - b11, b22, b11 + b12, b21 + b22)]

        def down(i, p, bs):
            a, b, o = slice(2 * p * FC, (2 * p + 1) * FC), slice((2 * p + 1) * FC, (2 * p + 2) * FC), slice(p * FC, (p + 1) * FC)
            lo, hi = slice(0, DHALF), slice(DHALF, D)
            lhs = (
                lambda: summed(i, wd5, 0, o, wdT, (lo, a), wdT, (hi, b), 1),
                lambda: summed(i, wd5, 1, o, wdT, (hi, a), wdT, (hi, b), 1),
                lambda: wdT[lo, a],
                lambda: wdT[hi, b],
                lambda: summed(i, wd5, 2, o, wdT, (lo, a), wdT, (lo, b), 1),
                lambda: summed(i, wd5, 3, o, wdT, (hi, a), wdT, (lo, a), -1),
                lambda: summed(i, wd5, 4, o, wdT, (lo, b), wdT, (hi, b), -1),
            )
            for n in (1, 3, 5, 0, 2, 4, 6):
                part = _dot_nt(lhs[n](), bs[n])
                if p == 0:
                    acc7[n] = part
                else:
                    acc7[n] += part

        out_cps = []

        def finish(i):
            s0 = i * TM
            for t in range(T // 128):
                sl = slice(t * 128, (t + 1) * 128)
                p1, p2, p3, p4, p5, p6, p7 = [acc7[n, :, sl] for n in range(7)]
                quads = ((0, 0, p1 + p4 - p5 + p7), (0, 1, p3 + p5), (1, 0, p2 + p4), (1, 1, p1 - p2 + p3 + p6))
                for dh, th, v in quads:
                    rows = slice(dh * DHALF, (dh + 1) * DHALF)
                    cols = slice(s0 + th * T + t * 128, s0 + th * T + (t + 1) * 128)
                    gate = modT[5 * D + dh * DHALF:5 * D + (dh + 1) * DHALF, :]
                    outT[rows, cols] = (x1[rows, cols] + gate * v).astype(BF)
            out_cps.append(copy_cols(outT, outT_hbm, s0, TM))

        with sc("p0_wait"):
            cp_wqkv.wait()
        with sc("p1_prep"):
            prep_wqkv()
        with sc("p2_qkv"):
            cp_m0.wait()
            cp_x0.wait()
            prep_mod(0, 2 * D, D, 2 * D)
            ln1(0)
            qkv_q(0), qkv_k(0), qkv_v(0)
        with sc("p3_wo"):
            cp_wo.wait()
            cp_m1.wait()
            for cp in cp_f[0]:
                cp.wait()
            prep_mod(2 * D, 4 * D, 2 * D, 3 * D)
            ln1(1)
            qkv_q(1), qkv_k(1)
            attention(0, chain0)
            prep_wo()
            wo_proj(0)
            qkv_v(1)
            ln2(0)
        for i in range(nb_run):
            with sc(f"p4_b{i}"):
                nxt = i + 1 < nb
                pend = None
                for p in range(nP):
                    if i == 0 and p in waits:
                        for q_ in waits[p]:
                            for cp in cp_f[q_]:
                                cp.wait()
                        if p == min(waits):
                            cp_x1.wait()
                    if nxt and i > 0 and p == qkv_at:
                        ln1(i + 1)
                        qkv_q(i + 1), qkv_k(i + 1), qkv_v(i + 1)
                    if nxt and p == wo_at:
                        attention(i + 1, chain)
                        wo_proj(i + 1)
                    bs = gate_up(i, p)
                    if swp:
                        if pend is not None:
                            down(i, p - 1, pend)
                        pend = bs
                    else:
                        down(i, p, bs)
                if swp:
                    down(i, nP - 1, pend)
                if nxt:
                    ln2(i + 1)
                finish(i)
        if nb_run < nb:
            out_cps.append(copy_cols(outT, outT_hbm, nb_run * TM, S - nb_run * TM))
        for cp in out_cps:
            cp.wait()

    n_sems = 7 + 3 * nP + nb
    hbm = pl.BlockSpec(memory_space=pltpu.HBM)

    def fn(A_x, A_wqkv, A_wo, B_x, B_w_gate, B_w_up, B_w_down, c, w_mod):
        del B_x
        outT = pl.pallas_call(
            kernel,
            in_specs=[pl.BlockSpec(memory_space=pltpu.VMEM)] + [hbm] * 7,
            out_specs=hbm,
            out_shape=jax.ShapeDtypeStruct((D, S), BF),
            scratch_shapes=[
                pltpu.VMEM((D, S), BF), pltpu.VMEM((D, 3 * D), BF), pltpu.VMEM((D, D), BF),
                pltpu.VMEM((D, F), BF), pltpu.VMEM((D, F), BF), pltpu.VMEM((D, F), BF),
                pltpu.VMEM((D, 6 * D), BF),
                pltpu.VMEM((NT, 1792, 128), F32), pltpu.VMEM((1792, D), BF), pltpu.VMEM((D, D), BF),
                pltpu.VMEM((6 * D, 128), F32),
                pltpu.VMEM((5, 256, F // 2), BF), pltpu.VMEM((5, 256, F // 2), BF), pltpu.VMEM((5, DHALF, F // 2), BF),
                pltpu.VMEM((NT, S, 128), F32), pltpu.VMEM((NT, HALO + S, 128), F32),
                pltpu.VMEM((NT, HALO + S, 128), F32),
                pltpu.VMEM((S, D), BF), pltpu.VMEM((S, D), BF),
                pltpu.VMEM((D, S), F32),
                pltpu.VMEM((nb, 7, T, 256), BF), pltpu.VMEM((nb, TM, 64), BF),
                pltpu.VMEM((7, DHALF, T), F32), pltpu.VMEM((D, S), BF),
                pltpu.SemaphoreType.DMA((n_sems,)),
            ],
            compiler_params=pltpu.CompilerParams(vmem_limit_bytes=120 * 2**20, flags=flags),
            name=name,
        )(c, A_x[0].T, A_wqkv, A_wo, B_w_gate, B_w_up, B_w_down.T, w_mod)
        return outT.T[None]

    return fn


@jax.jit
def pallas_adaLN_cond__sliding_local_dilated__glu_gated_bilinear__prompt_kernel(
    A_x: jax.Array,
    A_wqkv: jax.Array,
    A_wo: jax.Array,
    B_x: jax.Array,
    B_w_gate: jax.Array,
    B_w_up: jax.Array,
    B_w_down: jax.Array,
    c: jax.Array,
    w_mod: jax.Array,
):
    return make(chain=1, swp=True, R=8, chain0=4, qkv_at=1)(A_x, A_wqkv, A_wo, B_x, B_w_gate, B_w_up, B_w_down, c, w_mod)
```

```python
import contextlib
import functools

import jax
import jax.numpy as jnp
from jax import lax
import jax.experimental.pallas as pl
import jax.experimental.pallas.tpu as pltpu

S, D, H, DH, W, DIL, F = 2048, 576, 32, 18, 8, 2, 4608
HALO = 16
NT = 5
DHALF = D // 2
EPS = 1e-5
BF, F32, I32 = jnp.bfloat16, jnp.float32, jnp.int32
NT_DIMS = (((1,), (1,)), ((), ()))


def _tw(j):
    return min(128, D - 128 * j)


def _dot(a, b):
    return jnp.dot(a, b, preferred_element_type=F32)


def _dot_nt(a, b):
    return lax.dot_general(a, b, NT_DIMS, preferred_element_type=F32)


def _pack(v):
    return pltpu.bitcast(v, jnp.int32)


def _unpack(v):
    return pltpu.bitcast(v, BF)


def _colsum(x):
    return jnp.sum(jnp.sum(x.reshape(D // 32, 32, 128), axis=0), axis=0, keepdims=True)


def make(TM=512, FC=384, R=8, chain=1, chain0=4, waits=None, nb_run=None, flags=None, name="k4",
         scopes=False, wo_at=None, qkv_at=1, pro=256, prio=0, prio2=0, wo_at0=2):
    nb = S // TM
    T = TM // 2
    nP = F // (2 * FC)
    nb_run = nb if nb_run is None else nb_run
    wo_at = (2 * nP) // 3 if wo_at is None else wo_at
    waits = {0: [0, 1], 2: list(range(2, nP))} if waits is None else waits
    assert max(waits) > 0 and sorted(sum(waits.values(), [])) == list(range(nP))

    def kernel(c_ref, xT_hbm, wqkv_hbm, wo_hbm, wg_hbm, wu_hbm, wdT_hbm, wmod_hbm, outT_hbm,
               xT, wqkv, wo, wg, wu, wdT, wmod, tmpT, wpT, woT, modR, gateT, wg7, wu7, wr, wd7,
               ybuf, qbuf, kbuf, vbuf, hbuf, obuf, x1, a7, hr, acc7, outT, sems):
        sc = jax.named_scope if scopes else (lambda n: contextlib.nullcontext())
        sem_i = [0]

        def copy_cols(src, dst, c0, n, priority=0):
            cp = pltpu.make_async_copy(src.at[:, pl.ds(c0, n)], dst.at[:, pl.ds(c0, n)], sems.at[sem_i[0]])
            sem_i[0] += 1
            cp.start(priority=priority)
            return cp

        cp_x0 = copy_cols(xT_hbm, xT, 0, TM)
        cp_m0 = copy_cols(wmod_hbm, wmod, 0, 2 * D)
        cp_q = copy_cols(wqkv_hbm, wqkv, 0, 640)
        cp_k = copy_cols(wqkv_hbm, wqkv, 640, 512)
        cp_v = copy_cols(wqkv_hbm, wqkv, 1152, D)
        cp_x1 = copy_cols(xT_hbm, xT, TM, TM)
        cp_wo = copy_cols(wo_hbm, wo, 0, D, prio2)
        cp_m1 = copy_cols(wmod_hbm, wmod, 2 * D, 4 * D, prio2)
        cp_f = []
        for p in range(nP):
            cp_f.append([copy_cols(s, d, 2 * p * FC, 2 * FC, prio) for s, d in ((wg_hbm, wg), (wu_hbm, wu), (wdT_hbm, wdT))])
            if p == nP - 1:
                cp_x2 = copy_cols(xT_hbm, xT, 2 * TM, S - 2 * TM, prio)

        cbits = pltpu.bitcast(jnp.broadcast_to(c_ref[:, 0:128].astype(F32), (8, 128)), jnp.int32)
        keep = ((cbits * cbits) & 2) == 0

        def after(x, prev):
            k = jnp.broadcast_to(keep[0:1], x.shape[-2:])
            return jnp.where(k, x, prev)

        def prep_wqkv(part):
            for cb in (range(0, 5), range(5, 9), range(9, 14))[part]:
                cw = min(128, 3 * D - cb * 128)
                t = wqkv[:, cb * 128:cb * 128 + cw].astype(F32).T
                for j in range(NT):
                    tmpT[j, cb * 128:cb * 128 + cw, 0:_tw(j)] = t[:, j * 128:j * 128 + _tw(j)]
            for d in range(DH):
                if part == 0:
                    r0 = d * H
                elif part == 1:
                    r0 = 640 + d * H if d < 16 else D + (d - 16) * H
                else:
                    r0 = 1152 + d * H
                v = tmpT[:, pl.ds(part * D + d, H, stride=DH), :].astype(BF)
                for j in range(NT):
                    wpT[r0 // 2:(r0 + H) // 2, j * 128:j * 128 + _tw(j)] = _pack(v[j])[:, 0:_tw(j)]
            if part == 2:
                wpT[3 * D // 2:3 * D // 2 + 32, :] = jnp.zeros((32, D), jnp.int32)

        def prep_wo():
            for j in range(NT):
                tmpT[j, 0:D, 0:_tw(j)] = wo[:, j * 128:j * 128 + _tw(j)].astype(F32)
            for j in range(NT):
                p = jnp.concatenate([tmpT[j, pl.ds(d, H, stride=DH), :] for d in range(DH)], axis=0)
                woT[j * 64:j * 64 + _tw(j) // 2, :] = _pack(p[:, 0:_tw(j)].T.astype(BF))

        def modulation(c0, n):
            cf = c_ref[...].astype(F32)
            s = (cf * jax.nn.sigmoid(cf)).astype(BF)
            return _dot(jnp.broadcast_to(s, (16, D)), wmod[:, c0:c0 + n])[0:8]

        def to_column(row, n):
            for j in range(NT):
                r = row[0:1, j * 128:j * 128 + _tw(j)]
                gateT[n, j * 128:j * 128 + _tw(j), :] = jnp.broadcast_to(r, (128, _tw(j))).T

        def prep_mod0():
            m = modulation(0, 2 * D)
            modR[0] = m[:, 0:D]
            modR[1] = 1.0 + m[:, D:2 * D]

        def prep_mod1():
            m = modulation(2 * D, 4 * D)
            modR[2] = m[:, D:2 * D]
            modR[3] = 1.0 + m[:, 2 * D:3 * D]
            to_column(m[:, 0:D], 0)
            to_column(m[:, 3 * D:4 * D], 1)

        def normalize(xf):
            mean = _colsum(xf) * (1.0 / D)
            xc = xf - mean
            var = _colsum(xc * xc) * (1.0 / D)
            return (xc * lax.rsqrt(var + EPS)).T

        def modulate(y, n):
            return y * modR[2 * n + 1, 0:1, :] + modR[2 * n, 0:1, :]

        lane = lax.broadcasted_iota(jnp.int32, (1, 128), 1)

        def ln1(i):
            for t in range(TM // 128):
                r = i * TM + t * 128
                hbuf[r // 2:r // 2 + 64, :] = _pack(modulate(normalize(xT[:, r:r + 128].astype(F32)), 0).astype(BF))

        def qkv_q(i):
            s0 = i * TM
            res = _dot_nt(_unpack(hbuf[s0 // 2:(s0 + TM) // 2, :]), _unpack(wpT[0:256, :]))
            for j in range(4):
                qbuf[j, s0:s0 + TM, :] = res[:, j * 128:(j + 1) * 128] * DH ** -0.5

        def qkv_k(i):
            s0 = i * TM
            res = _dot_nt(_unpack(hbuf[s0 // 2:(s0 + TM) // 2, :]), _unpack(wpT[256:576, :]))
            xt = res[:, 0:128]
            qbuf[4, s0:s0 + TM, :] = jnp.where(lane < 64, xt * DH ** -0.5, 0.0)
            kbuf[4, HALO + s0:HALO + s0 + TM, :] = jnp.where(lane < 64, pltpu.roll(xt, 64, 1), 0.0)
            for j in range(4):
                kbuf[j, HALO + s0:HALO + s0 + TM, :] = res[:, (j + 1) * 128:(j + 2) * 128]

        def qkv_v(i, lo=0, hi=TM):
            s0 = i * TM
            res = _dot_nt(_unpack(hbuf[(s0 + lo) // 2:(s0 + hi) // 2, :]), _unpack(wpT[576:896, :]))
            for j in range(NT):
                vbuf[j, HALO + s0 + lo:HALO + s0 + hi, :] = res[:, j * 128:(j + 1) * 128]
            if i == 0:
                for j in range(NT):
                    kbuf[j, 0:HALO, :] = jnp.broadcast_to(kbuf[j, HALO:HALO + 1, :], (HALO, 128))
                    vbuf[j, 0:HALO, :] = jnp.broadcast_to(vbuf[j, HALO:HALO + 1, :], (HALO, 128))

        def attention(i, chained):
            done = []
            for gi in range(TM // R):
                r0 = i * TM + gi * R
                q = qbuf[:, r0:r0 + R, :]
                if chained and gi >= chained:
                    q = after(q, done[gi - chained])
                ls = []
                for w in range(W):
                    a = HALO + r0 - DIL * w
                    p = jnp.sum(q * kbuf[:, a:a + R, :], axis=0)
                    p = p + pltpu.roll(p, 64, 1)
                    p = p + pltpu.roll(p, 32, 1)
                    if r0 < DIL * w:
                        row = lax.broadcasted_iota(jnp.int32, (R, 128), 0) + r0
                        p = jnp.where(row >= DIL * w, p, -1e9)
                    ls.append(p)
                m = functools.reduce(jnp.maximum, ls)
                es = [jnp.exp(l - m) for l in ls]
                den = functools.reduce(jnp.add, es)
                acc = None
                for w in range(W):
                    a = HALO + r0 - DIL * w
                    t = es[w][None] * vbuf[:, a:a + R, :]
                    acc = t if acc is None else acc + t
                done.append(acc * (1.0 / den)[None])
                if R % 16 == 0:
                    o, ro, rn = done[-1].astype(BF), r0, R
                elif gi % 2 == 1:
                    o, ro, rn = jnp.concatenate(done[-2:], axis=1).astype(BF), r0 - R, 2 * R
                else:
                    continue
                for j in range(NT):
                    obuf[ro // 2:(ro + rn) // 2, j * 128:j * 128 + _tw(j)] = _pack(o[j])[:, 0:_tw(j)]

        def wo_proj(i):
            s0 = i * TM
            aT = _dot_nt(_unpack(woT[...]), _unpack(obuf[s0 // 2:(s0 + TM) // 2, :]))
            for t in range(TM // 128):
                sl = slice(s0 + t * 128, s0 + (t + 1) * 128)
                x1[:, sl] = xT[:, sl].astype(F32) + gateT[0] * aT[:, t * 128:(t + 1) * 128]

        def ln2(i):
            s0 = i * TM
            for t in range(T // 128):
                hs = []
                for half in range(2):
                    r = s0 + half * T + t * 128
                    h = modulate(normalize(x1[:, r:r + 128]), 1)
                    hr[i, (half * T + t * 128) // 2:(half * T + (t + 1) * 128) // 2, :] = _pack(h[:, 512:D].astype(BF))
                    hs.append(h)
                a11, a12, a21, a22 = hs[0][:, 0:256], hs[0][:, 256:512], hs[1][:, 0:256], hs[1][:, 256:512]
                for n, v in enumerate((a11 + a22, a21 + a22, a11, a22, a11 + a12, a21 - a11, a12 - a22)):
                    a7[i, n, t * 64:(t + 1) * 64, :] = _pack(v.astype(BF))

        def operand(i, dst, n, o, w, xi, yi=None, sign=1):
            if i > 0:
                return _unpack(dst[n, :, o])
            v = w[xi]
            if yi is not None:
                x, y = v.astype(F32), w[yi].astype(F32)
                v = (x + y if sign > 0 else x - y).astype(BF)
            dst[n, :, o] = _pack(v)
            return v

        def gate_up(i, p):
            a, b, o = slice(2 * p * FC, (2 * p + 1) * FC), slice((2 * p + 1) * FC, (2 * p + 2) * FC), slice(p * FC, (p + 1) * FC)
            ab = slice(2 * p * FC, (2 * p + 2) * FC)
            lo, hi = slice(0, 256), slice(256, 512)
            cs = []
            for n, (w, w7) in enumerate(((wg, wg7), (wu, wu7))):
                l = _dot(_unpack(hr[i]), operand(i, wr, n, ab, w, (slice(512, D), ab)))
                m2 = _dot(_unpack(a7[i, 1]), operand(i, w7, 1, o, w, (lo, a)))
                m5 = _dot(_unpack(a7[i, 4]), operand(i, w7, 4, o, w, (hi, b)))
                m1 = _dot(_unpack(a7[i, 0]), operand(i, w7, 0, o, w, (lo, a), (hi, b), 1))
                m3 = _dot(_unpack(a7[i, 2]), operand(i, w7, 2, o, w, (lo, b), (hi, b), -1))
                m4 = _dot(_unpack(a7[i, 3]), operand(i, w7, 3, o, w, (hi, a), (lo, a), -1))
                m6 = _dot(_unpack(a7[i, 5]), operand(i, w7, 5, o, w, (lo, a), (lo, b), 1))
                m7 = _dot(_unpack(a7[i, 6]), operand(i, w7, 6, o, w, (hi, a), (hi, b), 1))
                cs.append((l[:T, :FC] - m5 + m1 + m4 + m7, l[:T, FC:] + m5 + m3,
                           l[T:, :FC] + m2 + m4, l[T:, FC:] - m2 + m1 + m3 + m6))
            b11, b21, b12, b22 = [g * u for g, u in zip(*cs)]
            return [v.astype(BF) for v in (b11 + b22, b11, b12 - b22, b21 - b11, b22, b11 + b12, b21 + b22)]

        def down(i, p, bs):
            a, b, o = slice(2 * p * FC, (2 * p + 1) * FC), slice((2 * p + 1) * FC, (2 * p + 2) * FC), slice(p * FC, (p + 1) * FC)
            lo, hi = slice(0, DHALF), slice(DHALF, D)
            lhs = (((lo, a), (hi, b), 1), ((hi, a), (hi, b), 1), ((lo, a),), ((hi, b),),
                   ((lo, a), (lo, b), 1), ((hi, a), (lo, a), -1), ((lo, b), (hi, b), -1))
            for n in (1, 3, 5, 0, 2, 4, 6):
                part = _dot_nt(operand(i, wd7, n, o, wdT, *lhs[n]), bs[n])
                if p == 0:
                    acc7[n] = part
                else:
                    acc7[n] += part

        out_cps = []

        def finish(i):
            s0 = i * TM
            for t in range(T // 128):
                sl = slice(t * 128, (t + 1) * 128)
                p1, p2, p3, p4, p5, p6, p7 = [acc7[n, :, sl] for n in range(7)]
                quads = ((0, 0, p1 + p4 - p5 + p7), (0, 1, p3 + p5), (1, 0, p2 + p4), (1, 1, p1 - p2 + p3 + p6))
                for dh, th, v in quads:
                    rows = slice(dh * DHALF, (dh + 1) * DHALF)
                    cols = slice(s0 + th * T + t * 128, s0 + th * T + (t + 1) * 128)
                    outT[rows, cols] = (x1[rows, cols] + gateT[1, rows, :] * v).astype(BF)
            out_cps.append(copy_cols(outT, outT_hbm, s0, TM))

        with sc("p0_x"):
            cp_x0.wait()
            for t in range(TM // 128):
                ybuf[t * 128:(t + 1) * 128, :] = normalize(xT[:, t * 128:(t + 1) * 128].astype(F32))
        with sc("p1_m"):
            cp_m0.wait()
            prep_mod0()
            hbuf[0:TM // 2, :] = _pack(modulate(ybuf[...], 0).astype(BF))
        with sc("p2_pq"):
            cp_q.wait()
            prep_wqkv(0)
        with sc("p2_q"):
            cp_k.wait()
            prep_wqkv(1)
            qkv_q(0)
        with sc("p2_kv"):
            cp_v.wait()
            cp_x1.wait()
            prep_wqkv(2)
            qkv_k(0), qkv_v(0)
            ln1(1)
            qkv_q(1), qkv_k(1)
            if pro > 0:
                qkv_v(1, 0, pro)
            attention(0, chain0)
        with sc("p3_wo"):
            cp_wo.wait()
            cp_m1.wait()
            for q_ in waits[0]:
                for cp in cp_f[q_]:
                    cp.wait()
            prep_mod1()
            prep_wo()
            wo_proj(0)
            if pro < TM:
                qkv_v(1, pro, TM)
            ln2(0)
        for i in range(nb_run):
            with sc(f"p4_b{i}"):
                nxt = i + 1 < nb
                pend = None
                for p in range(nP):
                    if nxt and i > 0 and p == qkv_at:
                        ln1(i + 1)
                        qkv_q(i + 1), qkv_k(i + 1), qkv_v(i + 1)
                    if nxt and p == (wo_at if i > 0 else wo_at0):
                        attention(i + 1, chain)
                        wo_proj(i + 1)
                    if i == 0 and p > 0 and p in waits:
                        for q_ in waits[p]:
                            for cp in cp_f[q_]:
                                cp.wait()
                        if p == max(waits):
                            cp_x2.wait()
                    bs = gate_up(i, p)
                    if pend is not None:
                        down(i, p - 1, pend)
                    pend = bs
                down(i, nP - 1, pend)
                if nxt:
                    ln2(i + 1)
                finish(i)
        if nb_run < nb:
            out_cps.append(copy_cols(outT, outT_hbm, nb_run * TM, S - nb_run * TM))
        for cp in out_cps:
            cp.wait()

    n_sems = 10 + 3 * nP + nb
    hbm = pl.BlockSpec(memory_space=pltpu.HBM)

    def fn(A_x, A_wqkv, A_wo, B_x, B_w_gate, B_w_up, B_w_down, c, w_mod):
        del B_x
        outT = pl.pallas_call(
            kernel,
            in_specs=[pl.BlockSpec(memory_space=pltpu.VMEM)] + [hbm] * 7,
            out_specs=hbm,
            out_shape=jax.ShapeDtypeStruct((D, S), BF),
            scratch_shapes=[
                pltpu.VMEM((D, S), BF), pltpu.VMEM((D, 3 * D), BF), pltpu.VMEM((D, D), BF),
                pltpu.VMEM((D, F), BF), pltpu.VMEM((D, F), BF), pltpu.VMEM((D, F), BF),
                pltpu.VMEM((D, 6 * D), BF),
                pltpu.VMEM((NT, 1792, 128), F32), pltpu.VMEM((896, D), I32), pltpu.VMEM((D // 2, D), I32),
                pltpu.VMEM((4, 8, D), F32), pltpu.VMEM((2, D, 128), F32),
                pltpu.VMEM((7, 128, F // 2), I32), pltpu.VMEM((7, 128, F // 2), I32), pltpu.VMEM((2, 32, F), I32),
                pltpu.VMEM((7, DHALF // 2, F // 2), I32),
                pltpu.VMEM((TM, D), F32),
                pltpu.VMEM((NT, S, 128), F32), pltpu.VMEM((NT, HALO + S, 128), F32),
                pltpu.VMEM((NT, HALO + S, 128), F32),
                pltpu.VMEM((S // 2, D), I32), pltpu.VMEM((S // 2, D), I32),
                pltpu.VMEM((D, S), F32),
                pltpu.VMEM((nb, 7, T // 2, 256), I32), pltpu.VMEM((nb, TM // 2, 64), I32),
                pltpu.VMEM((7, DHALF, T), F32), pltpu.VMEM((D, S), BF),
                pltpu.SemaphoreType.DMA((n_sems,)),
            ],
            compiler_params=pltpu.CompilerParams(vmem_limit_bytes=120 * 2**20, flags=flags),
            name=name,
        )(c, A_x[0].T, A_wqkv, A_wo, B_w_gate, B_w_up, B_w_down.T, w_mod)
        return outT.T[None]

    return fn


@jax.jit
def pallas_adaLN_cond__sliding_local_dilated__glu_gated_bilinear__prompt_kernel(
    A_x: jax.Array,
    A_wqkv: jax.Array,
    A_wo: jax.Array,
    B_x: jax.Array,
    B_w_gate: jax.Array,
    B_w_up: jax.Array,
    B_w_down: jax.Array,
    c: jax.Array,
    w_mod: jax.Array,
):
    return make(chain0=3, pro=512, waits={0: [0], 1: [1, 2], 3: [3, 4, 5]}, wo_at0=5)(A_x, A_wqkv, A_wo, B_x, B_w_gate, B_w_up, B_w_down, c, w_mod)
```

```python
import contextlib
import functools

import jax
import jax.numpy as jnp
from jax import lax
import jax.experimental.pallas as pl
import jax.experimental.pallas.tpu as pltpu

S, D, H, DH, W, DIL, F = 2048, 576, 32, 18, 8, 2, 4608
HALO = 16
NT = 5
DHALF = D // 2
EPS = 1e-5
BF, F32, I32 = jnp.bfloat16, jnp.float32, jnp.int32
NT_DIMS = (((1,), (1,)), ((), ()))


def _tw(j):
    return min(128, D - 128 * j)


def _dot(a, b):
    return jnp.dot(a, b, preferred_element_type=F32)


def _dot_nt(a, b):
    return lax.dot_general(a, b, NT_DIMS, preferred_element_type=F32)


def _pack(v):
    return pltpu.bitcast(v, jnp.int32)


def _unpack(v):
    return pltpu.bitcast(v, BF)


def _colsum(x):
    return jnp.sum(jnp.sum(x.reshape(D // 32, 32, 128), axis=0), axis=0, keepdims=True)


KS = (256, 256, 384, 384, 192, 384, 256)
KO = (0, 256, 512, 896, 1280, 1536, 1920)
KT = 2176
S1A, S2A, S1B, R1, S2B, R2, R3 = (
    slice(0, 128), slice(128, 256), slice(256, 320), slice(320, 384), slice(384, 448), slice(448, 512), slice(512, 576))
RIGHT = (
    ((S1A, 0, 1, S2A, 1), (S1B, 0, 1, S2B, 1), (R1, 0)),
    ((S1A, 0), (S1B, 0), (R2, 0)),
    ((S1A, 1, -1, S2A, 1), (S1B, 1, -1, S2B, 1), (R1, 1), (R3, 1), (R2, 1)),
    ((S2A, 0, -1, S1A, 0), (S2B, 0, -1, S1B, 0), (R2, 0), (R3, 0), (R1, 0)),
    ((S2A, 1), (S2B, 1)),
    ((S1A, 0, 1, S1A, 1), (S1B, 0, 1, S1B, 1), (R1, 0, 1, R1, 1), (R3, 1), (R2, 0, 1, R2, 1)),
    ((S2A, 0, 1, S2A, 1), (S2B, 0, 1, S2B, 1), (R3, 0)),
)


def _left_operands(p, q, lo):
    d = [y - x for x, y in zip(p, q)]
    w = lambda a, b: jnp.where(lo, a, b)
    return (
        (p[0] + q[1], w(p[2] + q[3], p[2] - q[2])),
        (q[0] + q[1], w(q[2] + q[3], d[3])),
        (p[0], p[2], w(p[4], p[3])),
        (q[1], w(q[3], p[3]), w(q[4], q[2])),
        (p[0] + p[1], p[2] + p[3]),
        (d[0], d[2], w(d[4], d[3])),
        (d[1], w(d[3], d[4])),
    )


def make(TM=512, FC=384, R=8, chain=1, chain0=3, waits=None, nb_run=None, flags=None, name="k5",
         scopes=False, wo_at=None, qkv_at=1, pro=512, prio=0, prio2=0, wo_at0=5):
    nb = S // TM
    T = TM // 2
    nP = F // (2 * FC)
    nb_run = nb if nb_run is None else nb_run
    wo_at = (2 * nP) // 3 if wo_at is None else wo_at
    waits = {0: [0], 1: [1, 2], 3: [3, 4, 5]} if waits is None else waits
    assert max(waits) > 0 and sorted(sum(waits.values(), [])) == list(range(nP))

    def kernel(c_ref, xT_hbm, wqkv_hbm, wo_hbm, wg_hbm, wu_hbm, wdT_hbm, wmod_hbm, outT_hbm,
               xT, wqkv, wo, wg, wu, wdT, wmod, tmpT, wpT, woT, modR, gateT, wg17, wu17, wd7,
               ybuf, qbuf, kbuf, vbuf, hbuf, obuf, x1, a17, acc7, outT, sems):
        sc = jax.named_scope if scopes else (lambda n: contextlib.nullcontext())
        sem_i = [0]

        def copy_cols(src, dst, c0, n, priority=0):
            cp = pltpu.make_async_copy(src.at[:, pl.ds(c0, n)], dst.at[:, pl.ds(c0, n)], sems.at[sem_i[0]])
            sem_i[0] += 1
            cp.start(priority=priority)
            return cp

        cp_x0 = copy_cols(xT_hbm, xT, 0, TM)
        cp_m0 = copy_cols(wmod_hbm, wmod, 0, 2 * D)
        cp_q = copy_cols(wqkv_hbm, wqkv, 0, 640)
        cp_k = copy_cols(wqkv_hbm, wqkv, 640, 512)
        cp_v = copy_cols(wqkv_hbm, wqkv, 1152, D)
        cp_x1 = copy_cols(xT_hbm, xT, TM, TM)
        cp_wo = copy_cols(wo_hbm, wo, 0, D, prio2)
        cp_m1 = copy_cols(wmod_hbm, wmod, 2 * D, 4 * D, prio2)
        cp_f = []
        for p in range(nP):
            cp_f.append([copy_cols(s, d, 2 * p * FC, 2 * FC, prio) for s, d in ((wg_hbm, wg), (wu_hbm, wu), (wdT_hbm, wdT))])
            if p == nP - 1:
                cp_x2 = copy_cols(xT_hbm, xT, 2 * TM, S - 2 * TM, prio)

        cbits = pltpu.bitcast(jnp.broadcast_to(c_ref[:, 0:128].astype(F32), (8, 128)), jnp.int32)
        keep = ((cbits * cbits) & 2) == 0

        def after(x, prev):
            k = jnp.broadcast_to(keep[0:1], x.shape[-2:])
            return jnp.where(k, x, prev)

        def prep_wqkv(part):
            for cb in (range(0, 5), range(5, 9), range(9, 14))[part]:
                cw = min(128, 3 * D - cb * 128)
                t = wqkv[:, cb * 128:cb * 128 + cw].astype(F32).T
                for j in range(NT):
                    tmpT[j, cb * 128:cb * 128 + cw, 0:_tw(j)] = t[:, j * 128:j * 128 + _tw(j)]
            for d in range(DH):
                if part == 0:
                    r0 = d * H
                elif part == 1:
                    r0 = 640 + d * H if d < 16 else D + (d - 16) * H
                else:
                    r0 = 1152 + d * H
                v = tmpT[:, pl.ds(part * D + d, H, stride=DH), :].astype(BF)
                for j in range(NT):
                    wpT[r0 // 2:(r0 + H) // 2, j * 128:j * 128 + _tw(j)] = _pack(v[j])[:, 0:_tw(j)]
            if part == 2:
                wpT[3 * D // 2:3 * D // 2 + 32, :] = jnp.zeros((32, D), jnp.int32)

        def prep_wo():
            for j in range(NT):
                tmpT[j, 0:D, 0:_tw(j)] = wo[:, j * 128:j * 128 + _tw(j)].astype(F32)
            for j in range(NT):
                p = jnp.concatenate([tmpT[j, pl.ds(d, H, stride=DH), :] for d in range(DH)], axis=0)
                woT[j * 64:j * 64 + _tw(j) // 2, :] = _pack(p[:, 0:_tw(j)].T.astype(BF))

        def modulation(c0, n):
            cf = c_ref[...].astype(F32)
            s = (cf * jax.nn.sigmoid(cf)).astype(BF)
            return _dot(jnp.broadcast_to(s, (16, D)), wmod[:, c0:c0 + n])[0:8]

        def to_column(row, n):
            for j in range(NT):
                r = row[0:1, j * 128:j * 128 + _tw(j)]
                gateT[n, j * 128:j * 128 + _tw(j), :] = jnp.broadcast_to(r, (128, _tw(j))).T

        def widen(row):
            return jnp.concatenate([row, row[:, 512:D]], axis=1)

        def prep_mod0():
            m = modulation(0, 2 * D)
            modR[0] = widen(m[:, 0:D])
            modR[1] = widen(1.0 + m[:, D:2 * D])

        def prep_mod1():
            m = modulation(2 * D, 4 * D)
            modR[2] = widen(m[:, D:2 * D])
            modR[3] = widen(1.0 + m[:, 2 * D:3 * D])
            to_column(m[:, 0:D], 0)
            to_column(m[:, 3 * D:4 * D], 1)

        def normalize(xf):
            mean = _colsum(xf) * (1.0 / D)
            xc = xf - mean
            var = _colsum(xc * xc) * (1.0 / D)
            return xc * lax.rsqrt(var + EPS)

        def modulate(y, n):
            return y * modR[2 * n + 1, 0:1, 0:D] + modR[2 * n, 0:1, 0:D]

        def modulated_tiles(y, n):
            parts = [y[j * 128:(j + 1) * 128] for j in range(4)] + [jnp.concatenate([y[512:D], y[512:D]], axis=0)]
            return [t.T * modR[2 * n + 1, 0:1, j * 128:(j + 1) * 128] + modR[2 * n, 0:1, j * 128:(j + 1) * 128]
                    for j, t in enumerate(parts)]

        lane = lax.broadcasted_iota(jnp.int32, (1, 128), 1)

        def ln1(i):
            for t in range(TM // 128):
                r = i * TM + t * 128
                hbuf[r // 2:r // 2 + 64, :] = _pack(modulate(normalize(xT[:, r:r + 128].astype(F32)).T, 0).astype(BF))

        def qkv_q(i):
            s0 = i * TM
            res = _dot_nt(_unpack(hbuf[s0 // 2:(s0 + TM) // 2, :]), _unpack(wpT[0:256, :]))
            for j in range(4):
                qbuf[j, s0:s0 + TM, :] = res[:, j * 128:(j + 1) * 128] * DH ** -0.5

        def qkv_k(i):
            s0 = i * TM
            res = _dot_nt(_unpack(hbuf[s0 // 2:(s0 + TM) // 2, :]), _unpack(wpT[256:576, :]))
            xt = res[:, 0:128]
            qbuf[4, s0:s0 + TM, :] = jnp.where(lane < 64, xt * DH ** -0.5, 0.0)
            kbuf[4, HALO + s0:HALO + s0 + TM, :] = jnp.where(lane < 64, pltpu.roll(xt, 64, 1), 0.0)
            for j in range(4):
                kbuf[j, HALO + s0:HALO + s0 + TM, :] = res[:, (j + 1) * 128:(j + 2) * 128]

        def qkv_v(i, lo=0, hi=TM):
            s0 = i * TM
            res = _dot_nt(_unpack(hbuf[(s0 + lo) // 2:(s0 + hi) // 2, :]), _unpack(wpT[576:896, :]))
            for j in range(NT):
                vbuf[j, HALO + s0 + lo:HALO + s0 + hi, :] = res[:, j * 128:(j + 1) * 128]
            if i == 0:
                for j in range(NT):
                    kbuf[j, 0:HALO, :] = jnp.broadcast_to(kbuf[j, HALO:HALO + 1, :], (HALO, 128))
                    vbuf[j, 0:HALO, :] = jnp.broadcast_to(vbuf[j, HALO:HALO + 1, :], (HALO, 128))

        def attention(i, chained):
            done = []
            for gi in range(TM // R):
                r0 = i * TM + gi * R
                q = qbuf[:, r0:r0 + R, :]
                if chained and gi >= chained:
                    q = after(q, done[gi - chained])
                ls = []
                for w in range(W):
                    a = HALO + r0 - DIL * w
                    p = jnp.sum(q * kbuf[:, a:a + R, :], axis=0)
                    p = p + pltpu.roll(p, 64, 1)
                    p = p + pltpu.roll(p, 32, 1)
                    if r0 < DIL * w:
                        row = lax.broadcasted_iota(jnp.int32, (R, 128), 0) + r0
                        p = jnp.where(row >= DIL * w, p, -1e9)
                    ls.append(p)
                m = functools.reduce(jnp.maximum, ls)
                es = [jnp.exp(l - m) for l in ls]
                den = functools.reduce(jnp.add, es)
                acc = None
                for w in range(W):
                    a = HALO + r0 - DIL * w
                    t = es[w][None] * vbuf[:, a:a + R, :]
                    acc = t if acc is None else acc + t
                done.append(acc * (1.0 / den)[None])
                if R % 16 == 0:
                    o, ro, rn = done[-1].astype(BF), r0, R
                elif gi % 2 == 1:
                    o, ro, rn = jnp.concatenate(done[-2:], axis=1).astype(BF), r0 - R, 2 * R
                else:
                    continue
                for j in range(NT):
                    obuf[ro // 2:(ro + rn) // 2, j * 128:j * 128 + _tw(j)] = _pack(o[j])[:, 0:_tw(j)]

        def wo_proj(i):
            s0 = i * TM
            aT = _dot_nt(_unpack(woT[...]), _unpack(obuf[s0 // 2:(s0 + TM) // 2, :]))
            for t in range(TM // 128):
                sl = slice(s0 + t * 128, s0 + (t + 1) * 128)
                x1[:, sl] = xT[:, sl].astype(F32) + gateT[0] * aT[:, t * 128:(t + 1) * 128]

        def ln2(i):
            s0 = i * TM
            for t in range(T // 128):
                p, q = [modulated_tiles(normalize(x1[:, r:r + 128]), 1) for r in (s0 + t * 128, s0 + T + t * 128)]
                for n, tiles in enumerate(_left_operands(p, q, lane < 64)):
                    for j, v in enumerate(tiles):
                        c0 = KO[n] + j * 128
                        a17[i, t * 64:(t + 1) * 64, c0:c0 + 128] = _pack(v.astype(BF))

        def combine(x, sign=None, y=None):
            if sign is None:
                return x
            x, y = x.astype(F32), y.astype(F32)
            return (x + y if sign > 0 else x - y).astype(BF)

        def operand(i, dst, n, o, w, xi, yi=None, sign=None):
            if i > 0:
                return _unpack(dst[n, :, o])
            v = combine(w[xi], sign, None if yi is None else w[yi])
            dst[n, :, o] = _pack(v)
            return v

        def gate_up(i, p):
            cols = (slice(2 * p * FC, (2 * p + 1) * FC), slice((2 * p + 1) * FC, (2 * p + 2) * FC))
            o = slice(p * FC, (p + 1) * FC)
            cs = []
            for w, w17 in ((wg, wg17), (wu, wu17)):
                m = {}
                for n in (1, 4, 0, 2, 3, 5, 6):
                    rows = slice(KO[n] // 2, (KO[n] + KS[n]) // 2)
                    if i > 0:
                        rhs = _unpack(w17[rows, o])
                    else:
                        rhs = jnp.concatenate(
                            [combine(w[e[0], cols[e[1]]], *((e[2], w[e[3], cols[e[4]]]) if len(e) > 2 else ()))
                             for e in RIGHT[n]], axis=0)
                        w17[rows, o] = _pack(rhs)
                    m[n + 1] = _dot(_unpack(a17[i, :, KO[n]:KO[n] + KS[n]]), rhs)
                cs.append((m[1] - m[5] + m[4] - m[7], m[5] + m[3], m[2] + m[4], m[1] - m[2] + m[3] + m[6]))
            b11, b21, b12, b22 = [g * u for g, u in zip(*cs)]
            return [v.astype(BF) for v in (b11 + b22, b11, b12 - b22, b21 - b11, b22, b11 + b12, b21 + b22)]

        def down(i, p, bs):
            a, b, o = slice(2 * p * FC, (2 * p + 1) * FC), slice((2 * p + 1) * FC, (2 * p + 2) * FC), slice(p * FC, (p + 1) * FC)
            lo, hi = slice(0, DHALF), slice(DHALF, D)
            lhs = (((lo, a), (hi, b), 1), ((hi, a), (hi, b), 1), ((lo, a),), ((hi, b),),
                   ((lo, a), (lo, b), 1), ((hi, a), (lo, a), -1), ((lo, b), (hi, b), -1))
            for n in (1, 3, 5, 0, 2, 4, 6):
                part = _dot_nt(operand(i, wd7, n, o, wdT, *lhs[n]), bs[n])
                if p == 0:
                    acc7[n] = part
                else:
                    acc7[n] += part

        out_cps = []

        def finish(i):
            s0 = i * TM
            for t in range(T // 128):
                sl = slice(t * 128, (t + 1) * 128)
                p1, p2, p3, p4, p5, p6, p7 = [acc7[n, :, sl] for n in range(7)]
                quads = ((0, 0, p1 + p4 - p5 + p7), (0, 1, p3 + p5), (1, 0, p2 + p4), (1, 1, p1 - p2 + p3 + p6))
                for dh, th, v in quads:
                    rows = slice(dh * DHALF, (dh + 1) * DHALF)
                    cols = slice(s0 + th * T + t * 128, s0 + th * T + (t + 1) * 128)
                    outT[rows, cols] = (x1[rows, cols] + gateT[1, rows, :] * v).astype(BF)
            out_cps.append(copy_cols(outT, outT_hbm, s0, TM))

        with sc("p0_x"):
            cp_x0.wait()
            for t in range(TM // 128):
                ybuf[t * 128:(t + 1) * 128, :] = normalize(xT[:, t * 128:(t + 1) * 128].astype(F32)).T
        with sc("p1_m"):
            cp_m0.wait()
            prep_mod0()
            hbuf[0:TM // 2, :] = _pack(modulate(ybuf[...], 0).astype(BF))
        with sc("p2_pq"):
            cp_q.wait()
            prep_wqkv(0)
        with sc("p2_q"):
            cp_k.wait()
            prep_wqkv(1)
            qkv_q(0)
        with sc("p2_kv"):
            cp_v.wait()
            cp_x1.wait()
            prep_wqkv(2)
            qkv_k(0), qkv_v(0)
            ln1(1)
            qkv_q(1), qkv_k(1)
            if pro > 0:
                qkv_v(1, 0, pro)
            attention(0, chain0)
        with sc("p3_wo"):
            cp_wo.wait()
            cp_m1.wait()
            for q_ in waits[0]:
                for cp in cp_f[q_]:
                    cp.wait()
            prep_mod1()
            prep_wo()
            wo_proj(0)
            if pro < TM:
                qkv_v(1, pro, TM)
            ln2(0)
        for i in range(nb_run):
            with sc(f"p4_b{i}"):
                nxt = i + 1 < nb
                pend = None
                for p in range(nP):
                    if nxt and i > 0 and p == qkv_at:
                        ln1(i + 1)
                        qkv_q(i + 1), qkv_k(i + 1), qkv_v(i + 1)
                    if nxt and p == (wo_at if i > 0 else wo_at0):
                        attention(i + 1, chain)
                        wo_proj(i + 1)
                    if i == 0 and p > 0 and p in waits:
                        for q_ in waits[p]:
                            for cp in cp_f[q_]:
                                cp.wait()
                        if p == max(waits):
                            cp_x2.wait()
                    bs = gate_up(i, p)
                    if pend is not None:
                        down(i, p - 1, pend)
                    pend = bs
                down(i, nP - 1, pend)
                if nxt:
                    ln2(i + 1)
                finish(i)
        if nb_run < nb:
            out_cps.append(copy_cols(outT, outT_hbm, nb_run * TM, S - nb_run * TM))
        for cp in out_cps:
            cp.wait()

    n_sems = 10 + 3 * nP + nb
    hbm = pl.BlockSpec(memory_space=pltpu.HBM)

    def fn(A_x, A_wqkv, A_wo, B_x, B_w_gate, B_w_up, B_w_down, c, w_mod):
        del B_x
        outT = pl.pallas_call(
            kernel,
            in_specs=[pl.BlockSpec(memory_space=pltpu.VMEM)] + [hbm] * 7,
            out_specs=hbm,
            out_shape=jax.ShapeDtypeStruct((D, S), BF),
            scratch_shapes=[
                pltpu.VMEM((D, S), BF), pltpu.VMEM((D, 3 * D), BF), pltpu.VMEM((D, D), BF),
                pltpu.VMEM((D, F), BF), pltpu.VMEM((D, F), BF), pltpu.VMEM((D, F), BF),
                pltpu.VMEM((D, 6 * D), BF),
                pltpu.VMEM((NT, 1792, 128), F32), pltpu.VMEM((896, D), I32), pltpu.VMEM((D // 2, D), I32),
                pltpu.VMEM((4, 8, NT * 128), F32), pltpu.VMEM((2, D, 128), F32),
                pltpu.VMEM((KT // 2, F // 2), I32), pltpu.VMEM((KT // 2, F // 2), I32),
                pltpu.VMEM((7, DHALF // 2, F // 2), I32),
                pltpu.VMEM((TM, D), F32),
                pltpu.VMEM((NT, S, 128), F32), pltpu.VMEM((NT, HALO + S, 128), F32),
                pltpu.VMEM((NT, HALO + S, 128), F32),
                pltpu.VMEM((S // 2, D), I32), pltpu.VMEM((S // 2, D), I32),
                pltpu.VMEM((D, S), F32),
                pltpu.VMEM((nb, T // 2, KT), I32),
                pltpu.VMEM((7, DHALF, T), F32), pltpu.VMEM((D, S), BF),
                pltpu.SemaphoreType.DMA((n_sems,)),
            ],
            compiler_params=pltpu.CompilerParams(vmem_limit_bytes=120 * 2**20, flags=flags),
            name=name,
        )(c, A_x[0].T, A_wqkv, A_wo, B_w_gate, B_w_up, B_w_down.T, w_mod)
        return outT.T[None]

    return fn


@jax.jit
def pallas_adaLN_cond__sliding_local_dilated__glu_gated_bilinear__prompt_kernel(
    A_x: jax.Array,
    A_wqkv: jax.Array,
    A_wo: jax.Array,
    B_x: jax.Array,
    B_w_gate: jax.Array,
    B_w_up: jax.Array,
    B_w_down: jax.Array,
    c: jax.Array,
    w_mod: jax.Array,
):
    return make()(A_x, A_wqkv, A_wo, B_x, B_w_gate, B_w_up, B_w_down, c, w_mod)
```

```python
import contextlib
import functools

import jax
import jax.numpy as jnp
from jax import lax
import jax.experimental.pallas as pl
import jax.experimental.pallas.tpu as pltpu

S, D, H, DH, W, DIL, F = 2048, 576, 32, 18, 8, 2, 4608
HALO = 16
NT = 5
DHALF = D // 2
EPS = 1e-5
BF, F32, I32 = jnp.bfloat16, jnp.float32, jnp.int32
NT_DIMS = (((1,), (1,)), ((), ()))


def _tw(j):
    return min(128, D - 128 * j)


def _dot(a, b):
    return jnp.dot(a, b, preferred_element_type=F32)


def _dot_nt(a, b):
    return lax.dot_general(a, b, NT_DIMS, preferred_element_type=F32)


def _pack(v):
    return pltpu.bitcast(v, jnp.int32)


def _unpack(v):
    return pltpu.bitcast(v, BF)


def _colsum(x):
    return jnp.sum(jnp.sum(x.reshape(D // 32, 32, 128), axis=0), axis=0, keepdims=True)


KS = (256, 256, 384, 384, 192, 384, 256)
KO = (0, 256, 512, 896, 1280, 1536, 1920)
KT = 2176
S1A, S2A, S1B, R1, S2B, R2, R3 = (
    slice(0, 128), slice(128, 256), slice(256, 320), slice(320, 384), slice(384, 448), slice(448, 512), slice(512, 576))
RIGHT = (
    ((S1A, 0, 1, S2A, 1), (S1B, 0, 1, S2B, 1), (R1, 0)),
    ((S1A, 0), (S1B, 0), (R2, 0)),
    ((S1A, 1, -1, S2A, 1), (S1B, 1, -1, S2B, 1), (R1, 1), (R3, 1), (R2, 1)),
    ((S2A, 0, -1, S1A, 0), (S2B, 0, -1, S1B, 0), (R2, 0), (R3, 0), (R1, 0)),
    ((S2A, 1), (S2B, 1)),
    ((S1A, 0, 1, S1A, 1), (S1B, 0, 1, S1B, 1), (R1, 0, 1, R1, 1), (R3, 1), (R2, 0, 1, R2, 1)),
    ((S2A, 0, 1, S2A, 1), (S2B, 0, 1, S2B, 1), (R3, 0)),
)


def _left_operands(p, q, lo):
    d = [y - x for x, y in zip(p, q)]
    w = lambda a, b: jnp.where(lo, a, b)
    return (
        (p[0] + q[1], w(p[2] + q[3], p[2] - q[2])),
        (q[0] + q[1], w(q[2] + q[3], d[3])),
        (p[0], p[2], w(p[4], p[3])),
        (q[1], w(q[3], p[3]), w(q[4], q[2])),
        (p[0] + p[1], p[2] + p[3]),
        (d[0], d[2], w(d[4], d[3])),
        (d[1], w(d[3], d[4])),
    )


def _right_operands(a, b, lo):
    w = lambda x, y: jnp.where(lo, x, y)
    return (
        lambda: (a(0) + b(1), w(a(2) + b(3), a(2))),
        lambda: (a(0), w(a(2), a(3))),
        lambda: (b(0) - b(1), w(b(2) - b(3), b(2)), w(b(4), b(3))),
        lambda: (a(1) - a(0), w(a(3) - a(2), a(3)), w(a(4), a(2))),
        lambda: (b(1), b(3)),
        lambda: (a(0) + b(0), a(2) + b(2), w(b(4), a(3) + b(3))),
        lambda: (a(1) + b(1), w(a(3) + b(3), a(4))),
    )


def _quadrants(m):
    return m[0] - m[4] + m[3] - m[6], m[4] + m[2], m[1] + m[3], m[0] - m[1] + m[2] + m[5]


ORDER = (1, 4, 0, 2, 3, 5, 6)
_slabs = lambda part, lo, hi: [(part, d) for d in range(lo, hi)]
QKV_GROUPS = (
    (_slabs(0, 0, 8), _slabs(0, 8, 16)),
    (_slabs(1, 0, 8), _slabs(1, 8, 16)),
    (_slabs(2, 0, 8) + _slabs(0, 16, 18) + _slabs(1, 16, 18), _slabs(2, 8, 16) + _slabs(2, 16, 18) * 2),
)


def make(TM=512, FC=384, R=8, chain=1, chain0=3, waits=None, nb_run=None, flags=None, name="k6",
         scopes=False, wo_at=None, qkv_at=1, pro=3, merge_q=False, prio=0, prio2=0, wo_at0=5):
    nb = S // TM
    T = TM // 2
    nP = F // (2 * FC)
    nb_run = nb if nb_run is None else nb_run
    wo_at = (2 * nP) // 3 if wo_at is None else wo_at
    waits = {0: [0], 1: [1, 2], 3: [3, 4, 5]} if waits is None else waits
    assert max(waits) > 0 and sorted(sum(waits.values(), [])) == list(range(nP))

    def kernel(c_ref, xT_hbm, wqkv_hbm, wo_hbm, wg_hbm, wu_hbm, wdT_hbm, wmod_hbm, outT_hbm,
               xT, wqkv, wo, wg, wu, wdT, wmod, tmpT, tmpW, woT, wq17, wo17, modR, gateT, wg17, wu17, wd7,
               ybuf, qbuf, kbuf, vbuf, h17, o17, x1, a17, acc7, outT, sems):
        sc = jax.named_scope if scopes else (lambda n: contextlib.nullcontext())
        sem_i = [0]

        def copy_cols(src, dst, c0, n, priority=0):
            cp = pltpu.make_async_copy(src.at[:, pl.ds(c0, n)], dst.at[:, pl.ds(c0, n)], sems.at[sem_i[0]])
            sem_i[0] += 1
            cp.start(priority=priority)
            return cp

        cp_x0 = copy_cols(xT_hbm, xT, 0, TM)
        cp_m0 = copy_cols(wmod_hbm, wmod, 0, 2 * D)
        cp_q = copy_cols(wqkv_hbm, wqkv, 0, 640)
        cp_k = copy_cols(wqkv_hbm, wqkv, 640, 512)
        cp_v = copy_cols(wqkv_hbm, wqkv, 1152, D)
        cp_x1 = copy_cols(xT_hbm, xT, TM, TM)
        cp_wo = copy_cols(wo_hbm, wo, 0, D, prio2)
        cp_m1 = copy_cols(wmod_hbm, wmod, 2 * D, 4 * D, prio2)
        cp_f = []
        for p in range(nP):
            cp_f.append([copy_cols(s, d, 2 * p * FC, 2 * FC, prio) for s, d in ((wg_hbm, wg), (wu_hbm, wu), (wdT_hbm, wdT))])
            if p == nP - 1:
                cp_x2 = copy_cols(xT_hbm, xT, 2 * TM, S - 2 * TM, prio)

        cbits = pltpu.bitcast(jnp.broadcast_to(c_ref[:, 0:128].astype(F32), (8, 128)), jnp.int32)
        keep = ((cbits * cbits) & 2) == 0

        def after(x, prev):
            k = jnp.broadcast_to(keep[0:1], x.shape[-2:])
            return jnp.where(k, x, prev)

        lane = lax.broadcasted_iota(jnp.int32, (1, 128), 1)
        lo = lane < 64

        def feature_tiles(y):
            return [y[j * 128:(j + 1) * 128] for j in range(4)] + [jnp.concatenate([y[512:D], y[512:D]], axis=0)]

        def store_left(dst, rows, p, q):
            for n, tiles in enumerate(_left_operands(p, q, lo)):
                for j, v in enumerate(tiles):
                    c0 = KO[n] + j * 128
                    dst[rows, c0:c0 + 128] = _pack(v.astype(BF))

        def prep_wqkv(part):
            for cb in (range(0, 5), range(5, 9), range(9, 14))[part]:
                cw = min(128, 3 * D - cb * 128)
                for j, t in enumerate(feature_tiles(wqkv[:, cb * 128:cb * 128 + cw].astype(F32))):
                    tmpT[j, cb * 128:cb * 128 + cw, :] = t.T

        def prep_wo():
            for j in range(NT):
                tmpW[j, :, 0:_tw(j)] = wo[:, j * 128:j * 128 + _tw(j)].astype(F32)
            for j in range(NT):
                p = jnp.concatenate([tmpW[j, pl.ds(d, H, stride=DH), :] for d in range(DH)], axis=0)
                for n, t in enumerate(feature_tiles(p[:, 0:_tw(j)])):
                    woT[n, j * 128:j * 128 + _tw(j), :] = t.T
            store_left(wo17, slice(None), [woT[n, 0:DHALF, :] for n in range(NT)], [woT[n, DHALF:D, :] for n in range(NT)])

        def modulation(c0, n):
            cf = c_ref[...].astype(F32)
            s = (cf * jax.nn.sigmoid(cf)).astype(BF)
            return _dot(jnp.broadcast_to(s, (16, D)), wmod[:, c0:c0 + n])[0:8]

        def to_column(row, n):
            for j in range(NT):
                r = row[0:1, j * 128:j * 128 + _tw(j)]
                gateT[n, j * 128:j * 128 + _tw(j), :] = jnp.broadcast_to(r, (128, _tw(j))).T

        def widen(row):
            return jnp.concatenate([row, row[:, 512:D]], axis=1)

        def prep_mod0():
            m = modulation(0, 2 * D)
            modR[0] = widen(m[:, 0:D])
            modR[1] = widen(1.0 + m[:, D:2 * D])

        def prep_mod1():
            m = modulation(2 * D, 4 * D)
            modR[2] = widen(m[:, D:2 * D])
            modR[3] = widen(1.0 + m[:, 2 * D:3 * D])
            to_column(m[:, 0:D], 0)
            to_column(m[:, 3 * D:4 * D], 1)

        def normalize(xf):
            mean = _colsum(xf) * (1.0 / D)
            xc = xf - mean
            var = _colsum(xc * xc) * (1.0 / D)
            return xc * lax.rsqrt(var + EPS)

        def modulate(tiles, n):
            return [t * modR[2 * n + 1, 0:1, j * 128:(j + 1) * 128] + modR[2 * n, 0:1, j * 128:(j + 1) * 128]
                    for j, t in enumerate(tiles)]

        def norm_tiles(src, r):
            return [t.T for t in feature_tiles(normalize(src[:, r:r + 128].astype(F32)))]

        def ln1(i):
            for t in range(T // 128):
                p, q = [modulate(norm_tiles(xT, i * TM + half * T + t * 128), 0) for half in range(2)]
                store_left(h17.at[i % 2], slice(t * 64, (t + 1) * 64), p, q)

        def qkv(i, g):
            s0 = i * TM
            sa, sb = QKV_GROUPS[g]
            rows = slice(g * 128, g * 128 + len(sa) * H // 2)
            if i == 0:
                gather = lambda slabs: lambda j: jnp.concatenate(
                    [tmpT[j, pl.ds(part * D + d, H, stride=DH), :] for part, d in slabs], axis=0)
                make_rhs = _right_operands(gather(sa), gather(sb), lo)
            m = {}
            for n in ORDER:
                cols = slice(KO[n], KO[n] + KS[n])
                if i == 0:
                    rhs = jnp.concatenate(make_rhs[n](), axis=1).astype(BF)[:, 0:KS[n]]
                    wq17[rows, cols] = _pack(rhs)
                else:
                    rhs = _unpack(wq17[rows, cols])
                m[n] = _dot_nt(_unpack(h17[i % 2, :, cols]), rhs)
            c11, c12, c21, c22 = _quadrants(m)
            for half, (ca, cb) in enumerate(((c11, c12), (c21, c22))):
                r = s0 + half * T
                tile = lambda j: (ca if j < 2 else cb)[:, (j % 2) * 128:(j % 2 + 1) * 128]
                for j in range(4):
                    if g == 0:
                        qbuf[j, r:r + T, :] = tile(j) * DH ** -0.5
                    else:
                        (kbuf, vbuf)[g - 1][j, HALO + r:HALO + r + T, :] = tile(j)
                if g == 2:
                    xt = ca[:, 256:384]
                    qbuf[4, r:r + T, :] = jnp.where(lo, xt * DH ** -0.5, 0.0)
                    kbuf[4, HALO + r:HALO + r + T, :] = jnp.where(lo, pltpu.roll(xt, 64, 1), 0.0)
                    vbuf[4, HALO + r:HALO + r + T, :] = cb[:, 256:384]
            if i == 0 and g == 2:
                for j in range(NT):
                    kbuf[j, 0:HALO, :] = jnp.broadcast_to(kbuf[j, HALO:HALO + 1, :], (HALO, 128))
                    vbuf[j, 0:HALO, :] = jnp.broadcast_to(vbuf[j, HALO:HALO + 1, :], (HALO, 128))

        def attend(r0, prev):
            q = qbuf[:, r0:r0 + R, :]
            if prev is not None:
                q = after(q, prev)
            ls = []
            for w in range(W):
                a = HALO + r0 - DIL * w
                p = jnp.sum(q * kbuf[:, a:a + R, :], axis=0)
                p = p + pltpu.roll(p, 64, 1)
                p = p + pltpu.roll(p, 32, 1)
                if r0 < DIL * w:
                    row = lax.broadcasted_iota(jnp.int32, (R, 128), 0) + r0
                    p = jnp.where(row >= DIL * w, p, -1e9)
                ls.append(p)
            m = functools.reduce(jnp.maximum, ls)
            es = [jnp.exp(l - m) for l in ls]
            den = functools.reduce(jnp.add, es)
            acc = None
            for w in range(W):
                a = HALO + r0 - DIL * w
                t = es[w][None] * vbuf[:, a:a + R, :]
                acc = t if acc is None else acc + t
            return acc * (1.0 / den)[None]

        def attention(i, chained):
            done = []
            for r in range(0, T, 16):
                o = []
                for half in range(2):
                    for r0 in range(r, r + 16, R):
                        done.append(attend(i * TM + half * T + r0, done[-chained] if 0 < chained <= len(done) else None))
                    o.append(jnp.concatenate(done[-(16 // R):], axis=1))
                for n, tiles in enumerate(_right_operands(lambda j: o[0][j], lambda j: o[1][j], lo)):
                    for j, v in enumerate(tiles()):
                        c0 = KO[n] + j * 128
                        o17[r // 2:r // 2 + 8, c0:c0 + 128] = _pack(v.astype(BF))

        def wo_proj(i):
            s0 = i * TM
            m = {}
            for n in ORDER:
                cols = slice(KO[n], KO[n] + KS[n])
                m[n] = _dot_nt(_unpack(wo17[:, cols]), _unpack(o17[:, cols]))
            for n, v in enumerate(_quadrants(m)):
                rows = slice((n // 2) * DHALF, (n // 2 + 1) * DHALF)
                for t in range(T // 128):
                    c0 = (n % 2) * T + t * 128
                    x1[i % 2, rows, c0:c0 + 128] = (xT[rows, s0 + c0:s0 + c0 + 128].astype(F32)
                                                    + gateT[0, rows, :] * v[:, t * 128:(t + 1) * 128])

        def ln2(i):
            for t in range(T // 128):
                p, q = [modulate(norm_tiles(x1.at[i % 2], half * T + t * 128), 1) for half in range(2)]
                store_left(a17.at[i % 2], slice(t * 64, (t + 1) * 64), p, q)

        def combine(x, sign=None, y=None):
            if sign is None:
                return x
            x, y = x.astype(F32), y.astype(F32)
            return (x + y if sign > 0 else x - y).astype(BF)

        def operand(i, dst, n, o, w, xi, yi=None, sign=None):
            if i > 0:
                return _unpack(dst[n, :, o])
            v = combine(w[xi], sign, None if yi is None else w[yi])
            dst[n, :, o] = _pack(v)
            return v

        def gate_up(i, p):
            cols = (slice(2 * p * FC, (2 * p + 1) * FC), slice((2 * p + 1) * FC, (2 * p + 2) * FC))
            o = slice(p * FC, (p + 1) * FC)
            cs = []
            for w, w17 in ((wg, wg17), (wu, wu17)):
                m = {}
                for n in ORDER:
                    rows = slice(KO[n] // 2, (KO[n] + KS[n]) // 2)
                    if i > 0:
                        rhs = _unpack(w17[rows, o])
                    else:
                        rhs = jnp.concatenate(
                            [combine(w[e[0], cols[e[1]]], *((e[2], w[e[3], cols[e[4]]]) if len(e) > 2 else ()))
                             for e in RIGHT[n]], axis=0)
                        w17[rows, o] = _pack(rhs)
                    m[n] = _dot(_unpack(a17[i % 2, :, KO[n]:KO[n] + KS[n]]), rhs)
                cs.append(_quadrants(m))
            b11, b21, b12, b22 = [g * u for g, u in zip(*cs)]
            return [v.astype(BF) for v in (b11 + b22, b11, b12 - b22, b21 - b11, b22, b11 + b12, b21 + b22)]

        def down(i, p, bs):
            a, b, o = slice(2 * p * FC, (2 * p + 1) * FC), slice((2 * p + 1) * FC, (2 * p + 2) * FC), slice(p * FC, (p + 1) * FC)
            lo, hi = slice(0, DHALF), slice(DHALF, D)
            lhs = (((lo, a), (hi, b), 1), ((hi, a), (hi, b), 1), ((lo, a),), ((hi, b),),
                   ((lo, a), (lo, b), 1), ((hi, a), (lo, a), -1), ((lo, b), (hi, b), -1))
            for n in (1, 3, 5, 0, 2, 4, 6):
                part = _dot_nt(operand(i, wd7, n, o, wdT, *lhs[n]), bs[n])
                if p == 0:
                    acc7[n] = part
                else:
                    acc7[n] += part

        out_cps = []

        def finish(i):
            s0 = i * TM
            for t in range(T // 128):
                sl = slice(t * 128, (t + 1) * 128)
                p1, p2, p3, p4, p5, p6, p7 = [acc7[n, :, sl] for n in range(7)]
                quads = ((0, 0, p1 + p4 - p5 + p7), (0, 1, p3 + p5), (1, 0, p2 + p4), (1, 1, p1 - p2 + p3 + p6))
                for dh, th, v in quads:
                    rows = slice(dh * DHALF, (dh + 1) * DHALF)
                    c0 = th * T + t * 128
                    outT[rows, s0 + c0:s0 + c0 + 128] = (x1[i % 2, rows, c0:c0 + 128] + gateT[1, rows, :] * v).astype(BF)
            out_cps.append(copy_cols(outT, outT_hbm, s0, TM))

        with sc("p0_x"):
            cp_x0.wait()
            for t in range(TM // 128):
                for j, v in enumerate(norm_tiles(xT, t * 128)):
                    ybuf[j, t * 128:(t + 1) * 128, :] = v
        with sc("p1_m"):
            cp_m0.wait()
            prep_mod0()
            for t in range(T // 128):
                p, q = [modulate([ybuf[j, half * T + t * 128:half * T + (t + 1) * 128, :] for j in range(NT)], 0) for half in range(2)]
                store_left(h17.at[0], slice(t * 64, (t + 1) * 64), p, q)
        with sc("p2_pq"):
            cp_q.wait()
            prep_wqkv(0)
            if merge_q:
                cp_k.wait()
                prep_wqkv(1)
                qkv(0, 0)
        with sc("p2_q"):
            if not merge_q:
                cp_k.wait()
                prep_wqkv(1)
                qkv(0, 0)
        with sc("p2_kv"):
            cp_v.wait()
            cp_x1.wait()
            prep_wqkv(2)
            qkv(0, 1), qkv(0, 2)
            ln1(1)
            for g in range(pro):
                qkv(1, g)
            attention(0, chain0)
        with sc("p3_wo"):
            cp_wo.wait()
            cp_m1.wait()
            for q_ in waits[0]:
                for cp in cp_f[q_]:
                    cp.wait()
            prep_mod1()
            prep_wo()
            wo_proj(0)
            for g in range(pro, 3):
                qkv(1, g)
            ln2(0)
        for i in range(nb_run):
            with sc(f"p4_b{i}"):
                nxt = i + 1 < nb
                pend = None
                for p in range(nP):
                    if nxt and i > 0 and p == qkv_at:
                        ln1(i + 1)
                        qkv(i + 1, 0), qkv(i + 1, 1), qkv(i + 1, 2)
                    if nxt and p == (wo_at if i > 0 else wo_at0):
                        attention(i + 1, chain)
                        wo_proj(i + 1)
                    if i == 0 and p > 0 and p in waits:
                        for q_ in waits[p]:
                            for cp in cp_f[q_]:
                                cp.wait()
                        if p == max(waits):
                            cp_x2.wait()
                    bs = gate_up(i, p)
                    if pend is not None:
                        down(i, p - 1, pend)
                    pend = bs
                down(i, nP - 1, pend)
                if nxt:
                    ln2(i + 1)
                finish(i)
        if nb_run < nb:
            out_cps.append(copy_cols(outT, outT_hbm, nb_run * TM, S - nb_run * TM))
        for cp in out_cps:
            cp.wait()

    n_sems = 10 + 3 * nP + nb
    hbm = pl.BlockSpec(memory_space=pltpu.HBM)

    def fn(A_x, A_wqkv, A_wo, B_x, B_w_gate, B_w_up, B_w_down, c, w_mod):
        del B_x
        outT = pl.pallas_call(
            kernel,
            in_specs=[pl.BlockSpec(memory_space=pltpu.VMEM)] + [hbm] * 7,
            out_specs=hbm,
            out_shape=jax.ShapeDtypeStruct((D, S), BF),
            scratch_shapes=[
                pltpu.VMEM((D, S), BF), pltpu.VMEM((D, 3 * D), BF), pltpu.VMEM((D, D), BF),
                pltpu.VMEM((D, F), BF), pltpu.VMEM((D, F), BF), pltpu.VMEM((D, F), BF),
                pltpu.VMEM((D, 6 * D), BF),
                pltpu.VMEM((NT, 1792, 128), F32), pltpu.VMEM((NT, D, 128), F32), pltpu.VMEM((NT, D, 128), F32),
                pltpu.VMEM((448, KT), I32), pltpu.VMEM((DHALF // 2, KT), I32),
                pltpu.VMEM((4, 8, NT * 128), F32), pltpu.VMEM((2, D, 128), F32),
                pltpu.VMEM((KT // 2, F // 2), I32), pltpu.VMEM((KT // 2, F // 2), I32),
                pltpu.VMEM((7, DHALF // 2, F // 2), I32),
                pltpu.VMEM((NT, TM, 128), F32),
                pltpu.VMEM((NT, S, 128), F32), pltpu.VMEM((NT, HALO + S, 128), F32),
                pltpu.VMEM((NT, HALO + S, 128), F32),
                pltpu.VMEM((2, T // 2, KT), I32), pltpu.VMEM((T // 2, KT), I32),
                pltpu.VMEM((2, D, TM), F32),
                pltpu.VMEM((2, T // 2, KT), I32),
                pltpu.VMEM((7, DHALF, T), F32), pltpu.VMEM((D, S), BF),
                pltpu.SemaphoreType.DMA((n_sems,)),
            ],
            compiler_params=pltpu.CompilerParams(vmem_limit_bytes=120 * 2**20, flags=flags),
            name=name,
        )(c, A_x[0].T, A_wqkv, A_wo, B_w_gate, B_w_up, B_w_down.T, w_mod)
        return outT.T[None]

    return fn


@jax.jit
def pallas_adaLN_cond__sliding_local_dilated__glu_gated_bilinear__prompt_kernel(
    A_x: jax.Array,
    A_wqkv: jax.Array,
    A_wo: jax.Array,
    B_x: jax.Array,
    B_w_gate: jax.Array,
    B_w_up: jax.Array,
    B_w_down: jax.Array,
    c: jax.Array,
    w_mod: jax.Array,
):
    return make(chain0=4)(A_x, A_wqkv, A_wo, B_x, B_w_gate, B_w_up, B_w_down, c, w_mod)
```

```python
import contextlib
import functools

import jax
import jax.numpy as jnp
from jax import lax
import jax.experimental.pallas as pl
import jax.experimental.pallas.tpu as pltpu

S, D, H, DH, W, DIL, F = 2048, 576, 32, 18, 8, 2, 4608
HALO = 16
NT = 5
DHALF = D // 2
DQ = D // 4
EPS = 1e-5
LOG2E = 1.4426950408889634
QSCALE = DH ** -0.5 * LOG2E
BF, F32, I32 = jnp.bfloat16, jnp.float32, jnp.int32
NT_DIMS = (((1,), (1,)), ((), ()))


def _tw(j):
    return min(128, D - 128 * j)


def _dot(a, b):
    return jnp.dot(a, b, preferred_element_type=F32)


def _dot_nt(a, b):
    return lax.dot_general(a, b, NT_DIMS, preferred_element_type=F32)


def _pack(v):
    return pltpu.bitcast(v, jnp.int32)


def _unpack(v):
    return pltpu.bitcast(v, BF)


def _colsum(x):
    return jnp.sum(jnp.sum(x.reshape(D // 32, 32, 128), axis=0), axis=0, keepdims=True)


KS = (256, 256, 384, 384, 192, 384, 256)
KO = (0, 256, 512, 896, 1280, 1536, 1920)
KT = 2176
S1A, S2A, S1B, R1, S2B, R2, R3 = (
    slice(0, 128), slice(128, 256), slice(256, 320), slice(320, 384), slice(384, 448), slice(448, 512), slice(512, 576))
RIGHT = (
    ((S1A, 0, 1, S2A, 1), (S1B, 0, 1, S2B, 1), (R1, 0)),
    ((S1A, 0), (S1B, 0), (R2, 0)),
    ((S1A, 1, -1, S2A, 1), (S1B, 1, -1, S2B, 1), (R1, 1), (R3, 1), (R2, 1)),
    ((S2A, 0, -1, S1A, 0), (S2B, 0, -1, S1B, 0), (R2, 0), (R3, 0), (R1, 0)),
    ((S2A, 1), (S2B, 1)),
    ((S1A, 0, 1, S1A, 1), (S1B, 0, 1, S1B, 1), (R1, 0, 1, R1, 1), (R3, 1), (R2, 0, 1, R2, 1)),
    ((S2A, 0, 1, S2A, 1), (S2B, 0, 1, S2B, 1), (R3, 0)),
)


def _left_operands(p, q, lo):
    d = [y - x for x, y in zip(p, q)]
    w = lambda a, b: jnp.where(lo, a, b)
    return (
        (p[0] + q[1], w(p[2] + q[3], p[2] - q[2])),
        (q[0] + q[1], w(q[2] + q[3], d[3])),
        (p[0], p[2], w(p[4], p[3])),
        (q[1], w(q[3], p[3]), w(q[4], q[2])),
        (p[0] + p[1], p[2] + p[3]),
        (d[0], d[2], w(d[4], d[3])),
        (d[1], w(d[3], d[4])),
    )


def _right_operands(a, b, lo):
    w = lambda x, y: jnp.where(lo, x, y)
    return (
        lambda: (a(0) + b(1), w(a(2) + b(3), a(2))),
        lambda: (a(0), w(a(2), a(3))),
        lambda: (b(0) - b(1), w(b(2) - b(3), b(2)), w(b(4), b(3))),
        lambda: (a(1) - a(0), w(a(3) - a(2), a(3)), w(a(4), a(2))),
        lambda: (b(1), b(3)),
        lambda: (a(0) + b(0), a(2) + b(2), w(b(4), a(3) + b(3))),
        lambda: (a(1) + b(1), w(a(3) + b(3), a(4))),
    )


def _quadrants(m):
    return m[0] - m[4] + m[3] - m[6], m[4] + m[2], m[1] + m[3], m[0] - m[1] + m[2] + m[5]


def _lefts(a11, a12, a21, a22):
    return a11 + a22, a21 + a22, a11, a22, a11 + a12, a21 - a11, a22 - a12


def _rights(b11, b12, b21, b22):
    return b11 + b22, b11, b12 - b22, b21 - b11, b22, b11 + b12, b21 + b22


def _two_levels(combos, blocks):
    outer = [combos(*(blocks[e1][e2] for e1 in range(4))) for e2 in range(4)]
    return [v for n in range(7) for v in combos(*(outer[e2][n] for e2 in range(4)))]


ORDER = (1, 4, 0, 2, 3, 5, 6)
_slabs = lambda part, lo, hi: [(part, d) for d in range(lo, hi)]
QKV_GROUPS = (
    (_slabs(0, 0, 8), _slabs(0, 8, 16)),
    (_slabs(1, 0, 8), _slabs(1, 8, 16)),
    (_slabs(2, 0, 8) + _slabs(0, 16, 18) + _slabs(1, 16, 18), _slabs(2, 8, 16) + _slabs(2, 16, 18) * 2),
)


DMA_ORDER = "m0 x0 q k v x1 wo m1 f0 f1 f2 f3 f4 f5 x2 x3"


def make(TM=512, FC=384, R=8, sched=None, dma=DMA_ORDER, flags=None, name="k11"):
    nb = S // TM
    T = TM // 2
    nP = F // (2 * FC)
    if isinstance(sched, str):
        sched = [t.strip() for t in sched.split(";") if t.strip()]
    dma = dma.split()

    def kernel(c_ref, xT_hbm, wqkv_hbm, wo_hbm, wg_hbm, wu_hbm, wdT_hbm, wmod_hbm, outT_hbm,
               xT, wqkv, wo, wg, wu, wdT, wmod, tmpT, tmpW, woT, wq17, wo17, modR, gateT, wg17, wu17, wd49,
               qbuf, kbuf, vbuf, h17, o17, x1, a17, h49, acc7, sems):
        sem_i = [0]

        def copy_cols(src, dst, c0, n):
            cp = pltpu.make_async_copy(src.at[:, pl.ds(c0, n)], dst.at[:, pl.ds(c0, n)], sems.at[sem_i[0]])
            sem_i[0] += 1
            cp.start()
            return [cp]

        pieces = {"m0": [(wmod_hbm, wmod, 0, 2 * D)], "m1": [(wmod_hbm, wmod, 2 * D, 4 * D)],
                  "q": [(wqkv_hbm, wqkv, 0, 640)], "k": [(wqkv_hbm, wqkv, 640, 512)], "v": [(wqkv_hbm, wqkv, 1152, D)],
                  "wo": [(wo_hbm, wo, 0, D)]}
        for i in range(nb):
            pieces[f"x{i}"] = [(xT_hbm, xT, i * TM, TM)]
        for p in range(nP):
            pieces[f"f{p}"] = [(a, b, 2 * p * FC, 2 * FC) for a, b in ((wg_hbm, wg), (wu_hbm, wu), (wdT_hbm, wdT))]
        assert sorted(dma) == sorted(pieces)
        pending = {n: sum((copy_cols(*a) for a in pieces[n]), []) for n in dma}

        cbits = pltpu.bitcast(jnp.broadcast_to(c_ref[:, 0:128].astype(F32), (8, 128)), jnp.int32)
        keep = ((cbits * cbits) & 2) == 0

        def after(x, prev):
            k = jnp.broadcast_to(keep[0:1], x.shape[-2:])
            return jnp.where(k, x, prev)

        lane = lax.broadcasted_iota(jnp.int32, (1, 128), 1)
        lo = lane < 64

        def feature_tiles(y):
            return [y[j * 128:(j + 1) * 128] for j in range(4)] + [jnp.concatenate([y[512:D], y[512:D]], axis=0)]

        def store_left(dst, rows, p, q):
            for n, tiles in enumerate(_left_operands(p, q, lo)):
                for j, v in enumerate(tiles):
                    c0 = KO[n] + j * 128
                    dst[rows, c0:c0 + 128] = _pack(v.astype(BF))

        def prep_wqkv(part):
            for cb in (range(0, 5), range(5, 9), range(9, 14))[part]:
                cw = min(128, 3 * D - cb * 128)
                for j, t in enumerate(feature_tiles(wqkv[:, cb * 128:cb * 128 + cw].astype(F32))):
                    tmpT[j, cb * 128:cb * 128 + cw, :] = t.T

        def prep_wo():
            for j in range(NT):
                tmpW[j, :, 0:_tw(j)] = wo[:, j * 128:j * 128 + _tw(j)].astype(F32)
            for j in range(NT):
                p = jnp.concatenate([tmpW[j, pl.ds(d, H, stride=DH), :] for d in range(DH)], axis=0)
                for n, t in enumerate(feature_tiles(p[:, 0:_tw(j)])):
                    woT[n, j * 128:j * 128 + _tw(j), :] = t.T
            store_left(wo17, slice(None), [woT[n, 0:DHALF, :] for n in range(NT)], [woT[n, DHALF:D, :] for n in range(NT)])

        def modulation(c0, n):
            cf = c_ref[...].astype(F32)
            s = (cf * jax.nn.sigmoid(cf)).astype(BF)
            return _dot(jnp.broadcast_to(s, (16, D)), wmod[:, c0:c0 + n])[0:8]

        def to_column(row, n):
            for j in range(NT):
                r = row[0:1, j * 128:j * 128 + _tw(j)]
                gateT[n, j * 128:j * 128 + _tw(j), :] = jnp.broadcast_to(r, (128, _tw(j))).T

        def widen(row):
            return jnp.concatenate([row, row[:, 512:D]], axis=1)

        def prep_mod0():
            m = modulation(0, 2 * D)
            modR[0] = widen(m[:, 0:D])
            modR[1] = widen(1.0 + m[:, D:2 * D])

        def prep_mod1():
            to_column(modulation(2 * D, 640)[:, 0:D], 0)

        def prep_mod2():
            m = modulation(3 * D - 64, 3 * D + 64)
            modR[2] = widen(m[:, 64:64 + D])
            modR[3] = widen(1.0 + m[:, 64 + D:64 + 2 * D])
            to_column(m[:, 64 + 2 * D:64 + 3 * D], 1)

        def normalize(xf):
            mean = _colsum(xf) * (1.0 / D)
            xc = xf - mean
            var = _colsum(xc * xc) * (1.0 / D)
            return xc * lax.rsqrt(var + EPS)

        def modulate(t, j, n):
            return t * modR[2 * n + 1, 0:1, j * 128:(j + 1) * 128] + modR[2 * n, 0:1, j * 128:(j + 1) * 128]

        def layer_norm(dst, load, n, spread):
            prev = None
            for t in range(T // 128):
                halves = []
                for half in range(2):
                    xf = load(half * T + t * 128)
                    if prev is not None:
                        xf = jnp.concatenate([after(xf[0:128], prev), xf[128:D]], axis=0)
                    tiles = []
                    for j, y in enumerate(feature_tiles(normalize(xf))):
                        if spread and j > 0:
                            y = after(y, prev)
                        tiles.append(modulate(y.T, j, n))
                        prev = tiles[-1] if spread else None
                    halves.append(tiles)
                store_left(dst, slice(t * 64, (t + 1) * 64), *halves)

        def ln1(i, spread):
            layer_norm(h17.at[i % 2], lambda r: xT[:, i * TM + r:i * TM + r + 128].astype(F32), 0, spread)

        def ln2(i, spread):
            layer_norm(a17.at[i % 2], lambda r: x1[i % 2, :, r:r + 128], 1, spread)

        def qkv(i, g):
            s0 = i * TM
            sa, sb = QKV_GROUPS[g]
            rows = slice(g * 128, g * 128 + len(sa) * H // 2)
            if i == 0:
                gather = lambda slabs: lambda j: jnp.concatenate(
                    [tmpT[j, pl.ds(part * D + d, H, stride=DH), :] for part, d in slabs], axis=0)
                make_rhs = _right_operands(gather(sa), gather(sb), lo)
            m = {}
            for n in ORDER:
                cols = slice(KO[n], KO[n] + KS[n])
                if i == 0:
                    rhs = jnp.concatenate(make_rhs[n](), axis=1).astype(BF)[:, 0:KS[n]]
                    wq17[rows, cols] = _pack(rhs)
                else:
                    rhs = _unpack(wq17[rows, cols])
                m[n] = _dot_nt(_unpack(h17[i % 2, :, cols]), rhs)
            c11, c12, c21, c22 = _quadrants(m)
            for half, (ca, cb) in enumerate(((c11, c12), (c21, c22))):
                r = s0 + half * T
                tile = lambda j: (ca if j < 2 else cb)[:, (j % 2) * 128:(j % 2 + 1) * 128]
                for j in range(4):
                    if g == 0:
                        qbuf[j, r:r + T, :] = tile(j) * QSCALE
                    else:
                        (kbuf, vbuf)[g - 1][j, HALO + r:HALO + r + T, :] = tile(j)
                if g == 2:
                    xt = ca[:, 256:384]
                    qbuf[4, r:r + T, :] = jnp.where(lo, xt * QSCALE, 0.0)
                    kbuf[4, HALO + r:HALO + r + T, :] = jnp.where(lo, pltpu.roll(xt, 64, 1), 0.0)
                    vbuf[4, HALO + r:HALO + r + T, :] = cb[:, 256:384]
            if i == 0 and g == 2:
                for j in range(NT):
                    kbuf[j, 0:HALO, :] = jnp.broadcast_to(kbuf[j, HALO:HALO + 1, :], (HALO, 128))
                    vbuf[j, 0:HALO, :] = jnp.broadcast_to(vbuf[j, HALO:HALO + 1, :], (HALO, 128))

        def attend(r0, prev):
            q = qbuf[:, r0:r0 + R, :]
            if prev is not None:
                q = after(q, prev)
            ls = []
            for w in range(W):
                a = HALO + r0 - DIL * w
                p = jnp.sum(q * kbuf[:, a:a + R, :], axis=0)
                p = p + pltpu.roll(p, 64, 1)
                p = p + pltpu.roll(p, 32, 1)
                if r0 < DIL * w:
                    row = lax.broadcasted_iota(jnp.int32, (R, 128), 0) + r0
                    p = jnp.where(row >= DIL * w, p, -1e9 * LOG2E)
                ls.append(p)
            m = functools.reduce(jnp.maximum, ls)
            es = [jnp.exp2(l - m) for l in ls]
            den = functools.reduce(jnp.add, es)
            acc = None
            for w in range(W):
                a = HALO + r0 - DIL * w
                t = es[w][None] * vbuf[:, a:a + R, :]
                acc = t if acc is None else acc + t
            inv = pl.reciprocal(den, approx=True)
            inv = inv * (2.0 - den * inv)
            inv = inv * (2.0 - den * inv)
            return acc * inv[None]

        def attention(i, chained):
            done = []
            for r in range(0, T, 16):
                o = []
                for half in range(2):
                    for r0 in range(r, r + 16, R):
                        done.append(attend(i * TM + half * T + r0, done[-chained] if 0 < chained <= len(done) else None))
                    o.append(jnp.concatenate(done[-(16 // R):], axis=1))
                for n, tiles in enumerate(_right_operands(lambda j: o[0][j], lambda j: o[1][j], lo)):
                    for j, v in enumerate(tiles()):
                        c0 = KO[n] + j * 128
                        o17[r // 2:r // 2 + 8, c0:c0 + 128] = _pack(v.astype(BF))

        def wo_proj(i):
            s0 = i * TM
            m = {}
            for n in ORDER:
                cols = slice(KO[n], KO[n] + KS[n])
                m[n] = _dot_nt(_unpack(wo17[:, cols]), _unpack(o17[:, cols]))
            for n, v in enumerate(_quadrants(m)):
                rows = slice((n // 2) * DHALF, (n // 2 + 1) * DHALF)
                for t in range(T // 128):
                    c0 = (n % 2) * T + t * 128
                    x1[i % 2, rows, c0:c0 + 128] = (xT[rows, s0 + c0:s0 + c0 + 128].astype(F32)
                                                    + gateT[0, rows, :] * v[:, t * 128:(t + 1) * 128])

        def combine(x, sign=None, y=None):
            if sign is None:
                return x
            x, y = x.astype(F32), y.astype(F32)
            return (x + y if sign > 0 else x - y).astype(BF)

        def operand(i, dst, n, o, w, xi, yi=None, sign=None):
            if i > 0:
                return _unpack(dst[n, :, o])
            v = combine(w[xi], sign, None if yi is None else w[yi])
            dst[n, :, o] = _pack(v)
            return v

        def gate_up(i, p):
            cols = (slice(2 * p * FC, (2 * p + 1) * FC), slice((2 * p + 1) * FC, (2 * p + 2) * FC))
            o = slice(p * FC, (p + 1) * FC)
            cs = []
            for w, w17 in ((wg, wg17), (wu, wu17)):
                m = {}
                for n in ORDER:
                    rows = slice(KO[n] // 2, (KO[n] + KS[n]) // 2)
                    if i > 0:
                        rhs = _unpack(w17[rows, o])
                    else:
                        rhs = jnp.concatenate(
                            [combine(w[e[0], cols[e[1]]], *((e[2], w[e[3], cols[e[4]]]) if len(e) > 2 else ()))
                             for e in RIGHT[n]], axis=0)
                        w17[rows, o] = _pack(rhs)
                    m[n] = _dot(_unpack(a17[i % 2, :, KO[n]:KO[n] + KS[n]]), rhs)
                cs.append(_quadrants(m))
            return [g * u for g, u in zip(*cs)]

        def stage_hidden(q, h0, h1):
            blocks = [[h[2 * j1 + k2][j2 * 128:(j2 + 1) * 128] for k2 in range(2) for j2 in range(2)]
                      for h in (h0, h1) for j1 in range(2)]
            for n, v in enumerate(_two_levels(_rights, blocks)):
                h49[n, :, q * FC:(q + 1) * FC] = _pack(v.astype(BF))

        done = []

        def prep_down(q, dist, slow, fresh=1):
            if fresh:
                done.clear()
            for c in range(0, FC, 128):
                for r in range(0, DQ, 16):
                    outer = [_lefts(*(wdT[i1 * DHALF + i2 * DQ + r:i1 * DHALF + i2 * DQ + r + 16,
                                          (4 * q + 2 * k1 + k2) * FC + c:(4 * q + 2 * k1 + k2) * FC + c + 128].astype(F32)
                                      for i1 in range(2) for k1 in range(2)))
                             for i2 in range(2) for k2 in range(2)]
                    for n in range(7):
                        blocks = [o[n] for o in outer]
                        if len(done) >= dist:
                            blocks[0] = after(blocks[0], done[-dist])
                        packed = [_pack(v.astype(BF)) for v in _lefts(*blocks)]
                        for k, v in enumerate(packed):
                            wd49[7 * n + k, r // 2:r // 2 + 8, q * FC + c:q * FC + c + 128] = v
                        link = functools.reduce(jnp.bitwise_or, packed)
                        if slow:
                            link = pltpu.roll(link, 1, 1)
                        link = pltpu.bitcast(link, F32)
                        done.append(jnp.concatenate([link, link], axis=0))

        out_cps = []

        def write_out(i, rows, c0, v):
            s0 = i * TM
            xT[rows, s0 + c0:s0 + c0 + 128] = (x1[i % 2, rows, c0:c0 + 128] + gateT[1, rows, :] * v).astype(BF)

        def hidden_one_level(h):
            return [v.astype(BF) for v in _rights(h[0], h[2], h[1], h[3])]

        def down_one_level(i, p, rights):
            lefts = _lefts(*(wdT[i1 * DHALF:(i1 + 1) * DHALF, (2 * p + k) * FC:(2 * p + k + 1) * FC].astype(F32)
                             for i1 in range(2) for k in range(2)))
            for n in (1, 3, 5, 0, 2, 4, 6):
                part = _dot_nt(lefts[n].astype(BF), rights[n])
                if p == 0:
                    acc7[n] = part
                else:
                    acc7[n] += part
            if p == nP - 1:
                for t in range(T // 128):
                    for n, v in enumerate(_quadrants([acc7[n, :, t * 128:(t + 1) * 128] for n in range(7)])):
                        write_out(i, slice((n // 2) * DHALF, (n // 2 + 1) * DHALF), (n % 2) * T + t * 128, v)
                out_cps.extend(copy_cols(xT, outT_hbm, i * TM, TM))

        def down(i):
            s0 = i * TM
            inner = [_quadrants([_dot_nt(_unpack(wd49[7 * n + k]), _unpack(h49[7 * n + k])) for k in range(7)])
                     for n in range(7)]
            for e2 in range(4):
                for e1, v in enumerate(_quadrants([inner[n][e2] for n in range(7)])):
                    r0 = (e1 // 2) * DHALF + (e2 // 2) * DQ
                    c0 = (e1 % 2) * T + (e2 % 2) * 128
                    write_out(i, slice(r0, r0 + DQ), c0, v)
            out_cps.extend(copy_cols(xT, outT_hbm, s0, TM))

        hidden = {}
        scope = None
        for step in sched + ["scope"]:
            op, *a = step.split()
            if op == "scope":
                if scope is not None:
                    scope.__exit__(None, None, None)
                scope = jax.named_scope(a[0]) if a else None
                if scope is not None:
                    scope.__enter__()
                continue
            if op == "wait":
                for n in a:
                    for cp in pending.pop(n):
                        cp.wait()
                continue
            if op == "waitout":
                out_cps.pop(0).wait()
                continue
            a = [int(v) for v in a]
            if op == "gu":
                hidden[tuple(a)] = gate_up(*a)
                if a[0] == 0:
                    hidden[tuple(a)] = hidden_one_level(hidden[tuple(a)])
                elif a[1] % 2:
                    stage_hidden(a[1] // 2, hidden.pop((a[0], a[1] - 1)), hidden.pop(tuple(a)))
            elif op == "down1":
                down_one_level(*a, hidden.pop(tuple(a)))
            else:
                {"mod0": prep_mod0, "mod1": prep_mod1, "mod2": prep_mod2, "prep": prep_wqkv, "prepwo": prep_wo,
                 "ln1": ln1, "ln2": ln2, "qkv": qkv, "att": attention, "wo": wo_proj, "down": down, "prepd": prep_down}[op](*a)
        assert not pending
        for cp in out_cps:
            cp.wait()

    n_sems = 6 + 3 * nP + 5 * nb
    hbm = pl.BlockSpec(memory_space=pltpu.HBM)

    def fn(A_x, A_wqkv, A_wo, B_x, B_w_gate, B_w_up, B_w_down, c, w_mod):
        del B_x
        outT = pl.pallas_call(
            kernel,
            in_specs=[pl.BlockSpec(memory_space=pltpu.VMEM)] + [hbm] * 7,
            out_specs=hbm,
            out_shape=jax.ShapeDtypeStruct((D, S), BF),
            scratch_shapes=[
                pltpu.VMEM((D, S), BF), pltpu.VMEM((D, 3 * D), BF), pltpu.VMEM((D, D), BF),
                pltpu.VMEM((D, F), BF), pltpu.VMEM((D, F), BF), pltpu.VMEM((D, F), BF),
                pltpu.VMEM((D, 6 * D), BF),
                pltpu.VMEM((NT, 1792, 128), F32), pltpu.VMEM((NT, D, 128), F32), pltpu.VMEM((NT, D, 128), F32),
                pltpu.VMEM((448, KT), I32), pltpu.VMEM((DHALF // 2, KT), I32),
                pltpu.VMEM((4, 8, NT * 128), F32), pltpu.VMEM((2, D, 128), F32),
                pltpu.VMEM((KT // 2, F // 2), I32), pltpu.VMEM((KT // 2, F // 2), I32),
                pltpu.VMEM((49, DQ // 2, F // 4), I32),
                pltpu.VMEM((NT, S, 128), F32), pltpu.VMEM((NT, HALO + S, 128), F32),
                pltpu.VMEM((NT, HALO + S, 128), F32),
                pltpu.VMEM((2, T // 2, KT), I32), pltpu.VMEM((T // 2, KT), I32),
                pltpu.VMEM((2, D, TM), F32),
                pltpu.VMEM((2, T // 2, KT), I32),
                pltpu.VMEM((49, 64, F // 4), I32), pltpu.VMEM((7, DHALF, T), F32),
                pltpu.SemaphoreType.DMA((n_sems,)),
            ],
            compiler_params=pltpu.CompilerParams(vmem_limit_bytes=126 * 2**20, flags=flags),
            name=name,
        )(c, A_x[0].T, A_wqkv, A_wo, B_w_gate, B_w_up, B_w_down.T, w_mod)
        return outT.T[None]

    return fn


SCHEDULE = (
    "wait m0; mod0; wait x0; ln1 0 0; wait q; prep 0; qkv 0 0; wait k v; prep 1; prep 2; qkv 0 1; "
    "wait x1 x2; qkv 0 2; ln1 1 1; qkv 1 0; qkv 1 1; qkv 1 2; ln1 2 1; qkv 2 0; qkv 2 1; att 0 3; "
    "wait wo m1 f0 f1; mod1; prepwo; wo 0; mod2; qkv 2 2; ln2 0 0; gu 0 0; gu 0 1; down1 0 0; "
    "wait f2 f3 f4 f5; gu 0 2; down1 0 1; gu 0 3; down1 0 2; gu 0 4; down1 0 3; att 1 1; wo 1; gu 0 5; "
    "down1 0 4; down1 0 5; ln2 1 1; wait x3; gu 1 0; gu 1 1; gu 1 2; gu 1 3; gu 1 4; att 2 1; wo 2; "
    "gu 1 5; prepd 0 2 1; prepd 1 2 1 0; prepd 2 2 1 0; down 1; ln2 2 1; waitout; gu 2 0; ln1 3 1; "
    "qkv 3 0; qkv 3 1; qkv 3 2; gu 2 1; gu 2 2; gu 2 3; gu 2 4; att 3 1; wo 3; gu 2 5; down 2; ln2 3 1; "
    "waitout; gu 3 0; gu 3 1; gu 3 2; gu 3 3; gu 3 4; gu 3 5; down 3; "
)
DMA = "m0 x0 q k v x1 x2 wo m1 f0 f1 f2 f3 f4 f5 x3"


@jax.jit
def pallas_adaLN_cond__sliding_local_dilated__glu_gated_bilinear__prompt_kernel(
    A_x: jax.Array,
    A_wqkv: jax.Array,
    A_wo: jax.Array,
    B_x: jax.Array,
    B_w_gate: jax.Array,
    B_w_up: jax.Array,
    B_w_down: jax.Array,
    c: jax.Array,
    w_mod: jax.Array,
):
    return make(sched=SCHEDULE, dma=DMA)(A_x, A_wqkv, A_wo, B_x, B_w_gate, B_w_up, B_w_down, c, w_mod)
```

```python
import contextlib
import functools

import jax
import jax.numpy as jnp
from jax import lax
import jax.experimental.pallas as pl
import jax.experimental.pallas.tpu as pltpu

S, D, H, DH, W, DIL, F = 2048, 576, 32, 18, 8, 2, 4608
HALO = 16
NT = 5
DHALF = D // 2
DQ = D // 4
EPS = 1e-5
LOG2E = 1.4426950408889634
QSCALE = DH ** -0.5 * LOG2E
BF, F32, I32 = jnp.bfloat16, jnp.float32, jnp.int32
NT_DIMS = (((1,), (1,)), ((), ()))


def _tw(j):
    return min(128, D - 128 * j)


def _dot(a, b):
    return jnp.dot(a, b, preferred_element_type=F32)


def _dot_nt(a, b):
    return lax.dot_general(a, b, NT_DIMS, preferred_element_type=F32)


def _pack(v):
    return pltpu.bitcast(v, jnp.int32)


def _unpack(v):
    return pltpu.bitcast(v, BF)


def _colsum(x):
    return jnp.sum(jnp.sum(x.reshape(D // 32, 32, 128), axis=0), axis=0, keepdims=True)


KS = (256, 256, 384, 384, 192, 384, 256)
KO = (0, 256, 512, 896, 1280, 1536, 1920)
KT = 2176
S1A, S2A, S1B, R1, S2B, R2, R3 = (
    slice(0, 128), slice(128, 256), slice(256, 320), slice(320, 384), slice(384, 448), slice(448, 512), slice(512, 576))
RIGHT = (
    ((S1A, 0, 1, S2A, 1), (S1B, 0, 1, S2B, 1), (R1, 0)),
    ((S1A, 0), (S1B, 0), (R2, 0)),
    ((S1A, 1, -1, S2A, 1), (S1B, 1, -1, S2B, 1), (R1, 1), (R3, 1), (R2, 1)),
    ((S2A, 0, -1, S1A, 0), (S2B, 0, -1, S1B, 0), (R2, 0), (R3, 0), (R1, 0)),
    ((S2A, 1), (S2B, 1)),
    ((S1A, 0, 1, S1A, 1), (S1B, 0, 1, S1B, 1), (R1, 0, 1, R1, 1), (R3, 1), (R2, 0, 1, R2, 1)),
    ((S2A, 0, 1, S2A, 1), (S2B, 0, 1, S2B, 1), (R3, 0)),
)


def _left_operands(p, q, lo):
    d = [y - x for x, y in zip(p, q)]
    w = lambda a, b: jnp.where(lo, a, b)
    return (
        (p[0] + q[1], w(p[2] + q[3], p[2] - q[2])),
        (q[0] + q[1], w(q[2] + q[3], d[3])),
        (p[0], p[2], w(p[4], p[3])),
        (q[1], w(q[3], p[3]), w(q[4], q[2])),
        (p[0] + p[1], p[2] + p[3]),
        (d[0], d[2], w(d[4], d[3])),
        (d[1], w(d[3], d[4])),
    )


def _right_operands(a, b, lo):
    w = lambda x, y: jnp.where(lo, x, y)
    return (
        lambda: (a(0) + b(1), w(a(2) + b(3), a(2))),
        lambda: (a(0), w(a(2), a(3))),
        lambda: (b(0) - b(1), w(b(2) - b(3), b(2)), w(b(4), b(3))),
        lambda: (a(1) - a(0), w(a(3) - a(2), a(3)), w(a(4), a(2))),
        lambda: (b(1), b(3)),
        lambda: (a(0) + b(0), a(2) + b(2), w(b(4), a(3) + b(3))),
        lambda: (a(1) + b(1), w(a(3) + b(3), a(4))),
    )


def _quadrant(m, e):
    return (lambda: m[0] - m[4] + m[3] - m[6], lambda: m[4] + m[2],
            lambda: m[1] + m[3], lambda: m[0] - m[1] + m[2] + m[5])[e]()


def _quadrants(m):
    return [_quadrant(m, e) for e in range(4)]


def _lefts(a11, a12, a21, a22):
    return a11 + a22, a21 + a22, a11, a22, a11 + a12, a21 - a11, a22 - a12


def _rights(b11, b12, b21, b22):
    return b11 + b22, b11, b12 - b22, b21 - b11, b22, b11 + b12, b21 + b22


def _two_levels(combos, blocks):
    outer = [combos(*(blocks[e1][e2] for e1 in range(4))) for e2 in range(4)]
    return [v for n in range(7) for v in combos(*(outer[e2][n] for e2 in range(4)))]


ORDER = (1, 4, 0, 2, 3, 5, 6)
_slabs = lambda part, lo, hi: [(part, d) for d in range(lo, hi)]
QKV_GROUPS = (
    (_slabs(0, 0, 8), _slabs(0, 8, 16)),
    (_slabs(1, 0, 8), _slabs(1, 8, 16)),
    (_slabs(2, 0, 8) + _slabs(0, 16, 18) + _slabs(1, 16, 18), _slabs(2, 8, 16) + _slabs(2, 16, 18) * 2),
)


DMA_ORDER = "m0 x0 q k v x1 wo m1 f0 f1 f2 f3 f4 f5 x2 x3"


def make(TM=512, FC=384, R=8, sched=None, dma=DMA_ORDER, flags=None, name="k12"):
    nb = S // TM
    T = TM // 2
    nP = F // (2 * FC)
    if isinstance(sched, str):
        sched = [t.strip() for t in sched.split(";") if t.strip()]
    dma = dma.split()

    def kernel(c_ref, xT_hbm, wqkv_hbm, wo_hbm, wg_hbm, wu_hbm, wdT_hbm, wmod_hbm, outT_hbm,
               xT, wqkv, wo, wg, wu, wdT, wmod, tmpT, tmpW, woT, wq17, wo17, modR, gateT, wg17, wu17, wd49,
               qbuf, kbuf, vbuf, h17, o17, x1, a17, h49, acc7, sems):
        sem_i = [0]

        def start_copy(src, dst):
            cp = pltpu.make_async_copy(src, dst, sems.at[sem_i[0]])
            sem_i[0] += 1
            cp.start()
            return cp

        def copy_cols(src, dst, c0, n):
            return [start_copy(src.at[:, pl.ds(c0, n)], dst.at[:, pl.ds(c0, n)])]

        pieces = {"m0": [(wmod_hbm, wmod, 0, 2 * D)], "m1": [(wmod_hbm, wmod, 2 * D, 4 * D)],
                  "qa": [(wqkv_hbm, wqkv, 0, 384)], "qb": [(wqkv_hbm, wqkv, 384, 256)],
                  "k": [(wqkv_hbm, wqkv, 640, 512)], "v": [(wqkv_hbm, wqkv, 1152, D)],
                  "wo": [(wo_hbm, wo, 0, D)]}
        for i in range(nb):
            pieces[f"x{i}"] = [(xT_hbm, xT, i * TM, TM)]
        for p in range(nP):
            pieces[f"f{p}"] = [(a, b, 2 * p * FC, 2 * FC) for a, b in ((wg_hbm, wg), (wu_hbm, wu), (wdT_hbm, wdT))]
        assert sorted(dma) == sorted(pieces)
        pending = {n: sum((copy_cols(*a) for a in pieces[n]), []) for n in dma}

        cbits = pltpu.bitcast(jnp.broadcast_to(c_ref[:, 0:128].astype(F32), (8, 128)), jnp.int32)
        keep = ((cbits * cbits) & 2) == 0

        def after(x, prev):
            k = jnp.broadcast_to(keep[0:1], x.shape[-2:])
            return jnp.where(k, x, prev)

        lane = lax.broadcasted_iota(jnp.int32, (1, 128), 1)
        lo = lane < 64

        def feature_tiles(y):
            return [y[j * 128:(j + 1) * 128] for j in range(4)] + [jnp.concatenate([y[512:D], y[512:D]], axis=0)]

        def store_left(dst, rows, p, q):
            for n, tiles in enumerate(_left_operands(p, q, lo)):
                for j, v in enumerate(tiles):
                    c0 = KO[n] + j * 128
                    dst[rows, c0:c0 + 128] = _pack(v.astype(BF))

        def prep_wqkv(first, last):
            for cb in range(first, last):
                cw = min(128, 3 * D - cb * 128)
                for j, t in enumerate(feature_tiles(wqkv[:, cb * 128:cb * 128 + cw].astype(F32))):
                    tmpT[j, cb * 128:cb * 128 + cw, :] = t.T

        def prep_wo():
            for j in range(NT):
                tmpW[j, :, 0:_tw(j)] = wo[:, j * 128:j * 128 + _tw(j)].astype(F32)
            for j in range(NT):
                p = jnp.concatenate([tmpW[j, pl.ds(d, H, stride=DH), :] for d in range(DH)], axis=0)
                for n, t in enumerate(feature_tiles(p[:, 0:_tw(j)])):
                    woT[n, j * 128:j * 128 + _tw(j), :] = t.T
            store_left(wo17, slice(None), [woT[n, 0:DHALF, :] for n in range(NT)], [woT[n, DHALF:D, :] for n in range(NT)])

        def modulation(c0, n):
            cf = c_ref[...].astype(F32)
            s = (cf * jax.nn.sigmoid(cf)).astype(BF)
            return _dot(jnp.broadcast_to(s, (16, D)), wmod[:, c0:c0 + n])[0:8]

        def to_column(row, n):
            for j in range(NT):
                r = row[0:1, j * 128:j * 128 + _tw(j)]
                gateT[n, j * 128:j * 128 + _tw(j), :] = jnp.broadcast_to(r, (128, _tw(j))).T

        def widen(row):
            return jnp.concatenate([row, row[:, 512:D]], axis=1)

        def prep_mod0():
            m = modulation(0, 2 * D)
            modR[0] = widen(m[:, 0:D])
            modR[1] = widen(1.0 + m[:, D:2 * D])

        def prep_mod1():
            to_column(modulation(2 * D, 640)[:, 0:D], 0)

        def prep_mod2():
            m = modulation(3 * D - 64, 3 * D + 64)
            modR[2] = widen(m[:, 64:64 + D])
            modR[3] = widen(1.0 + m[:, 64 + D:64 + 2 * D])
            to_column(m[:, 64 + 2 * D:64 + 3 * D], 1)

        def normalize(xf):
            mean = _colsum(xf) * (1.0 / D)
            xc = xf - mean
            var = _colsum(xc * xc) * (1.0 / D)
            return xc * lax.rsqrt(var + EPS)

        def modulate(t, j, n):
            return t * modR[2 * n + 1, 0:1, j * 128:(j + 1) * 128] + modR[2 * n, 0:1, j * 128:(j + 1) * 128]

        def layer_norm(dst, load, n, spread):
            prev = None
            for t in range(T // 128):
                halves = []
                for half in range(2):
                    xf = load(half * T + t * 128)
                    if prev is not None:
                        xf = jnp.concatenate([after(xf[0:128], prev), xf[128:D]], axis=0)
                    tiles = []
                    for j, y in enumerate(feature_tiles(normalize(xf))):
                        if spread and j > 0:
                            y = after(y, prev)
                        tiles.append(modulate(y.T, j, n))
                        prev = tiles[-1] if spread else None
                    halves.append(tiles)
                store_left(dst, slice(t * 64, (t + 1) * 64), *halves)

        def ln1(i, spread):
            layer_norm(h17.at[i % 2], lambda r: xT[:, i * TM + r:i * TM + r + 128].astype(F32), 0, spread)

        def ln2(i, spread):
            layer_norm(a17.at[i % 2], lambda r: x1[i % 2, :, r:r + 128], 1, spread)

        def qkv(i, g):
            s0 = i * TM
            sa, sb = QKV_GROUPS[g]
            rows = slice(g * 128, g * 128 + len(sa) * H // 2)
            if i == 0:
                gather = lambda slabs: lambda j: jnp.concatenate(
                    [tmpT[j, pl.ds(part * D + d, H, stride=DH), :] for part, d in slabs], axis=0)
                make_rhs = _right_operands(gather(sa), gather(sb), lo)
            m = {}
            for n in ORDER:
                cols = slice(KO[n], KO[n] + KS[n])
                if i == 0:
                    rhs = jnp.concatenate(make_rhs[n](), axis=1).astype(BF)[:, 0:KS[n]]
                    wq17[rows, cols] = _pack(rhs)
                else:
                    rhs = _unpack(wq17[rows, cols])
                m[n] = _dot_nt(_unpack(h17[i % 2, :, cols]), rhs)
            c11, c12, c21, c22 = _quadrants(m)
            for half, (ca, cb) in enumerate(((c11, c12), (c21, c22))):
                r = s0 + half * T
                tile = lambda j: (ca if j < 2 else cb)[:, (j % 2) * 128:(j % 2 + 1) * 128]
                for j in range(4):
                    if g == 0:
                        qbuf[j, r:r + T, :] = tile(j) * QSCALE
                    else:
                        (kbuf, vbuf)[g - 1][j, HALO + r:HALO + r + T, :] = tile(j)
                if g == 2:
                    xt = ca[:, 256:384]
                    qbuf[4, r:r + T, :] = jnp.where(lo, xt * QSCALE, 0.0)
                    kbuf[4, HALO + r:HALO + r + T, :] = jnp.where(lo, pltpu.roll(xt, 64, 1), 0.0)
                    vbuf[4, HALO + r:HALO + r + T, :] = cb[:, 256:384]
            if i == 0 and g == 2:
                for j in range(NT):
                    kbuf[j, 0:HALO, :] = jnp.broadcast_to(kbuf[j, HALO:HALO + 1, :], (HALO, 128))
                    vbuf[j, 0:HALO, :] = jnp.broadcast_to(vbuf[j, HALO:HALO + 1, :], (HALO, 128))

        def attend(r0, prev):
            q = qbuf[:, r0:r0 + R, :]
            if prev is not None:
                q = after(q, prev)
            ls = []
            for w in range(W):
                a = HALO + r0 - DIL * w
                p = jnp.sum(q * kbuf[:, a:a + R, :], axis=0)
                p = p + pltpu.roll(p, 64, 1)
                p = p + pltpu.roll(p, 32, 1)
                if r0 < DIL * w:
                    row = lax.broadcasted_iota(jnp.int32, (R, 128), 0) + r0
                    p = jnp.where(row >= DIL * w, p, -1e9 * LOG2E)
                ls.append(p)
            m = functools.reduce(jnp.maximum, ls)
            es = [jnp.exp2(l - m) for l in ls]
            den = functools.reduce(jnp.add, es)
            acc = None
            for w in range(W):
                a = HALO + r0 - DIL * w
                t = es[w][None] * vbuf[:, a:a + R, :]
                acc = t if acc is None else acc + t
            inv = pl.reciprocal(den, approx=True)
            inv = inv * (2.0 - den * inv)
            inv = inv * (2.0 - den * inv)
            return acc * inv[None]

        def attention(i, chained):
            done = []
            for r in range(0, T, 16):
                o = []
                for half in range(2):
                    for r0 in range(r, r + 16, R):
                        done.append(attend(i * TM + half * T + r0, done[-chained] if 0 < chained <= len(done) else None))
                    o.append(jnp.concatenate(done[-(16 // R):], axis=1))
                for n, tiles in enumerate(_right_operands(lambda j: o[0][j], lambda j: o[1][j], lo)):
                    for j, v in enumerate(tiles()):
                        c0 = KO[n] + j * 128
                        o17[r // 2:r // 2 + 8, c0:c0 + 128] = _pack(v.astype(BF))

        def wo_proj(i):
            s0 = i * TM
            m = {}
            for n in ORDER:
                cols = slice(KO[n], KO[n] + KS[n])
                m[n] = _dot_nt(_unpack(wo17[:, cols]), _unpack(o17[:, cols]))
            for n, v in enumerate(_quadrants(m)):
                rows = slice((n // 2) * DHALF, (n // 2 + 1) * DHALF)
                for t in range(T // 128):
                    c0 = (n % 2) * T + t * 128
                    x1[i % 2, rows, c0:c0 + 128] = (xT[rows, s0 + c0:s0 + c0 + 128].astype(F32)
                                                    + gateT[0, rows, :] * v[:, t * 128:(t + 1) * 128])

        def combine(x, sign=None, y=None):
            if sign is None:
                return x
            x, y = x.astype(F32), y.astype(F32)
            return (x + y if sign > 0 else x - y).astype(BF)

        def operand(i, dst, n, o, w, xi, yi=None, sign=None):
            if i > 0:
                return _unpack(dst[n, :, o])
            v = combine(w[xi], sign, None if yi is None else w[yi])
            dst[n, :, o] = _pack(v)
            return v

        def gate_up(i, p):
            cols = (slice(2 * p * FC, (2 * p + 1) * FC), slice((2 * p + 1) * FC, (2 * p + 2) * FC))
            o = slice(p * FC, (p + 1) * FC)
            cs = []
            for w, w17 in ((wg, wg17), (wu, wu17)):
                m = {}
                for n in ORDER:
                    rows = slice(KO[n] // 2, (KO[n] + KS[n]) // 2)
                    if i > 0:
                        rhs = _unpack(w17[rows, o])
                    else:
                        rhs = jnp.concatenate(
                            [combine(w[e[0], cols[e[1]]], *((e[2], w[e[3], cols[e[4]]]) if len(e) > 2 else ()))
                             for e in RIGHT[n]], axis=0)
                        w17[rows, o] = _pack(rhs)
                    m[n] = _dot(_unpack(a17[i % 2, :, KO[n]:KO[n] + KS[n]]), rhs)
                cs.append(_quadrants(m))
            return [g * u for g, u in zip(*cs)]

        def stage_hidden(q, h0, h1):
            blocks = [[h[2 * j1 + k2][j2 * 128:(j2 + 1) * 128] for k2 in range(2) for j2 in range(2)]
                      for h in (h0, h1) for j1 in range(2)]
            for n, v in enumerate(_two_levels(_rights, blocks)):
                h49[n, :, q * FC:(q + 1) * FC] = _pack(v.astype(BF))

        done = []

        def prep_down(q, dist, slow, fresh=1):
            if fresh:
                done.clear()
            for c in range(0, FC, 128):
                for r in range(0, DQ, 16):
                    outer = [_lefts(*(wdT[i1 * DHALF + i2 * DQ + r:i1 * DHALF + i2 * DQ + r + 16,
                                          (4 * q + 2 * k1 + k2) * FC + c:(4 * q + 2 * k1 + k2) * FC + c + 128].astype(F32)
                                      for i1 in range(2) for k1 in range(2)))
                             for i2 in range(2) for k2 in range(2)]
                    for n in range(7):
                        blocks = [o[n] for o in outer]
                        if len(done) >= dist:
                            blocks[0] = after(blocks[0], done[-dist])
                        packed = [_pack(v.astype(BF)) for v in _lefts(*blocks)]
                        for k, v in enumerate(packed):
                            wd49[7 * n + k, r // 2:r // 2 + 8, q * FC + c:q * FC + c + 128] = v
                        link = functools.reduce(jnp.bitwise_or, packed)
                        if slow:
                            link = pltpu.roll(link, 1, 1)
                        link = pltpu.bitcast(link, F32)
                        done.append(jnp.concatenate([link, link], axis=0))

        out_cps = []

        def write_out(i, rows, c0, v):
            s0 = i * TM
            xT[rows, s0 + c0:s0 + c0 + 128] = (x1[i % 2, rows, c0:c0 + 128] + gateT[1, rows, :] * v).astype(BF)

        def hidden_one_level(h):
            return [v.astype(BF) for v in _rights(h[0], h[2], h[1], h[3])]

        def down_one_level(i, p, rights):
            lefts = _lefts(*(wdT[i1 * DHALF:(i1 + 1) * DHALF, (2 * p + k) * FC:(2 * p + k + 1) * FC].astype(F32)
                             for i1 in range(2) for k in range(2)))
            for n in (1, 3, 5, 0, 2, 4, 6):
                part = _dot_nt(lefts[n].astype(BF), rights[n])
                if p == 0:
                    acc7[n] = part
                else:
                    acc7[n] += part
            if p == nP - 1:
                for t in range(T // 128):
                    for n, v in enumerate(_quadrants([acc7[n, :, t * 128:(t + 1) * 128] for n in range(7)])):
                        write_out(i, slice((n // 2) * DHALF, (n // 2 + 1) * DHALF), (n % 2) * T + t * 128, v)
                out_cps.append(copy_cols(xT, outT_hbm, i * TM, TM))

        def down(i):
            inner = {}
            for products, e1 in (((4, 2), 1), ((1, 3), 2), ((0, 5), 3), ((6,), 0)):
                for n in products:
                    inner[n] = _quadrants([_dot_nt(_unpack(wd49[7 * n + k]), _unpack(h49[7 * n + k])) for k in range(7)])
                r0, c0 = (e1 // 2) * DHALF, (e1 % 2) * T
                for e2 in range(4):
                    v = _quadrant({n: q[e2] for n, q in inner.items()}, e1)
                    write_out(i, slice(r0 + (e2 // 2) * DQ, r0 + (e2 // 2 + 1) * DQ), c0 + (e2 % 2) * 128, v)
                if i == nb - 1:
                    out_cps.append([start_copy(*(a.at[pl.ds(r0, DHALF), pl.ds(i * TM + c0, T)] for a in (xT, outT_hbm)))])
            if i < nb - 1:
                out_cps.append(copy_cols(xT, outT_hbm, i * TM, TM))

        hidden = {}
        scope = None
        for step in sched + ["scope"]:
            op, *a = step.split()
            if op == "scope":
                if scope is not None:
                    scope.__exit__(None, None, None)
                scope = jax.named_scope(a[0]) if a else None
                if scope is not None:
                    scope.__enter__()
                continue
            if op == "wait":
                for n in a:
                    for cp in pending.pop(n):
                        cp.wait()
                continue
            if op == "waitout":
                for cp in out_cps.pop(0):
                    cp.wait()
                continue
            a = [int(v) for v in a]
            if op == "gu":
                hidden[tuple(a)] = gate_up(*a)
                if a[0] == 0:
                    hidden[tuple(a)] = hidden_one_level(hidden[tuple(a)])
                elif a[1] % 2:
                    stage_hidden(a[1] // 2, hidden.pop((a[0], a[1] - 1)), hidden.pop(tuple(a)))
            elif op == "down1":
                down_one_level(*a, hidden.pop(tuple(a)))
            else:
                {"mod0": prep_mod0, "mod1": prep_mod1, "mod2": prep_mod2, "prep": prep_wqkv, "prepwo": prep_wo,
                 "ln1": ln1, "ln2": ln2, "qkv": qkv, "att": attention, "wo": wo_proj, "down": down, "prepd": prep_down}[op](*a)
        assert not pending
        for cp in sum(out_cps, []):
            cp.wait()

    n_sems = 7 + 3 * nP + 2 * nb + 3
    hbm = pl.BlockSpec(memory_space=pltpu.HBM)

    def fn(A_x, A_wqkv, A_wo, B_x, B_w_gate, B_w_up, B_w_down, c, w_mod):
        del B_x
        outT = pl.pallas_call(
            kernel,
            in_specs=[pl.BlockSpec(memory_space=pltpu.VMEM)] + [hbm] * 7,
            out_specs=hbm,
            out_shape=jax.ShapeDtypeStruct((D, S), BF),
            scratch_shapes=[
                pltpu.VMEM((D, S), BF), pltpu.VMEM((D, 3 * D), BF), pltpu.VMEM((D, D), BF),
                pltpu.VMEM((D, F), BF), pltpu.VMEM((D, F), BF), pltpu.VMEM((D, F), BF),
                pltpu.VMEM((D, 6 * D), BF),
                pltpu.VMEM((NT, 1792, 128), F32), pltpu.VMEM((NT, D, 128), F32), pltpu.VMEM((NT, D, 128), F32),
                pltpu.VMEM((448, KT), I32), pltpu.VMEM((DHALF // 2, KT), I32),
                pltpu.VMEM((4, 8, NT * 128), F32), pltpu.VMEM((2, D, 128), F32),
                pltpu.VMEM((KT // 2, F // 2), I32), pltpu.VMEM((KT // 2, F // 2), I32),
                pltpu.VMEM((49, DQ // 2, F // 4), I32),
                pltpu.VMEM((NT, S, 128), F32), pltpu.VMEM((NT, HALO + S, 128), F32),
                pltpu.VMEM((NT, HALO + S, 128), F32),
                pltpu.VMEM((2, T // 2, KT), I32), pltpu.VMEM((T // 2, KT), I32),
                pltpu.VMEM((2, D, TM), F32),
                pltpu.VMEM((2, T // 2, KT), I32),
                pltpu.VMEM((49, 64, F // 4), I32), pltpu.VMEM((7, DHALF, T), F32),
                pltpu.SemaphoreType.DMA((n_sems,)),
            ],
            compiler_params=pltpu.CompilerParams(vmem_limit_bytes=126 * 2**20, flags=flags),
            name=name,
        )(c, A_x[0].T, A_wqkv, A_wo, B_w_gate, B_w_up, B_w_down.T, w_mod)
        return outT.T[None]

    return fn


SCHEDULE = (
    "wait m0; mod0; wait x0; ln1 0 0; wait qa; prep 0 3; wait qb; prep 3 5; qkv 0 0; wait k v; prep 5 9; "
    "prep 9 14; qkv 0 1; wait x1 x2; qkv 0 2; ln1 1 1; qkv 1 0; qkv 1 1; qkv 1 2; ln1 2 1; qkv 2 0; "
    "qkv 2 1; att 0 5; wait wo m1 f0 f1; mod1; prepwo; wo 0; mod2; qkv 2 2; ln2 0 0; gu 0 0; gu 0 1; "
    "down1 0 0; wait f2 f3 f4 f5; gu 0 2; down1 0 1; gu 0 3; down1 0 2; gu 0 4; down1 0 3; att 1 1; wo 1; "
    "gu 0 5; down1 0 4; down1 0 5; ln2 1 1; wait x3; gu 1 0; gu 1 1; gu 1 2; gu 1 3; gu 1 4; att 2 1; "
    "wo 2; gu 1 5; prepd 0 2 1; prepd 1 2 1 0; prepd 2 2 1 0; down 1; ln2 2 1; waitout; gu 2 0; ln1 3 1; "
    "qkv 3 0; qkv 3 1; qkv 3 2; gu 2 1; gu 2 2; gu 2 3; gu 2 4; att 3 1; wo 3; gu 2 5; down 2; ln2 3 1; "
    "gu 3 0; gu 3 1; gu 3 2; gu 3 3; gu 3 4; gu 3 5; down 3; "
)
DMA = "m0 x0 qa qb k v x1 x2 wo m1 f0 f1 f2 f3 f4 f5 x3"


@jax.jit
def pallas_adaLN_cond__sliding_local_dilated__glu_gated_bilinear__prompt_kernel(
    A_x: jax.Array,
    A_wqkv: jax.Array,
    A_wo: jax.Array,
    B_x: jax.Array,
    B_w_gate: jax.Array,
    B_w_up: jax.Array,
    B_w_down: jax.Array,
    c: jax.Array,
    w_mod: jax.Array,
):
    return make(sched=SCHEDULE, dma=DMA)(A_x, A_wqkv, A_wo, B_x, B_w_gate, B_w_up, B_w_down, c, w_mod)
```

```python
import contextlib
import functools

import jax
import jax.numpy as jnp
from jax import lax
import jax.experimental.pallas as pl
import jax.experimental.pallas.tpu as pltpu

S, D, H, DH, W, DIL, F = 2048, 576, 32, 18, 8, 2, 4608
HALO = 16
NT = 5
DHALF = D // 2
DQ = D // 4
EPS = 1e-5
LOG2E = 1.4426950408889634
QSCALE = DH ** -0.5 * LOG2E
BF, F32, I32 = jnp.bfloat16, jnp.float32, jnp.int32
NT_DIMS = (((1,), (1,)), ((), ()))


def _tw(j):
    return min(128, D - 128 * j)


def _dot(a, b):
    return jnp.dot(a, b, preferred_element_type=F32)


def _dot_nt(a, b):
    return lax.dot_general(a, b, NT_DIMS, preferred_element_type=F32)


def _pack(v):
    return pltpu.bitcast(v, jnp.int32)


def _unpack(v):
    return pltpu.bitcast(v, BF)


def _colsum(x):
    return jnp.sum(jnp.sum(x.reshape(D // 32, 32, 128), axis=0), axis=0, keepdims=True)


KS = (256, 256, 384, 384, 192, 384, 256)
KO = (0, 256, 512, 896, 1280, 1536, 1920)
KT = 2176
LEFT3 = (
    ((0, 1, 0), (0, 0, 0)), ((0, 0, -1), (0, 0, 0)), ((-1, 0, 1), (0, 0, 0)), ((-1, 1, 0), (0, 0, 0)),
    ((0, -1, 0), (0, 1, 0)), ((0, 0, 0), (0, 0, -1)), ((0, -1, 1), (0, 1, -1)), ((0, -1, 0), (0, 1, -1)),
    ((0, 0, 0), (0, 1, -1)), ((1, 0, -1), (-1, 0, 1)), ((1, 0, 0), (-1, 0, 0)), ((1, 0, -1), (-1, 0, 0)),
    ((0, 0, 0), (-1, 0, 0)), ((0, 1, 0), (-1, 0, 0)), ((0, 0, 0), (-1, 1, 0)))
RIGHT3 = (
    ((0, -1, 0), (0, -1, 1), (0, 0, 0)), ((0, 0, -1), (0, 0, 0), (0, 1, -1)), ((0, 0, -1), (0, 0, 0), (0, 0, 0)),
    ((0, 1, 0), (0, 0, 0), (0, 0, 0)), ((0, 0, 0), (1, -1, 0), (0, -1, 0)), ((0, 0, 0), (0, 0, 1), (1, 0, 1)),
    ((0, 0, 0), (0, 0, 0), (0, 1, 0)), ((0, 0, 0), (0, 0, 1), (0, 1, 0)), ((0, 0, 0), (0, 0, 1), (0, 0, 0)),
    ((0, 0, 0), (0, 0, 0), (1, 0, 0)), ((1, -1, 0), (0, 0, 0), (1, 0, 0)), ((0, 0, -1), (0, 0, 0), (1, 0, 0)),
    ((-1, 0, -1), (-1, 0, 0), (0, 0, 0)), ((0, -1, 0), (-1, 0, 0), (0, 0, 0)), ((0, 0, 0), (-1, 0, 0), (0, 0, 0)))
EXTRA3 = (
    {1: ((1, 0), (0, 0, 1)), 3: ((1, 0), (0, -1, 0)), 4: ((1, -1), (-1, 1, 0)),
     5: ((0, 1), (0, 0, -1)), 13: ((1, 0), (-1, 1, 0)), 14: ((0, 1), (-1, 0, 0))},
    {1: ((1, 0), (0, -1, 1)), 4: ((0, 1), (0, -1, 0)), 5: ((0, 1), (-1, 0, -1)),
     6: ((1, 0), (0, 1, 0)), 9: ((0, 1), (1, 0, 0)), 10: ((1, 0), (1, 0, 0))},
    {3: ((1, 0), (0, -1, 1)), 6: ((1, 0), (0, 0, 1)), 9: ((0, 1), (0, 0, -1)),
     10: ((1, -1), (1, -1, 1)), 13: ((0, 1), (-1, 1, -1)), 14: ((0, 1), (-1, 0, -1))})
SLICES3 = tuple({(1, 2): (2, 1)}.get(s, s) for s in (tuple(k for k in range(3) if n in EXTRA3[k]) for n in range(15)))
KS3 = tuple(128 + 64 * len(s) for s in SLICES3)
KO3 = tuple(sum(KS3[:n]) for n in range(15))
KT3 = sum(KS3)
ORDER3 = (2, 11, 9, 12, 14, 5, 8, 7, 0, 3, 6, 1, 10, 13, 4)


def _outputs3(m):
    a, b = m[2] + m[11], m[7] - m[8]
    c, d = m[0] + b, m[9] - a
    return (m[10] + m[12] - m[3] - m[13] - a, m[6] - m[3] - c, m[1] + m[2] + m[6] - b,
            m[12] - m[14] + d, m[13] - m[4] - m[14] - c, m[8] - m[5] - d)


def _parts3(n):
    parts = [([(c, (i, k)) for i in range(2) for k, c in enumerate(LEFT3[n][i]) if c],
              [(c, (128 * k, 128, j)) for k in range(3) for j, c in enumerate(RIGHT3[n][k]) if c])]
    for s in SLICES3[n]:
        left, right = EXTRA3[s][n]
        parts.append(([(c, (i, 4 if s == 2 else 3)) for i, c in enumerate(left) if c],
                      [(c, (384 + 64 * s, 64, j)) for j, c in enumerate(right) if c]))
    return [([(c * r[0][0], x) for c, x in l], [(c * r[0][0], x) for c, x in r]) for l, r in parts]


def _signed_sum(terms):
    terms = sorted(terms, key=lambda t: -t[0])
    total = terms[0][1] if terms[0][0] > 0 else -terms[0][1]
    for c, v in terms[1:]:
        total = total + v if c > 0 else total - v
    return total


def _left_operands(p, q, lo):
    d = [y - x for x, y in zip(p, q)]
    w = lambda a, b: jnp.where(lo, a, b)
    return (
        (p[0] + q[1], w(p[2] + q[3], p[2] - q[2])),
        (q[0] + q[1], w(q[2] + q[3], d[3])),
        (p[0], p[2], w(p[4], p[3])),
        (q[1], w(q[3], p[3]), w(q[4], q[2])),
        (p[0] + p[1], p[2] + p[3]),
        (d[0], d[2], w(d[4], d[3])),
        (d[1], w(d[3], d[4])),
    )


def _right_operands(a, b, lo):
    w = lambda x, y: jnp.where(lo, x, y)
    return (
        lambda: (a(0) + b(1), w(a(2) + b(3), a(2))),
        lambda: (a(0), w(a(2), a(3))),
        lambda: (b(0) - b(1), w(b(2) - b(3), b(2)), w(b(4), b(3))),
        lambda: (a(1) - a(0), w(a(3) - a(2), a(3)), w(a(4), a(2))),
        lambda: (b(1), b(3)),
        lambda: (a(0) + b(0), a(2) + b(2), w(b(4), a(3) + b(3))),
        lambda: (a(1) + b(1), w(a(3) + b(3), a(4))),
    )


def _quadrant(m, e):
    return (lambda: m[0] - m[4] + m[3] - m[6], lambda: m[4] + m[2],
            lambda: m[1] + m[3], lambda: m[0] - m[1] + m[2] + m[5])[e]()


def _quadrants(m):
    return [_quadrant(m, e) for e in range(4)]


def _lefts(a11, a12, a21, a22):
    return a11 + a22, a21 + a22, a11, a22, a11 + a12, a21 - a11, a22 - a12


def _rights(b11, b12, b21, b22):
    return b11 + b22, b11, b12 - b22, b21 - b11, b22, b11 + b12, b21 + b22


def _two_levels(combos, blocks):
    outer = [combos(*(blocks[e1][e2] for e1 in range(4))) for e2 in range(4)]
    return [v for n in range(7) for v in combos(*(outer[e2][n] for e2 in range(4)))]


ORDER = (1, 4, 0, 2, 3, 5, 6)
PROGRESSIVE = (((4, 2), 1), ((1, 3), 2), ((0, 5), 3), ((6,), 0))
_slabs = lambda part, lo, hi: [(part, d) for d in range(lo, hi)]
QKV_GROUPS = (
    (_slabs(0, 0, 8), _slabs(0, 8, 16)),
    (_slabs(1, 0, 8), _slabs(1, 8, 16)),
    (_slabs(2, 0, 8) + _slabs(0, 16, 18) + _slabs(1, 16, 18), _slabs(2, 8, 16) + _slabs(2, 16, 18) * 2),
)


DMA_ORDER = "m0 x0 q k v x1 wo m1 f0 f1 f2 f3 f4 f5 x2 x3"


def make(TM=512, FC=384, R=8, sched=None, dma=DMA_ORDER, flags=None, name="k14"):
    nb = S // TM
    T = TM // 2
    nP = F // (2 * FC)
    if isinstance(sched, str):
        sched = [t.strip() for t in sched.split(";") if t.strip()]
    dma = dma.split()

    def kernel(c_ref, xT_hbm, wqkv_hbm, wo_hbm, wg_hbm, wu_hbm, wdT_hbm, wmod_hbm, outT_hbm,
               xT, wqkv, wo, wg, wu, wdT, wmod, tmpT, tmpW, woT, wq17, wo17, modR, gateT, wg24, wu24, wd49,
               qbuf, kbuf, vbuf, h17, o17, x1, a24, h49, acc7, sems):
        sem_i = [0]

        def start_copy(src, dst):
            cp = pltpu.make_async_copy(src, dst, sems.at[sem_i[0]])
            sem_i[0] += 1
            cp.start()
            return cp

        def copy_cols(src, dst, c0, n):
            return [start_copy(src.at[:, pl.ds(c0, n)], dst.at[:, pl.ds(c0, n)])]

        pieces = {"m0": [(wmod_hbm, wmod, 0, 2 * D)], "m1": [(wmod_hbm, wmod, 2 * D, 4 * D)],
                  "qa": [(wqkv_hbm, wqkv, 0, 384)], "qb": [(wqkv_hbm, wqkv, 384, 256)],
                  "k": [(wqkv_hbm, wqkv, 640, 512)], "v": [(wqkv_hbm, wqkv, 1152, D)],
                  "wo": [(wo_hbm, wo, 0, D)]}
        for i in range(nb):
            pieces[f"x{i}"] = [(xT_hbm, xT, i * TM, TM)]
        for p in range(nP):
            pieces[f"f{p}"] = [(a, b, 2 * p * FC, 2 * FC) for a, b in ((wg_hbm, wg), (wu_hbm, wu), (wdT_hbm, wdT))]
        assert sorted(dma) == sorted(pieces)
        pending = {n: sum((copy_cols(*a) for a in pieces[n]), []) for n in dma}

        cbits = pltpu.bitcast(jnp.broadcast_to(c_ref[:, 0:128].astype(F32), (8, 128)), jnp.int32)
        keep = ((cbits * cbits) & 2) == 0

        def after(x, prev):
            k = jnp.broadcast_to(keep[0:1], x.shape[-2:])
            return jnp.where(k, x, prev)

        lane = lax.broadcasted_iota(jnp.int32, (1, 128), 1)
        lo = lane < 64

        def feature_tiles(y):
            return [y[j * 128:(j + 1) * 128] for j in range(4)] + [jnp.concatenate([y[512:D], y[512:D]], axis=0)]

        def store_left(dst, rows, p, q):
            for n, tiles in enumerate(_left_operands(p, q, lo)):
                for j, v in enumerate(tiles):
                    c0 = KO[n] + j * 128
                    dst[rows, c0:c0 + 128] = _pack(v.astype(BF))

        def store_left3(dst, rows, *groups):
            for n in range(15):
                parts = [_signed_sum([(c, groups[i][k]) for c, (i, k) in left]) for left, _ in _parts3(n)]
                tiles = parts[:1] + ([jnp.where(lo, *parts[1:])] if len(parts) > 1 else [])
                for j, v in enumerate(tiles):
                    dst[rows, KO3[n] + j * 128:KO3[n] + (j + 1) * 128] = _pack(v.astype(BF))

        def prep_wqkv(first, last):
            for cb in range(first, last):
                cw = min(128, 3 * D - cb * 128)
                for j, t in enumerate(feature_tiles(wqkv[:, cb * 128:cb * 128 + cw].astype(F32))):
                    tmpT[j, cb * 128:cb * 128 + cw, :] = t.T

        def prep_wo():
            for j in range(NT):
                tmpW[j, :, 0:_tw(j)] = wo[:, j * 128:j * 128 + _tw(j)].astype(F32)
            for j in range(NT):
                p = jnp.concatenate([tmpW[j, pl.ds(d, H, stride=DH), :] for d in range(DH)], axis=0)
                for n, t in enumerate(feature_tiles(p[:, 0:_tw(j)])):
                    woT[n, j * 128:j * 128 + _tw(j), :] = t.T
            store_left(wo17, slice(None), [woT[n, 0:DHALF, :] for n in range(NT)], [woT[n, DHALF:D, :] for n in range(NT)])

        def modulation(c0, n):
            cf = c_ref[...].astype(F32)
            s = (cf * jax.nn.sigmoid(cf)).astype(BF)
            return _dot(jnp.broadcast_to(s, (16, D)), wmod[:, c0:c0 + n])[0:8]

        def to_column(row, n):
            for j in range(NT):
                r = row[0:1, j * 128:j * 128 + _tw(j)]
                gateT[n, j * 128:j * 128 + _tw(j), :] = jnp.broadcast_to(r, (128, _tw(j))).T

        def widen(row):
            return jnp.concatenate([row, row[:, 512:D]], axis=1)

        def prep_mod0():
            m = modulation(0, 2 * D)
            modR[0] = widen(m[:, 0:D])
            modR[1] = widen(1.0 + m[:, D:2 * D])

        def prep_mod1():
            to_column(modulation(2 * D, 640)[:, 0:D], 0)

        def prep_mod2():
            m = modulation(3 * D - 64, 3 * D + 64)
            modR[2] = widen(m[:, 64:64 + D])
            modR[3] = widen(1.0 + m[:, 64 + D:64 + 2 * D])
            to_column(m[:, 64 + 2 * D:64 + 3 * D], 1)

        def normalize(xf):
            mean = _colsum(xf) * (1.0 / D)
            xc = xf - mean
            var = _colsum(xc * xc) * (1.0 / D)
            return xc * lax.rsqrt(var + EPS)

        def modulate(t, j, n):
            return t * modR[2 * n + 1, 0:1, j * 128:(j + 1) * 128] + modR[2 * n, 0:1, j * 128:(j + 1) * 128]

        def layer_norm(store, load, n, spread):
            prev = None
            for t in range(T // 128):
                halves = []
                for half in range(2):
                    xf = load(half * T + t * 128)
                    if prev is not None:
                        xf = jnp.concatenate([after(xf[0:128], prev), xf[128:D]], axis=0)
                    tiles = []
                    for j, y in enumerate(feature_tiles(normalize(xf))):
                        if spread and j > 0:
                            y = after(y, prev)
                        tiles.append(modulate(y.T, j, n))
                        prev = tiles[-1] if spread else None
                    halves.append(tiles)
                store(slice(t * 64, (t + 1) * 64), *halves)

        def ln1(i, spread):
            layer_norm(functools.partial(store_left, h17.at[i % 2]), lambda r: xT[:, i * TM + r:i * TM + r + 128].astype(F32), 0, spread)

        def ln2(i, spread):
            layer_norm(functools.partial(store_left3, a24.at[i % 2]), lambda r: x1[i % 2, :, r:r + 128], 1, spread)

        partial = {}

        def qkv(i, g, first=0, last=7):
            s0 = i * TM
            sa, sb = QKV_GROUPS[g]
            rows = slice(g * 128, g * 128 + len(sa) * H // 2)
            if i == 0:
                gather = lambda slabs: lambda j: jnp.concatenate(
                    [tmpT[j, pl.ds(part * D + d, H, stride=DH), :] for part, d in slabs], axis=0)
                make_rhs = _right_operands(gather(sa), gather(sb), lo)
            m = partial.setdefault((i, g), {})
            for n in ORDER[first:last]:
                cols = slice(KO[n], KO[n] + KS[n])
                if i == 0:
                    rhs = jnp.concatenate(make_rhs[n](), axis=1).astype(BF)[:, 0:KS[n]]
                    wq17[rows, cols] = _pack(rhs)
                else:
                    rhs = _unpack(wq17[rows, cols])
                m[n] = _dot_nt(_unpack(h17[i % 2, :, cols]), rhs)
            if last < 7:
                return
            c11, c12, c21, c22 = _quadrants(m)
            for half, (ca, cb) in enumerate(((c11, c12), (c21, c22))):
                r = s0 + half * T
                tile = lambda j: (ca if j < 2 else cb)[:, (j % 2) * 128:(j % 2 + 1) * 128]
                for j in range(4):
                    if g == 0:
                        qbuf[j, r:r + T, :] = tile(j) * QSCALE
                    else:
                        (kbuf, vbuf)[g - 1][j, HALO + r:HALO + r + T, :] = tile(j)
                if g == 2:
                    xt = ca[:, 256:384]
                    qbuf[4, r:r + T, :] = jnp.where(lo, xt * QSCALE, 0.0)
                    kbuf[4, HALO + r:HALO + r + T, :] = jnp.where(lo, pltpu.roll(xt, 64, 1), 0.0)
                    vbuf[4, HALO + r:HALO + r + T, :] = cb[:, 256:384]
            if i == 0 and g == 2:
                for j in range(NT):
                    kbuf[j, 0:HALO, :] = jnp.broadcast_to(kbuf[j, HALO:HALO + 1, :], (HALO, 128))
                    vbuf[j, 0:HALO, :] = jnp.broadcast_to(vbuf[j, HALO:HALO + 1, :], (HALO, 128))

        def attend(r0, prev):
            q = qbuf[:, r0:r0 + R, :]
            if prev is not None:
                q = after(q, prev)
            ls = []
            for w in range(W):
                a = HALO + r0 - DIL * w
                p = jnp.sum(q * kbuf[:, a:a + R, :], axis=0)
                p = p + pltpu.roll(p, 64, 1)
                p = p + pltpu.roll(p, 32, 1)
                if r0 < DIL * w:
                    row = lax.broadcasted_iota(jnp.int32, (R, 128), 0) + r0
                    p = jnp.where(row >= DIL * w, p, -1e9 * LOG2E)
                ls.append(p)
            m = functools.reduce(jnp.maximum, ls)
            es = [jnp.exp2(l - m) for l in ls]
            den = functools.reduce(jnp.add, es)
            acc = None
            for w in range(W):
                a = HALO + r0 - DIL * w
                t = es[w][None] * vbuf[:, a:a + R, :]
                acc = t if acc is None else acc + t
            inv = pl.reciprocal(den, approx=True)
            inv = inv * (2.0 - den * inv)
            inv = inv * (2.0 - den * inv)
            return acc * inv[None]

        def attention(i, chained):
            done = []
            for r in range(0, T, 16):
                o = []
                for half in range(2):
                    for r0 in range(r, r + 16, R):
                        done.append(attend(i * TM + half * T + r0, done[-chained] if 0 < chained <= len(done) else None))
                    o.append(jnp.concatenate(done[-(16 // R):], axis=1))
                for n, tiles in enumerate(_right_operands(lambda j: o[0][j], lambda j: o[1][j], lo)):
                    for j, v in enumerate(tiles()):
                        c0 = KO[n] + j * 128
                        o17[r // 2:r // 2 + 8, c0:c0 + 128] = _pack(v.astype(BF))

        def wo_proj(i):
            s0 = i * TM
            m = {}
            for n in ORDER:
                cols = slice(KO[n], KO[n] + KS[n])
                m[n] = _dot_nt(_unpack(wo17[:, cols]), _unpack(o17[:, cols]))
            for n, v in enumerate(_quadrants(m)):
                rows = slice((n // 2) * DHALF, (n // 2 + 1) * DHALF)
                for t in range(T // 128):
                    c0 = (n % 2) * T + t * 128
                    x1[i % 2, rows, c0:c0 + 128] = (xT[rows, s0 + c0:s0 + c0 + 128].astype(F32)
                                                    + gateT[0, rows, :] * v[:, t * 128:(t + 1) * 128])

        def gate_up(i, p):
            fc = 2 * FC // 3
            cs = []
            for w, w24 in ((wg, wg24), (wu, wu24)):
                m = {}
                for n in ORDER3:
                    where = (slice(KO3[n] // 2, (KO3[n] + KS3[n]) // 2), slice(p * fc, (p + 1) * fc))
                    if i > 0:
                        rhs = _unpack(w24[where])
                    else:
                        parts = []
                        for _, right in _parts3(n):
                            terms = [(c, w[r:r + k, (3 * p + j) * fc:(3 * p + j + 1) * fc]) for c, (r, k, j) in right]
                            parts.append(terms[0][1] if len(terms) == 1 else
                                         _signed_sum([(c, v.astype(F32)) for c, v in terms]).astype(BF))
                        rhs = jnp.concatenate(parts, axis=0)
                        w24[where] = _pack(rhs)
                    m[n] = _dot(_unpack(a24[i % 2, :, KO3[n]:KO3[n] + KS3[n]]), rhs)
                cs.append(_outputs3(m))
            h = [g * u for g, u in zip(*cs)]
            h = [jnp.concatenate(h[3 * half:3 * half + 3], axis=1) for half in range(2)]
            return [v[:, k * FC:(k + 1) * FC] for v in h for k in range(2)]

        def stage_hidden(q, h0, h1):
            blocks = [[h[2 * j1 + k2][j2 * 128:(j2 + 1) * 128] for k2 in range(2) for j2 in range(2)]
                      for h in (h0, h1) for j1 in range(2)]
            for n, v in enumerate(_two_levels(_rights, blocks)):
                h49[n, :, q * FC:(q + 1) * FC] = _pack(v.astype(BF))

        done = []

        def prep_down(q, dist, slow, fresh=1):
            if fresh:
                done.clear()
            for c in range(0, FC, 128):
                for r in range(0, DQ, 16):
                    outer = [_lefts(*(wdT[i1 * DHALF + i2 * DQ + r:i1 * DHALF + i2 * DQ + r + 16,
                                          (4 * q + 2 * k1 + k2) * FC + c:(4 * q + 2 * k1 + k2) * FC + c + 128].astype(F32)
                                      for i1 in range(2) for k1 in range(2)))
                             for i2 in range(2) for k2 in range(2)]
                    for n in range(7):
                        blocks = [o[n] for o in outer]
                        if len(done) >= dist:
                            blocks[0] = after(blocks[0], done[-dist])
                        packed = [_pack(v.astype(BF)) for v in _lefts(*blocks)]
                        for k, v in enumerate(packed):
                            wd49[7 * n + k, r // 2:r // 2 + 8, q * FC + c:q * FC + c + 128] = v
                        link = functools.reduce(jnp.bitwise_or, packed)
                        if slow:
                            link = pltpu.roll(link, 1, 1)
                        link = pltpu.bitcast(link, F32)
                        done.append(jnp.concatenate([link, link], axis=0))

        out_cps = []

        def write_out(i, rows, c0, v):
            s0 = i * TM
            xT[rows, s0 + c0:s0 + c0 + 128] = (x1[i % 2, rows, c0:c0 + 128] + gateT[1, rows, :] * v).astype(BF)

        def hidden_one_level(h):
            return [v.astype(BF) for v in _rights(h[0], h[2], h[1], h[3])]

        def down_one_level(i, p, rights):
            lefts = _lefts(*(wdT[i1 * DHALF:(i1 + 1) * DHALF, (2 * p + k) * FC:(2 * p + k + 1) * FC].astype(F32)
                             for i1 in range(2) for k in range(2)))
            prods = {}
            for products, e in PROGRESSIVE:
                for n in products:
                    part = _dot_nt(lefts[n].astype(BF), rights[n])
                    prods[n] = part if p == 0 else acc7[n] + part
                    if p < nP - 1:
                        acc7[n] = prods[n]
                if p == nP - 1:
                    v = _quadrant(prods, e)
                    for t in range(T // 128):
                        write_out(i, slice((e // 2) * DHALF, (e // 2 + 1) * DHALF), (e % 2) * T + t * 128,
                                  v[:, t * 128:(t + 1) * 128])
            if p == nP - 1:
                out_cps.append(copy_cols(xT, outT_hbm, i * TM, TM))

        def down(i):
            inner = {}
            for products, e1 in PROGRESSIVE:
                for n in products:
                    inner[n] = _quadrants([_dot_nt(_unpack(wd49[7 * n + k]), _unpack(h49[7 * n + k])) for k in range(7)])
                r0, c0 = (e1 // 2) * DHALF, (e1 % 2) * T
                for e2 in range(4):
                    v = _quadrant({n: q[e2] for n, q in inner.items()}, e1)
                    write_out(i, slice(r0 + (e2 // 2) * DQ, r0 + (e2 // 2 + 1) * DQ), c0 + (e2 % 2) * 128, v)
                if i == nb - 1:
                    out_cps.append([start_copy(*(a.at[pl.ds(r0, DHALF), pl.ds(i * TM + c0, T)] for a in (xT, outT_hbm)))])
            if i < nb - 1:
                out_cps.append(copy_cols(xT, outT_hbm, i * TM, TM))

        hidden = {}
        scope = None
        for step in sched + ["scope"]:
            op, *a = step.split()
            if op == "scope":
                if scope is not None:
                    scope.__exit__(None, None, None)
                scope = jax.named_scope(a[0]) if a else None
                if scope is not None:
                    scope.__enter__()
                continue
            if op == "wait":
                for n in a:
                    for cp in pending.pop(n):
                        cp.wait()
                continue
            if op == "waitout":
                for cp in out_cps.pop(0):
                    cp.wait()
                continue
            a = [int(v) for v in a]
            if op == "gu":
                hidden[tuple(a)] = gate_up(*a)
                if a[0] == 0:
                    hidden[tuple(a)] = hidden_one_level(hidden[tuple(a)])
                elif a[1] % 2:
                    stage_hidden(a[1] // 2, hidden.pop((a[0], a[1] - 1)), hidden.pop(tuple(a)))
            elif op == "down1":
                down_one_level(*a, hidden.pop(tuple(a)))
            else:
                {"mod0": prep_mod0, "mod1": prep_mod1, "mod2": prep_mod2, "prep": prep_wqkv, "prepwo": prep_wo,
                 "ln1": ln1, "ln2": ln2, "qkv": qkv, "att": attention, "wo": wo_proj, "down": down, "prepd": prep_down}[op](*a)
        assert not pending
        for cp in sum(out_cps, []):
            cp.wait()

    n_sems = 7 + 3 * nP + 2 * nb + 3
    hbm = pl.BlockSpec(memory_space=pltpu.HBM)

    def fn(A_x, A_wqkv, A_wo, B_x, B_w_gate, B_w_up, B_w_down, c, w_mod):
        del B_x
        outT = pl.pallas_call(
            kernel,
            in_specs=[pl.BlockSpec(memory_space=pltpu.VMEM)] + [hbm] * 7,
            out_specs=hbm,
            out_shape=jax.ShapeDtypeStruct((D, S), BF),
            scratch_shapes=[
                pltpu.VMEM((D, S), BF), pltpu.VMEM((D, 3 * D), BF), pltpu.VMEM((D, D), BF),
                pltpu.VMEM((D, F), BF), pltpu.VMEM((D, F), BF), pltpu.VMEM((D, F), BF),
                pltpu.VMEM((D, 6 * D), BF),
                pltpu.VMEM((NT, 1792, 128), F32), pltpu.VMEM((NT, D, 128), F32), pltpu.VMEM((NT, D, 128), F32),
                pltpu.VMEM((448, KT), I32), pltpu.VMEM((DHALF // 2, KT), I32),
                pltpu.VMEM((4, 8, NT * 128), F32), pltpu.VMEM((2, D, 128), F32),
                pltpu.VMEM((KT3 // 2, F // 3), I32), pltpu.VMEM((KT3 // 2, F // 3), I32),
                pltpu.VMEM((49, DQ // 2, F // 4), I32),
                pltpu.VMEM((NT, S, 128), F32), pltpu.VMEM((NT, HALO + S, 128), F32),
                pltpu.VMEM((NT, HALO + S, 128), F32),
                pltpu.VMEM((2, T // 2, KT), I32), pltpu.VMEM((T // 2, KT), I32),
                pltpu.VMEM((2, D, TM), F32),
                pltpu.VMEM((2, T // 2, KT3), I32),
                pltpu.VMEM((49, 64, F // 4), I32), pltpu.VMEM((7, DHALF, T), F32),
                pltpu.SemaphoreType.DMA((n_sems,)),
            ],
            compiler_params=pltpu.CompilerParams(vmem_limit_bytes=126 * 2**20, flags=flags),
            name=name,
        )(c, A_x[0].T, A_wqkv, A_wo, B_w_gate, B_w_up, B_w_down.T, w_mod)
        return outT.T[None]

    return fn


SCHEDULE = (
    "wait m0; mod0; wait x0; ln1 0 0; wait qa; prep 0 3; wait qb; prep 3 5; qkv 0 0 0 4; wait k; prep 5 9; "
    "qkv 0 0 4 7; qkv 0 1 0 2; wait v; prep 9 14; qkv 0 1 2 7; wait x1 x2; qkv 0 2; ln1 1 1; qkv 1 0; "
    "qkv 1 1; qkv 1 2; ln1 2 1; qkv 2 0; qkv 2 1; att 0 5; wait wo m1 f0 f1; mod1; prepwo; wo 0; mod2; "
    "qkv 2 2; ln2 0 0; gu 0 0; gu 0 1; down1 0 0; wait f2 f3 f4 f5; gu 0 2; down1 0 1; gu 0 3; down1 0 2; "
    "gu 0 4; down1 0 3; att 1 1; wo 1; gu 0 5; down1 0 4; down1 0 5; ln2 1 1; wait x3; gu 1 0; gu 1 1; "
    "gu 1 2; gu 1 3; gu 1 4; att 2 1; wo 2; gu 1 5; prepd 0 3 1; prepd 1 3 1 0; prepd 2 3 1 0; down 1; "
    "ln2 2 1; waitout; gu 2 0; ln1 3 1; qkv 3 0; qkv 3 1; qkv 3 2; gu 2 1; gu 2 2; gu 2 3; gu 2 4; "
    "att 3 1; wo 3; gu 2 5; down 2; ln2 3 1; gu 3 0; gu 3 1; gu 3 2; gu 3 3; gu 3 4; gu 3 5; down 3; "
)
DMA = "m0 x0 qa qb k v x1 x2 wo m1 f0 f1 f2 f3 f4 f5 x3"


@jax.jit
def pallas_adaLN_cond__sliding_local_dilated__glu_gated_bilinear__prompt_kernel(
    A_x: jax.Array,
    A_wqkv: jax.Array,
    A_wo: jax.Array,
    B_x: jax.Array,
    B_w_gate: jax.Array,
    B_w_up: jax.Array,
    B_w_down: jax.Array,
    c: jax.Array,
    w_mod: jax.Array,
):
    return make(sched=SCHEDULE, dma=DMA)(A_x, A_wqkv, A_wo, B_x, B_w_gate, B_w_up, B_w_down, c, w_mod)
```

```python
import contextlib
import functools

import jax
import jax.numpy as jnp
from jax import lax
import jax.experimental.pallas as pl
import jax.experimental.pallas.tpu as pltpu

S, D, H, DH, W, DIL, F = 2048, 576, 32, 18, 8, 2, 4608
HALO = 16
NT = 5
DHALF = D // 2
DQ = D // 4
EPS = 1e-5
LOG2E = 1.4426950408889634
QSCALE = DH ** -0.5 * LOG2E
BF, F32, I32 = jnp.bfloat16, jnp.float32, jnp.int32
NT_DIMS = (((1,), (1,)), ((), ()))


def _tw(j):
    return min(128, D - 128 * j)


def _dot(a, b):
    return jnp.dot(a, b, preferred_element_type=F32)


def _dot_nt(a, b):
    return lax.dot_general(a, b, NT_DIMS, preferred_element_type=F32)


def _pack(v):
    return pltpu.bitcast(v, jnp.int32)


def _unpack(v):
    return pltpu.bitcast(v, BF)


def _colsum(x):
    return jnp.sum(jnp.sum(x.reshape(D // 32, 32, 128), axis=0), axis=0, keepdims=True)


KS = (256, 256, 384, 384, 192, 384, 256)
KO = (0, 256, 512, 896, 1280, 1536, 1920)
KT = 2176
LEFT3 = (
    ((0, 1, 0), (0, 0, 0)), ((0, 0, -1), (0, 0, 0)), ((-1, 0, 1), (0, 0, 0)), ((-1, 1, 0), (0, 0, 0)),
    ((0, -1, 0), (0, 1, 0)), ((0, 0, 0), (0, 0, -1)), ((0, -1, 1), (0, 1, -1)), ((0, -1, 0), (0, 1, -1)),
    ((0, 0, 0), (0, 1, -1)), ((1, 0, -1), (-1, 0, 1)), ((1, 0, 0), (-1, 0, 0)), ((1, 0, -1), (-1, 0, 0)),
    ((0, 0, 0), (-1, 0, 0)), ((0, 1, 0), (-1, 0, 0)), ((0, 0, 0), (-1, 1, 0)))
RIGHT3 = (
    ((0, -1, 0), (0, -1, 1), (0, 0, 0)), ((0, 0, -1), (0, 0, 0), (0, 1, -1)), ((0, 0, -1), (0, 0, 0), (0, 0, 0)),
    ((0, 1, 0), (0, 0, 0), (0, 0, 0)), ((0, 0, 0), (1, -1, 0), (0, -1, 0)), ((0, 0, 0), (0, 0, 1), (1, 0, 1)),
    ((0, 0, 0), (0, 0, 0), (0, 1, 0)), ((0, 0, 0), (0, 0, 1), (0, 1, 0)), ((0, 0, 0), (0, 0, 1), (0, 0, 0)),
    ((0, 0, 0), (0, 0, 0), (1, 0, 0)), ((1, -1, 0), (0, 0, 0), (1, 0, 0)), ((0, 0, -1), (0, 0, 0), (1, 0, 0)),
    ((-1, 0, -1), (-1, 0, 0), (0, 0, 0)), ((0, -1, 0), (-1, 0, 0), (0, 0, 0)), ((0, 0, 0), (-1, 0, 0), (0, 0, 0)))
EXTRA3 = (
    {1: ((1, 0), (0, 0, 1)), 3: ((1, 0), (0, -1, 0)), 4: ((1, -1), (-1, 1, 0)),
     5: ((0, 1), (0, 0, -1)), 13: ((1, 0), (-1, 1, 0)), 14: ((0, 1), (-1, 0, 0))},
    {1: ((1, 0), (0, -1, 1)), 4: ((0, 1), (0, -1, 0)), 5: ((0, 1), (-1, 0, -1)),
     6: ((1, 0), (0, 1, 0)), 9: ((0, 1), (1, 0, 0)), 10: ((1, 0), (1, 0, 0))},
    {3: ((1, 0), (0, -1, 1)), 6: ((1, 0), (0, 0, 1)), 9: ((0, 1), (0, 0, -1)),
     10: ((1, -1), (1, -1, 1)), 13: ((0, 1), (-1, 1, -1)), 14: ((0, 1), (-1, 0, -1))})
SLICES3 = tuple({(1, 2): (2, 1)}.get(s, s) for s in (tuple(k for k in range(3) if n in EXTRA3[k]) for n in range(15)))
KS3 = tuple(128 + 64 * len(s) for s in SLICES3)
KO3 = tuple(sum(KS3[:n]) for n in range(15))
KT3 = sum(KS3)
ORDER3 = (2, 11, 9, 12, 14, 8, 5, 7, 0, 3, 6, 1, 13, 10, 4)


def _outputs3(m):
    a, b = m[2] + m[11], m[7] - m[8]
    c, d = m[0] + b, m[9] - a
    return (m[12] - a - m[3] - m[13] + m[10], m[6] - (c + m[3]), m[2] - b + m[6] + m[1],
            m[12] + d - m[14], m[13] - (m[14] + c) - m[4], m[8] - d - m[5])


def _parts3(n):
    parts = [([(c, (i, k)) for i in range(2) for k, c in enumerate(LEFT3[n][i]) if c],
              [(c, (128 * k, 128, j)) for k in range(3) for j, c in enumerate(RIGHT3[n][k]) if c])]
    for s in SLICES3[n]:
        left, right = EXTRA3[s][n]
        parts.append(([(c, (i, 4 if s == 2 else 3)) for i, c in enumerate(left) if c],
                      [(c, (384 + 64 * s, 64, j)) for j, c in enumerate(right) if c]))
    return [([(c * r[0][0], x) for c, x in l], [(c * r[0][0], x) for c, x in r]) for l, r in parts]


def _signed_sum(terms):
    terms = sorted(terms, key=lambda t: -t[0])
    total = terms[0][1] if terms[0][0] > 0 else -terms[0][1]
    for c, v in terms[1:]:
        total = total + v if c > 0 else total - v
    return total


def _left_operands(p, q, lo):
    d = [y - x for x, y in zip(p, q)]
    w = lambda a, b: jnp.where(lo, a, b)
    return (
        (p[0] + q[1], w(p[2] + q[3], p[2] - q[2])),
        (q[0] + q[1], w(q[2] + q[3], d[3])),
        (p[0], p[2], w(p[4], p[3])),
        (q[1], w(q[3], p[3]), w(q[4], q[2])),
        (p[0] + p[1], p[2] + p[3]),
        (d[0], d[2], w(d[4], d[3])),
        (d[1], w(d[3], d[4])),
    )


def _right_operands(a, b, lo):
    w = lambda x, y: jnp.where(lo, x, y)
    return (
        lambda: (a(0) + b(1), w(a(2) + b(3), a(2))),
        lambda: (a(0), w(a(2), a(3))),
        lambda: (b(0) - b(1), w(b(2) - b(3), b(2)), w(b(4), b(3))),
        lambda: (a(1) - a(0), w(a(3) - a(2), a(3)), w(a(4), a(2))),
        lambda: (b(1), b(3)),
        lambda: (a(0) + b(0), a(2) + b(2), w(b(4), a(3) + b(3))),
        lambda: (a(1) + b(1), w(a(3) + b(3), a(4))),
    )


def _quadrant(m, e):
    return (lambda: m[0] - m[4] + m[3] - m[6], lambda: m[4] + m[2],
            lambda: m[1] + m[3], lambda: m[0] - m[1] + m[2] + m[5])[e]()


def _quadrants(m):
    return [_quadrant(m, e) for e in range(4)]


def _lefts(a11, a12, a21, a22):
    return a11 + a22, a21 + a22, a11, a22, a11 + a12, a21 - a11, a22 - a12


def _rights(b11, b12, b21, b22):
    return b11 + b22, b11, b12 - b22, b21 - b11, b22, b11 + b12, b21 + b22


def _two_levels(combos, blocks):
    outer = [combos(*(blocks[e1][e2] for e1 in range(4))) for e2 in range(4)]
    return [v for n in range(7) for v in combos(*(outer[e2][n] for e2 in range(4)))]


ORDER = (1, 4, 0, 2, 3, 5, 6)
PROGRESSIVE = (((4, 2), 1), ((1, 3), 2), ((0, 5), 3), ((6,), 0))
_slabs = lambda part, lo, hi: [(part, d) for d in range(lo, hi)]
QKV_GROUPS = (
    (_slabs(0, 0, 8), _slabs(0, 8, 16)),
    (_slabs(1, 0, 8), _slabs(1, 8, 16)),
    (_slabs(2, 0, 8) + _slabs(0, 16, 18) + _slabs(1, 16, 18), _slabs(2, 8, 16) + _slabs(2, 16, 18) * 2),
)


DMA_ORDER = "m0 x0 q k v x1 wo m1 f0 f1 f2 f3 f4 f5 x2 x3"


def make(order3=ORDER3, TM=512, FC=384, R=8, sched=None, dma=DMA_ORDER, flags=None, name="k15"):
    nb = S // TM
    T = TM // 2
    nP = F // (2 * FC)
    if isinstance(sched, str):
        sched = [t.strip() for t in sched.split(";") if t.strip()]
    dma = dma.split()

    def kernel(c_ref, xT_hbm, wqkv_hbm, wo_hbm, wg_hbm, wu_hbm, wdT_hbm, wmod_hbm, outT_hbm,
               xT, wqkv, wo, wg, wu, wdT, wmod, tmpT, tmpW, woT, wq17, wo17, modR, gateT, wg24, wu24, wd49,
               qbuf, kbuf, vbuf, h17, o17, x1, a24, acc7, sems):
        sem_i = [0]

        def start_copy(src, dst):
            cp = pltpu.make_async_copy(src, dst, sems.at[sem_i[0]])
            sem_i[0] += 1
            cp.start()
            return cp

        def copy_cols(src, dst, c0, n):
            return [start_copy(src.at[:, pl.ds(c0, n)], dst.at[:, pl.ds(c0, n)])]

        pieces = {"m0": [(wmod_hbm, wmod, 0, 2 * D)], "m1": [(wmod_hbm, wmod, 2 * D, 4 * D)],
                  "qa": [(wqkv_hbm, wqkv, 0, 384)], "qb": [(wqkv_hbm, wqkv, 384, 256)],
                  "k": [(wqkv_hbm, wqkv, 640, 512)], "v": [(wqkv_hbm, wqkv, 1152, D)],
                  "wo": [(wo_hbm, wo, 0, D)]}
        for i in range(nb):
            pieces[f"x{i}"] = [(xT_hbm, xT, i * TM, TM)]
        for p in range(nP):
            pieces[f"f{p}"] = [(a, b, 2 * p * FC, 2 * FC) for a, b in ((wg_hbm, wg), (wu_hbm, wu), (wdT_hbm, wdT))]
        assert sorted(dma) == sorted(pieces)
        pending = {n: sum((copy_cols(*a) for a in pieces[n]), []) for n in dma}

        cbits = pltpu.bitcast(jnp.broadcast_to(c_ref[:, 0:128].astype(F32), (8, 128)), jnp.int32)
        keep = ((cbits * cbits) & 2) == 0

        def after(x, prev):
            k = jnp.broadcast_to(keep[0:1], x.shape[-2:])
            return jnp.where(k, x, prev)

        lane = lax.broadcasted_iota(jnp.int32, (1, 128), 1)
        lo = lane < 64

        def feature_tiles(y):
            return [y[j * 128:(j + 1) * 128] for j in range(4)] + [jnp.concatenate([y[512:D], y[512:D]], axis=0)]

        def store_left(dst, rows, p, q):
            for n, tiles in enumerate(_left_operands(p, q, lo)):
                for j, v in enumerate(tiles):
                    c0 = KO[n] + j * 128
                    dst[rows, c0:c0 + 128] = _pack(v.astype(BF))

        def store_left3(dst, rows, *groups):
            for n in range(15):
                parts = [_signed_sum([(c, groups[i][k]) for c, (i, k) in left]) for left, _ in _parts3(n)]
                tiles = parts[:1] + ([jnp.where(lo, *parts[1:])] if len(parts) > 1 else [])
                for j, v in enumerate(tiles):
                    dst[rows, KO3[n] + j * 128:KO3[n] + (j + 1) * 128] = _pack(v.astype(BF))

        def prep_wqkv(first, last):
            for cb in range(first, last):
                cw = min(128, 3 * D - cb * 128)
                for j, t in enumerate(feature_tiles(wqkv[:, cb * 128:cb * 128 + cw].astype(F32))):
                    tmpT[j, cb * 128:cb * 128 + cw, :] = t.T

        def prep_wo():
            for j in range(NT):
                tmpW[j, :, 0:_tw(j)] = wo[:, j * 128:j * 128 + _tw(j)].astype(F32)
            for j in range(NT):
                p = jnp.concatenate([tmpW[j, pl.ds(d, H, stride=DH), :] for d in range(DH)], axis=0)
                for n, t in enumerate(feature_tiles(p[:, 0:_tw(j)])):
                    woT[n, j * 128:j * 128 + _tw(j), :] = t.T
            store_left(wo17, slice(None), [woT[n, 0:DHALF, :] for n in range(NT)], [woT[n, DHALF:D, :] for n in range(NT)])

        def modulation(c0, n):
            cf = c_ref[...].astype(F32)
            s = (cf * jax.nn.sigmoid(cf)).astype(BF)
            return _dot(jnp.broadcast_to(s, (16, D)), wmod[:, c0:c0 + n])[0:8]

        def to_column(row, n):
            for j in range(NT):
                r = row[0:1, j * 128:j * 128 + _tw(j)]
                gateT[n, j * 128:j * 128 + _tw(j), :] = jnp.broadcast_to(r, (128, _tw(j))).T

        def widen(row):
            return jnp.concatenate([row, row[:, 512:D]], axis=1)

        def prep_mod0():
            m = modulation(0, 2 * D)
            modR[0] = widen(m[:, 0:D])
            modR[1] = widen(1.0 + m[:, D:2 * D])

        def prep_mod1():
            to_column(modulation(2 * D, 640)[:, 0:D], 0)

        def prep_mod2():
            m = modulation(3 * D - 64, 3 * D + 64)
            modR[2] = widen(m[:, 64:64 + D])
            modR[3] = widen(1.0 + m[:, 64 + D:64 + 2 * D])
            to_column(m[:, 64 + 2 * D:64 + 3 * D], 1)

        def normalize(xf):
            mean = _colsum(xf) * (1.0 / D)
            xc = xf - mean
            var = _colsum(xc * xc) * (1.0 / D)
            return xc * lax.rsqrt(var + EPS)

        def modulate(t, j, n):
            return t * modR[2 * n + 1, 0:1, j * 128:(j + 1) * 128] + modR[2 * n, 0:1, j * 128:(j + 1) * 128]

        def layer_norm(store, load, n, spread):
            prev = None
            for t in range(T // 128):
                halves = []
                for half in range(2):
                    xf = load(half * T + t * 128)
                    if prev is not None:
                        xf = jnp.concatenate([after(xf[0:128], prev), xf[128:D]], axis=0)
                    tiles = []
                    for j, y in enumerate(feature_tiles(normalize(xf))):
                        if spread and j > 0:
                            y = after(y, prev)
                        tiles.append(modulate(y.T, j, n))
                        prev = tiles[-1] if spread else None
                    halves.append(tiles)
                store(slice(t * 64, (t + 1) * 64), *halves)

        def ln1(i, spread):
            layer_norm(functools.partial(store_left, h17.at[i % 2]), lambda r: xT[:, i * TM + r:i * TM + r + 128].astype(F32), 0, spread)

        def ln2(i, spread):
            layer_norm(functools.partial(store_left3, a24.at[i % 2]), lambda r: x1[i % 2, :, r:r + 128], 1, spread)

        partial = {}

        def qkv(i, g, first=0, last=7):
            s0 = i * TM
            sa, sb = QKV_GROUPS[g]
            rows = slice(g * 128, g * 128 + len(sa) * H // 2)
            if i == 0:
                gather = lambda slabs: lambda j: jnp.concatenate(
                    [tmpT[j, pl.ds(part * D + d, H, stride=DH), :] for part, d in slabs], axis=0)
                make_rhs = _right_operands(gather(sa), gather(sb), lo)
            m = partial.setdefault((i, g), {})
            for n in ORDER[first:last]:
                cols = slice(KO[n], KO[n] + KS[n])
                if i == 0:
                    rhs = jnp.concatenate(make_rhs[n](), axis=1).astype(BF)[:, 0:KS[n]]
                    wq17[rows, cols] = _pack(rhs)
                else:
                    rhs = _unpack(wq17[rows, cols])
                m[n] = _dot_nt(_unpack(h17[i % 2, :, cols]), rhs)
            if last < 7:
                return
            c11, c12, c21, c22 = _quadrants(m)
            for half, (ca, cb) in enumerate(((c11, c12), (c21, c22))):
                r = s0 + half * T
                tile = lambda j: (ca if j < 2 else cb)[:, (j % 2) * 128:(j % 2 + 1) * 128]
                for j in range(4):
                    if g == 0:
                        qbuf[j, r:r + T, :] = tile(j) * QSCALE
                    else:
                        (kbuf, vbuf)[g - 1][j, HALO + r:HALO + r + T, :] = tile(j)
                if g == 2:
                    xt = ca[:, 256:384]
                    qbuf[4, r:r + T, :] = jnp.where(lo, xt * QSCALE, 0.0)
                    kbuf[4, HALO + r:HALO + r + T, :] = jnp.where(lo, pltpu.roll(xt, 64, 1), 0.0)
                    vbuf[4, HALO + r:HALO + r + T, :] = cb[:, 256:384]
            if i == 0 and g == 2:
                for j in range(NT):
                    kbuf[j, 0:HALO, :] = jnp.broadcast_to(kbuf[j, HALO:HALO + 1, :], (HALO, 128))
                    vbuf[j, 0:HALO, :] = jnp.broadcast_to(vbuf[j, HALO:HALO + 1, :], (HALO, 128))

        def attend(r0, prev):
            q = qbuf[:, r0:r0 + R, :]
            if prev is not None:
                q = after(q, prev)
            ls = []
            for w in range(W):
                a = HALO + r0 - DIL * w
                p = jnp.sum(q * kbuf[:, a:a + R, :], axis=0)
                p = p + pltpu.roll(p, 64, 1)
                p = p + pltpu.roll(p, 32, 1)
                if r0 < DIL * w:
                    row = lax.broadcasted_iota(jnp.int32, (R, 128), 0) + r0
                    p = jnp.where(row >= DIL * w, p, -1e9 * LOG2E)
                ls.append(p)
            m = functools.reduce(jnp.maximum, ls)
            es = [jnp.exp2(l - m) for l in ls]
            den = functools.reduce(jnp.add, es)
            acc = None
            for w in range(W):
                a = HALO + r0 - DIL * w
                t = es[w][None] * vbuf[:, a:a + R, :]
                acc = t if acc is None else acc + t
            inv = pl.reciprocal(den, approx=True)
            inv = inv * (2.0 - den * inv)
            inv = inv * (2.0 - den * inv)
            return acc * inv[None]

        def attention(i, chained):
            done = []
            for r in range(0, T, 16):
                o = []
                for half in range(2):
                    for r0 in range(r, r + 16, R):
                        done.append(attend(i * TM + half * T + r0, done[-chained] if 0 < chained <= len(done) else None))
                    o.append(jnp.concatenate(done[-(16 // R):], axis=1))
                for n, tiles in enumerate(_right_operands(lambda j: o[0][j], lambda j: o[1][j], lo)):
                    for j, v in enumerate(tiles()):
                        c0 = KO[n] + j * 128
                        o17[r // 2:r // 2 + 8, c0:c0 + 128] = _pack(v.astype(BF))

        def wo_proj(i):
            s0 = i * TM
            m = {}
            for n in ORDER:
                cols = slice(KO[n], KO[n] + KS[n])
                m[n] = _dot_nt(_unpack(wo17[:, cols]), _unpack(o17[:, cols]))
            for n, v in enumerate(_quadrants(m)):
                rows = slice((n // 2) * DHALF, (n // 2 + 1) * DHALF)
                for t in range(T // 128):
                    c0 = (n % 2) * T + t * 128
                    x1[i % 2, rows, c0:c0 + 128] = (xT[rows, s0 + c0:s0 + c0 + 128].astype(F32)
                                                    + gateT[0, rows, :] * v[:, t * 128:(t + 1) * 128])

        def gate_up(i, p):
            fc = 2 * FC // 3
            cs = []
            for w, w24 in ((wg, wg24), (wu, wu24)):
                m = {}
                for n in order3:
                    where = (slice(KO3[n] // 2, (KO3[n] + KS3[n]) // 2), slice(p * fc, (p + 1) * fc))
                    if i > 0:
                        rhs = _unpack(w24[where])
                    else:
                        terms = [[(c, w[r:r + k, (3 * p + j) * fc:(3 * p + j + 1) * fc]) for c, (r, k, j) in right]
                                 for _, right in _parts3(n)]
                        if all(len(t) == 1 for t in terms):
                            rhs = jnp.concatenate([t[0][1] for t in terms], axis=0)
                        else:
                            rhs = jnp.concatenate([_signed_sum([(c, v.astype(F32)) for c, v in t]) for t in terms],
                                                  axis=0).astype(BF)
                        w24[where] = _pack(rhs)
                    m[n] = _dot(_unpack(a24[i % 2, :, KO3[n]:KO3[n] + KS3[n]]), rhs)
                cs.append(_outputs3(m))
            h = [g * u for g, u in zip(*cs)]
            h = [jnp.concatenate(h[3 * half:3 * half + 3], axis=1) for half in range(2)]
            return [v[:, k * FC:(k + 1) * FC] for v in h for k in range(2)]

        h49 = {}

        def stage_hidden(q, h0, h1):
            blocks = [[h[2 * j1 + k2][j2 * 128:(j2 + 1) * 128] for k2 in range(2) for j2 in range(2)]
                      for h in (h0, h1) for j1 in range(2)]
            for n, v in enumerate(_two_levels(_rights, blocks)):
                h49.setdefault(n, []).append(v)

        done = []

        def prep_down(q, dist, slow, fresh=1):
            if fresh:
                done.clear()
            for c in range(0, FC, 128):
                for r in range(0, DQ, 16):
                    outer = [_lefts(*(wdT[i1 * DHALF + i2 * DQ + r:i1 * DHALF + i2 * DQ + r + 16,
                                          (4 * q + 2 * k1 + k2) * FC + c:(4 * q + 2 * k1 + k2) * FC + c + 128].astype(F32)
                                      for i1 in range(2) for k1 in range(2)))
                             for i2 in range(2) for k2 in range(2)]
                    for n in range(7):
                        blocks = [o[n] for o in outer]
                        if len(done) >= dist:
                            blocks[0] = after(blocks[0], done[-dist])
                        where = (slice(r // 2, r // 2 + 8), slice(q * FC + c, q * FC + c + 128))
                        for k, v in enumerate(_lefts(*blocks)):
                            wd49.at[7 * n + k][where] = _pack(v.astype(BF))
                        stored = wd49[(slice(7 * n, 7 * n + 7),) + where]
                        link = functools.reduce(jnp.bitwise_or, [stored[k] for k in range(7)])
                        if slow:
                            link = pltpu.roll(link, 1, 1)
                        link = pltpu.bitcast(link, F32)
                        done.append(jnp.concatenate([link, link], axis=0))

        out_cps = []

        def write_out(i, rows, c0, v):
            s0 = i * TM
            xT[rows, s0 + c0:s0 + c0 + 128] = (x1[i % 2, rows, c0:c0 + 128] + gateT[1, rows, :] * v).astype(BF)

        def hidden_one_level(h):
            return [v.astype(BF) for v in _rights(h[0], h[2], h[1], h[3])]

        def down_one_level(i, p, rights):
            lefts = _lefts(*(wdT[i1 * DHALF:(i1 + 1) * DHALF, (2 * p + k) * FC:(2 * p + k + 1) * FC].astype(F32)
                             for i1 in range(2) for k in range(2)))
            prods = {}
            for products, e in PROGRESSIVE:
                for n in products:
                    part = _dot_nt(lefts[n].astype(BF), rights[n])
                    prods[n] = part if p == 0 else acc7[n] + part
                    if p < nP - 1:
                        acc7[n] = prods[n]
                if p == nP - 1:
                    v = _quadrant(prods, e)
                    for t in range(T // 128):
                        write_out(i, slice((e // 2) * DHALF, (e // 2 + 1) * DHALF), (e % 2) * T + t * 128,
                                  v[:, t * 128:(t + 1) * 128])
            if p == nP - 1:
                out_cps.append(copy_cols(xT, outT_hbm, i * TM, TM))

        def down(i):
            inner = {}
            for products, e1 in PROGRESSIVE:
                for n in products:
                    inner[n] = _quadrants([_dot_nt(_unpack(wd49[7 * n + k]), jnp.concatenate(h49.pop(7 * n + k), axis=1).astype(BF)) for k in range(7)])
                r0, c0 = (e1 // 2) * DHALF, (e1 % 2) * T
                for e2 in range(4):
                    v = _quadrant({n: q[e2] for n, q in inner.items()}, e1)
                    write_out(i, slice(r0 + (e2 // 2) * DQ, r0 + (e2 // 2 + 1) * DQ), c0 + (e2 % 2) * 128, v)
                if i == nb - 1:
                    out_cps.append([start_copy(*(a.at[pl.ds(r0, DHALF), pl.ds(i * TM + c0, T)] for a in (xT, outT_hbm)))])
            if i < nb - 1:
                out_cps.append(copy_cols(xT, outT_hbm, i * TM, TM))

        hidden = {}
        scope = None
        for step in sched + ["scope"]:
            op, *a = step.split()
            if op == "scope":
                if scope is not None:
                    scope.__exit__(None, None, None)
                scope = jax.named_scope(a[0]) if a else None
                if scope is not None:
                    scope.__enter__()
                continue
            if op == "wait":
                for n in a:
                    for cp in pending.pop(n):
                        cp.wait()
                continue
            if op == "waitout":
                for cp in out_cps.pop(0):
                    cp.wait()
                continue
            a = [int(v) for v in a]
            if op == "gu":
                hidden[tuple(a)] = gate_up(*a)
                if a[0] == 0:
                    hidden[tuple(a)] = hidden_one_level(hidden[tuple(a)])
                elif a[1] % 2:
                    stage_hidden(a[1] // 2, hidden.pop((a[0], a[1] - 1)), hidden.pop(tuple(a)))
            elif op == "down1":
                down_one_level(*a, hidden.pop(tuple(a)))
            else:
                {"mod0": prep_mod0, "mod1": prep_mod1, "mod2": prep_mod2, "prep": prep_wqkv, "prepwo": prep_wo,
                 "ln1": ln1, "ln2": ln2, "qkv": qkv, "att": attention, "wo": wo_proj, "down": down, "prepd": prep_down}[op](*a)
        assert not pending
        for cp in sum(out_cps, []):
            cp.wait()

    n_sems = 7 + 3 * nP + 2 * nb + 3
    hbm = pl.BlockSpec(memory_space=pltpu.HBM)

    def fn(A_x, A_wqkv, A_wo, B_x, B_w_gate, B_w_up, B_w_down, c, w_mod):
        del B_x
        outT = pl.pallas_call(
            kernel,
            in_specs=[pl.BlockSpec(memory_space=pltpu.VMEM)] + [hbm] * 7,
            out_specs=hbm,
            out_shape=jax.ShapeDtypeStruct((D, S), BF),
            scratch_shapes=[
                pltpu.VMEM((D, S), BF), pltpu.VMEM((D, 3 * D), BF), pltpu.VMEM((D, D), BF),
                pltpu.VMEM((D, F), BF), pltpu.VMEM((D, F), BF), pltpu.VMEM((D, F), BF),
                pltpu.VMEM((D, 6 * D), BF),
                pltpu.VMEM((NT, 1792, 128), F32), pltpu.VMEM((NT, D, 128), F32), pltpu.VMEM((NT, D, 128), F32),
                pltpu.VMEM((448, KT), I32), pltpu.VMEM((DHALF // 2, KT), I32),
                pltpu.VMEM((4, 8, NT * 128), F32), pltpu.VMEM((2, D, 128), F32),
                pltpu.VMEM((KT3 // 2, F // 3), I32), pltpu.VMEM((KT3 // 2, F // 3), I32),
                pltpu.VMEM((49, DQ // 2, F // 4), I32),
                pltpu.VMEM((NT, S, 128), F32), pltpu.VMEM((NT, HALO + S, 128), F32),
                pltpu.VMEM((NT, HALO + S, 128), F32),
                pltpu.VMEM((2, T // 2, KT), I32), pltpu.VMEM((T // 2, KT), I32),
                pltpu.VMEM((2, D, TM), F32),
                pltpu.VMEM((2, T // 2, KT3), I32),
                pltpu.VMEM((7, DHALF, T), F32),
                pltpu.SemaphoreType.DMA((n_sems,)),
            ],
            compiler_params=pltpu.CompilerParams(vmem_limit_bytes=126 * 2**20, flags=flags),
            name=name,
        )(c, A_x[0].T, A_wqkv, A_wo, B_w_gate, B_w_up, B_w_down.T, w_mod)
        return outT.T[None]

    return fn


SCHEDULE = (
    "wait m0; mod0; wait x0; ln1 0 0; wait qa; prep 0 3; wait qb; prep 3 5; qkv 0 0 0 4; wait k; prep 5 9; "
    "qkv 0 0 4 7; qkv 0 1 0 2; wait v; prep 9 14; qkv 0 1 2 7; wait x1 x2; qkv 0 2; ln1 1 1; qkv 1 0; "
    "qkv 1 1; qkv 1 2; ln1 2 1; qkv 2 0; qkv 2 1; att 0 5; wait wo m1 f0 f1; mod1; prepwo; wo 0; mod2; "
    "qkv 2 2; ln2 0 0; gu 0 0; gu 0 1; down1 0 0; wait f2 f3 f4 f5; gu 0 2; down1 0 1; gu 0 3; down1 0 2; "
    "gu 0 4; down1 0 3; att 1 1; wo 1; gu 0 5; down1 0 4; down1 0 5; ln2 1 1; wait x3; gu 1 0; gu 1 1; "
    "gu 1 2; gu 1 3; gu 1 4; att 2 1; wo 2; gu 1 5; prepd 0 3 1; prepd 1 3 1 0; prepd 2 3 1 0; down 1; "
    "ln2 2 1; waitout; gu 2 0; ln1 3 1; qkv 3 0; qkv 3 1; qkv 3 2; gu 2 1; gu 2 2; gu 2 3; gu 2 4; "
    "att 3 1; wo 3; gu 2 5; down 2; ln2 3 1; gu 3 0; gu 3 1; gu 3 2; gu 3 3; gu 3 4; gu 3 5; down 3; "
)
DMA = "m0 x0 qa qb k v x1 x2 wo m1 f0 f1 f2 f3 f4 f5 x3"


@jax.jit
def pallas_adaLN_cond__sliding_local_dilated__glu_gated_bilinear__prompt_kernel(
    A_x: jax.Array,
    A_wqkv: jax.Array,
    A_wo: jax.Array,
    B_x: jax.Array,
    B_w_gate: jax.Array,
    B_w_up: jax.Array,
    B_w_down: jax.Array,
    c: jax.Array,
    w_mod: jax.Array,
):
    return make(sched=SCHEDULE, dma=DMA)(A_x, A_wqkv, A_wo, B_x, B_w_gate, B_w_up, B_w_down, c, w_mod)
```

```python
import contextlib
import functools

import jax
import jax.numpy as jnp
from jax import lax
import jax.experimental.pallas as pl
import jax.experimental.pallas.tpu as pltpu

S, D, H, DH, W, DIL, F = 2048, 576, 32, 18, 8, 2, 4608
HALO = 16
NT = 5
DHALF = D // 2
DQ = D // 4
EPS = 1e-5
LOG2E = 1.4426950408889634
QSCALE = DH ** -0.5 * LOG2E
BF, F32, I32 = jnp.bfloat16, jnp.float32, jnp.int32
NT_DIMS = (((1,), (1,)), ((), ()))


def _tw(j):
    return min(128, D - 128 * j)


def _dot(a, b):
    return jnp.dot(a, b, preferred_element_type=F32)


def _dot_nt(a, b):
    return lax.dot_general(a, b, NT_DIMS, preferred_element_type=F32)


def _pack(v):
    return pltpu.bitcast(v, jnp.int32)


def _unpack(v):
    return pltpu.bitcast(v, BF)


def _colsum(x):
    return jnp.sum(jnp.sum(x.reshape(D // 32, 32, 128), axis=0), axis=0, keepdims=True)


KS = (256, 256, 384, 384, 192, 384, 256)
KO = (0, 256, 512, 896, 1280, 1536, 1920)
KT = 2176
LEFT3 = (
    ((0, 1, 0), (0, 0, 0)), ((0, 0, -1), (0, 0, 0)), ((-1, 0, 1), (0, 0, 0)), ((-1, 1, 0), (0, 0, 0)),
    ((0, -1, 0), (0, 1, 0)), ((0, 0, 0), (0, 0, -1)), ((0, -1, 1), (0, 1, -1)), ((0, -1, 0), (0, 1, -1)),
    ((0, 0, 0), (0, 1, -1)), ((1, 0, -1), (-1, 0, 1)), ((1, 0, 0), (-1, 0, 0)), ((1, 0, -1), (-1, 0, 0)),
    ((0, 0, 0), (-1, 0, 0)), ((0, 1, 0), (-1, 0, 0)), ((0, 0, 0), (-1, 1, 0)))
RIGHT3 = (
    ((0, -1, 0), (0, -1, 1), (0, 0, 0)), ((0, 0, -1), (0, 0, 0), (0, 1, -1)), ((0, 0, -1), (0, 0, 0), (0, 0, 0)),
    ((0, 1, 0), (0, 0, 0), (0, 0, 0)), ((0, 0, 0), (1, -1, 0), (0, -1, 0)), ((0, 0, 0), (0, 0, 1), (1, 0, 1)),
    ((0, 0, 0), (0, 0, 0), (0, 1, 0)), ((0, 0, 0), (0, 0, 1), (0, 1, 0)), ((0, 0, 0), (0, 0, 1), (0, 0, 0)),
    ((0, 0, 0), (0, 0, 0), (1, 0, 0)), ((1, -1, 0), (0, 0, 0), (1, 0, 0)), ((0, 0, -1), (0, 0, 0), (1, 0, 0)),
    ((-1, 0, -1), (-1, 0, 0), (0, 0, 0)), ((0, -1, 0), (-1, 0, 0), (0, 0, 0)), ((0, 0, 0), (-1, 0, 0), (0, 0, 0)))
EXTRA3 = (
    {1: ((1, 0), (0, 0, 1)), 3: ((1, 0), (0, -1, 0)), 4: ((1, -1), (-1, 1, 0)),
     5: ((0, 1), (0, 0, -1)), 13: ((1, 0), (-1, 1, 0)), 14: ((0, 1), (-1, 0, 0))},
    {1: ((1, 0), (0, -1, 1)), 4: ((0, 1), (0, -1, 0)), 5: ((0, 1), (-1, 0, -1)),
     6: ((1, 0), (0, 1, 0)), 9: ((0, 1), (1, 0, 0)), 10: ((1, 0), (1, 0, 0))},
    {3: ((1, 0), (0, -1, 1)), 6: ((1, 0), (0, 0, 1)), 9: ((0, 1), (0, 0, -1)),
     10: ((1, -1), (1, -1, 1)), 13: ((0, 1), (-1, 1, -1)), 14: ((0, 1), (-1, 0, -1))})
SLICES3 = tuple({(1, 2): (2, 1)}.get(s, s) for s in (tuple(k for k in range(3) if n in EXTRA3[k]) for n in range(15)))
KS3 = tuple(128 + 64 * len(s) for s in SLICES3)
KO3 = tuple(sum(KS3[:n]) for n in range(15))
KT3 = sum(KS3)
ORDER3 = (2, 11, 9, 12, 14, 8, 5, 7, 0, 3, 6, 1, 13, 10, 4)


def _outputs3(m):
    a, b = m[2] + m[11], m[7] - m[8]
    c, d = m[0] + b, m[9] - a
    return (m[12] - a - m[3] - m[13] + m[10], m[6] - (c + m[3]), m[2] - b + m[6] + m[1],
            m[12] + d - m[14], m[13] - (m[14] + c) - m[4], m[8] - d - m[5])


def _parts3(n):
    parts = [([(c, (i, k)) for i in range(2) for k, c in enumerate(LEFT3[n][i]) if c],
              [(c, (128 * k, 128, j)) for k in range(3) for j, c in enumerate(RIGHT3[n][k]) if c])]
    for s in SLICES3[n]:
        left, right = EXTRA3[s][n]
        parts.append(([(c, (i, 4 if s == 2 else 3)) for i, c in enumerate(left) if c],
                      [(c, (384 + 64 * s, 64, j)) for j, c in enumerate(right) if c]))
    return [([(c * r[0][0], x) for c, x in l], [(c * r[0][0], x) for c, x in r]) for l, r in parts]


def _signed_sum(terms):
    terms = sorted(terms, key=lambda t: -t[0])
    total = terms[0][1] if terms[0][0] > 0 else -terms[0][1]
    for c, v in terms[1:]:
        total = total + v if c > 0 else total - v
    return total


def _left_operands(p, q, lo):
    d = [y - x for x, y in zip(p, q)]
    w = lambda a, b: jnp.where(lo, a, b)
    return (
        (p[0] + q[1], w(p[2] + q[3], p[2] - q[2])),
        (q[0] + q[1], w(q[2] + q[3], d[3])),
        (p[0], p[2], w(p[4], p[3])),
        (q[1], w(q[3], p[3]), w(q[4], q[2])),
        (p[0] + p[1], p[2] + p[3]),
        (d[0], d[2], w(d[4], d[3])),
        (d[1], w(d[3], d[4])),
    )


def _right_operands(a, b, lo):
    w = lambda x, y: jnp.where(lo, x, y)
    return (
        lambda: (a(0) + b(1), w(a(2) + b(3), a(2))),
        lambda: (a(0), w(a(2), a(3))),
        lambda: (b(0) - b(1), w(b(2) - b(3), b(2)), w(b(4), b(3))),
        lambda: (a(1) - a(0), w(a(3) - a(2), a(3)), w(a(4), a(2))),
        lambda: (b(1), b(3)),
        lambda: (a(0) + b(0), a(2) + b(2), w(b(4), a(3) + b(3))),
        lambda: (a(1) + b(1), w(a(3) + b(3), a(4))),
    )


def _quadrant(m, e):
    return (lambda: m[0] - m[4] + m[3] - m[6], lambda: m[4] + m[2],
            lambda: m[1] + m[3], lambda: m[0] - m[1] + m[2] + m[5])[e]()


def _quadrants(m):
    return [_quadrant(m, e) for e in range(4)]


def _lefts(a11, a12, a21, a22):
    return a11 + a22, a21 + a22, a11, a22, a11 + a12, a21 - a11, a22 - a12


def _rights(b11, b12, b21, b22):
    return b11 + b22, b11, b12 - b22, b21 - b11, b22, b11 + b12, b21 + b22


def _two_levels(combos, blocks):
    outer = [combos(*(blocks[e1][e2] for e1 in range(4))) for e2 in range(4)]
    return [v for n in range(7) for v in combos(*(outer[e2][n] for e2 in range(4)))]


ORDER = (1, 4, 0, 2, 3, 5, 6)
PROGRESSIVE = (((4, 2), 1), ((1, 3), 2), ((0, 5), 3), ((6,), 0))
_slabs = lambda part, lo, hi: [(part, d) for d in range(lo, hi)]
QKV_GROUPS = (
    (_slabs(0, 0, 8), _slabs(0, 8, 16)),
    (_slabs(1, 0, 8), _slabs(1, 8, 16)),
    (_slabs(2, 0, 8) + _slabs(0, 16, 18) + _slabs(1, 16, 18), _slabs(2, 8, 16) + _slabs(2, 16, 18) * 2),
)


DMA_ORDER = "m0 x0 q k v x1 wo m1 f0 f1 f2 f3 f4 f5 x2 x3"


def make(order3=ORDER3, inner_order=(4, 2, 1, 3, 0, 5, 6), TM=512, FC=384, R=8, sched=None, dma=DMA_ORDER, flags=None, nocheck=False, name="k16"):
    nb = S // TM
    T = TM // 2
    nP = F // (2 * FC)
    if isinstance(sched, str):
        sched = [t.strip() for t in sched.split(";") if t.strip()]
    dma = dma.split()

    def kernel(c_hbm, xT_hbm, wqkv_hbm, wo_hbm, wg_hbm, wu_hbm, wdT_hbm, wmod_hbm, outT_hbm,
               c_ref, xT, wqkv, wo, wg, wu, wdT, wmod, tmpT, tmpW, woT, wq17, wo17, modR, gateT, wg24, wu24, wd49,
               qbuf, kbuf, vbuf, h17, o17, x1, a24, acc7, sems):

        def start_copy(src, dst, sem):
            cp = pltpu.make_async_copy(src, dst, sems.at[sem])
            cp.start()
            return cp

        def copy_cols(sem, src, dst, c0, n):
            return start_copy(src.at[:, pl.ds(c0, n)], dst.at[:, pl.ds(c0, n)], sem)

        ffn = ((wg_hbm, wg), (wu_hbm, wu), (wdT_hbm, wdT))
        pieces = {"m0": [(c_hbm, c_ref, 0, D), (wmod_hbm, wmod, 0, 2 * D)],
                  "qa": [(wqkv_hbm, wqkv, 0, 384)], "qb": [(wqkv_hbm, wqkv, 384, 256)],
                  "k": [(wqkv_hbm, wqkv, 640, 512)], "v": [(wqkv_hbm, wqkv, 1152, D)],
                  "x0": [(xT_hbm, xT, 0, TM)], "x12": [(xT_hbm, xT, TM, 2 * TM)], "x3": [(xT_hbm, xT, 3 * TM, TM)],
                  "f01": [(wo_hbm, wo, 0, D), (wmod_hbm, wmod, 2 * D, 4 * D)] + [(a, b, 0, 4 * FC) for a, b in ffn],
                  "f25": [(a, b, 4 * FC, F - 4 * FC) for a, b in ffn]}
        assert sorted(dma) == sorted(pieces)
        pending = {n: [copy_cols(sem, *a) for a in pieces[n]] for sem, n in enumerate(dma)}
        masks = []

        def after(x, prev):
            if not masks:
                bits = pltpu.bitcast(jnp.broadcast_to(c_ref[:, 0:128].astype(F32), (8, 128)), jnp.int32)
                masks.append(((bits * bits) & 2) == 0)
            k = jnp.broadcast_to(masks[0][0:1], x.shape[-2:])
            return jnp.where(k, x, prev)

        lane = lax.broadcasted_iota(jnp.int32, (1, 128), 1)
        lo = lane < 64

        def feature_tiles(y):
            return [y[j * 128:(j + 1) * 128] for j in range(4)] + [jnp.concatenate([y[512:D], y[512:D]], axis=0)]

        def store_left(dst, rows, p, q):
            for n, tiles in enumerate(_left_operands(p, q, lo)):
                for j, v in enumerate(tiles):
                    c0 = KO[n] + j * 128
                    dst[rows, c0:c0 + 128] = _pack(v.astype(BF))

        def store_left3(dst, rows, *groups):
            for n in range(15):
                parts = [_signed_sum([(c, groups[i][k]) for c, (i, k) in left]) for left, _ in _parts3(n)]
                tiles = parts[:1] + ([jnp.where(lo, *parts[1:])] if len(parts) > 1 else [])
                for j, v in enumerate(tiles):
                    dst[rows, KO3[n] + j * 128:KO3[n] + (j + 1) * 128] = _pack(v.astype(BF))

        def prep_wqkv(first, last):
            for cb in range(first, last):
                cw = min(128, 3 * D - cb * 128)
                for j, t in enumerate(feature_tiles(wqkv[:, cb * 128:cb * 128 + cw].astype(F32))):
                    tmpT[j, cb * 128:cb * 128 + cw, :] = t.T

        def prep_wo():
            for j in range(NT):
                tmpW[j, :, 0:_tw(j)] = wo[:, j * 128:j * 128 + _tw(j)].astype(F32)
            for j in range(NT):
                p = jnp.concatenate([tmpW[j, pl.ds(d, H, stride=DH), :] for d in range(DH)], axis=0)
                for n, t in enumerate(feature_tiles(p[:, 0:_tw(j)])):
                    woT[n, j * 128:j * 128 + _tw(j), :] = t.T
            store_left(wo17, slice(None), [woT[n, 0:DHALF, :] for n in range(NT)], [woT[n, DHALF:D, :] for n in range(NT)])

        def modulation(c0, n):
            cf = c_ref[...].astype(F32)
            s = (cf * jax.nn.sigmoid(cf)).astype(BF)
            return _dot(jnp.broadcast_to(s, (16, D)), wmod[:, c0:c0 + n])[0:8]

        def to_column(row, n):
            for j in range(NT):
                r = row[0:1, j * 128:j * 128 + _tw(j)]
                gateT[n, j * 128:j * 128 + _tw(j), :] = jnp.broadcast_to(r, (128, _tw(j))).T

        def widen(row):
            return jnp.concatenate([row, row[:, 512:D]], axis=1)

        def prep_mod0():
            m = modulation(0, 2 * D)
            modR[0] = widen(m[:, 0:D])
            modR[1] = widen(1.0 + m[:, D:2 * D])

        def prep_mod1():
            to_column(modulation(2 * D, 640)[:, 0:D], 0)

        def prep_mod2():
            m = modulation(3 * D - 64, 3 * D + 64)
            modR[2] = widen(m[:, 64:64 + D])
            modR[3] = widen(1.0 + m[:, 64 + D:64 + 2 * D])
            to_column(m[:, 64 + 2 * D:64 + 3 * D], 1)

        def normalize(xf):
            mean = _colsum(xf) * (1.0 / D)
            xc = xf - mean
            var = _colsum(xc * xc) * (1.0 / D)
            return xc * lax.rsqrt(var + EPS)

        def modulate(t, j, n):
            return t * modR[2 * n + 1, 0:1, j * 128:(j + 1) * 128] + modR[2 * n, 0:1, j * 128:(j + 1) * 128]

        def layer_norm(store, load, n, spread):
            prev = None
            for t in range(T // 128):
                halves = []
                for half in range(2):
                    xf = load(half * T + t * 128)
                    if prev is not None:
                        xf = jnp.concatenate([after(xf[0:128], prev), xf[128:D]], axis=0)
                    tiles = []
                    for j, y in enumerate(feature_tiles(normalize(xf))):
                        if spread and j > 0:
                            y = after(y, prev)
                        tiles.append(modulate(y.T, j, n))
                        prev = delayed(tiles[-1], spread - 1) if spread else None
                    halves.append(tiles)
                store(slice(t * 64, (t + 1) * 64), *halves)

        def ln1(i, spread):
            layer_norm(functools.partial(store_left, h17.at[i % 2]), lambda r: xT[:, i * TM + r:i * TM + r + 128].astype(F32), 0, spread)

        def ln2(i, spread):
            layer_norm(functools.partial(store_left3, a24.at[i % 2]), lambda r: x1[i % 2, :, r:r + 128], 1, spread)

        partial = {}

        def qkv(i, g, first=0, last=7):
            s0 = i * TM
            sa, sb = QKV_GROUPS[g]
            rows = slice(g * 128, g * 128 + len(sa) * H // 2)
            if i == 0:
                gather = lambda slabs: lambda j: jnp.concatenate(
                    [tmpT[j, pl.ds(part * D + d, H, stride=DH), :] for part, d in slabs], axis=0)
                make_rhs = _right_operands(gather(sa), gather(sb), lo)
            m = partial.setdefault((i, g), {})
            for n in ORDER[first:last]:
                cols = slice(KO[n], KO[n] + KS[n])
                if i == 0:
                    rhs = jnp.concatenate(make_rhs[n](), axis=1).astype(BF)[:, 0:KS[n]]
                    wq17[rows, cols] = _pack(rhs)
                else:
                    rhs = _unpack(wq17[rows, cols])
                m[n] = _dot_nt(_unpack(h17[i % 2, :, cols]), rhs)
            if last < 7:
                return
            c11, c12, c21, c22 = _quadrants(m)
            for half, (ca, cb) in enumerate(((c11, c12), (c21, c22))):
                r = s0 + half * T
                tile = lambda j: (ca if j < 2 else cb)[:, (j % 2) * 128:(j % 2 + 1) * 128]
                for j in range(4):
                    if g == 0:
                        qbuf[j, r:r + T, :] = tile(j) * QSCALE
                    else:
                        (kbuf, vbuf)[g - 1][j, HALO + r:HALO + r + T, :] = tile(j)
                if g == 2:
                    xt = ca[:, 256:384]
                    qbuf[4, r:r + T, :] = jnp.where(lo, xt * QSCALE, 0.0)
                    kbuf[4, HALO + r:HALO + r + T, :] = jnp.where(lo, pltpu.roll(xt, 64, 1), 0.0)
                    vbuf[4, HALO + r:HALO + r + T, :] = cb[:, 256:384]
            if i == 0 and g == 2:
                for j in range(NT):
                    kbuf[j, 0:HALO, :] = jnp.broadcast_to(kbuf[j, HALO:HALO + 1, :], (HALO, 128))
                    vbuf[j, 0:HALO, :] = jnp.broadcast_to(vbuf[j, HALO:HALO + 1, :], (HALO, 128))

        def attend(r0, prev):
            q = qbuf[:, r0:r0 + R, :]
            if prev is not None:
                q = after(q, prev)
            ls = []
            for w in range(W):
                a = HALO + r0 - DIL * w
                p = jnp.sum(q * kbuf[:, a:a + R, :], axis=0)
                p = p + pltpu.roll(p, 64, 1)
                p = p + pltpu.roll(p, 32, 1)
                if r0 < DIL * w:
                    row = lax.broadcasted_iota(jnp.int32, (R, 128), 0) + r0
                    p = jnp.where(row >= DIL * w, p, -1e9 * LOG2E)
                ls.append(p)
            m = functools.reduce(jnp.maximum, ls)
            es = [jnp.exp2(l - m) for l in ls]
            den = functools.reduce(jnp.add, es)
            acc = None
            for w in range(W):
                a = HALO + r0 - DIL * w
                t = es[w][None] * vbuf[:, a:a + R, :]
                acc = t if acc is None else acc + t
            inv = pl.reciprocal(den, approx=True)
            inv = inv * (2.0 - den * inv)
            inv = inv * (2.0 - den * inv)
            return acc * inv[None]

        def delayed(v, n):
            head = v[..., 0:8, :]
            for _ in range(n):
                head = pltpu.roll(head, 1, head.ndim - 1)
            return jnp.concatenate([head, v[..., 8:, :]], axis=-2) if v.shape[-2] > 8 else head

        def attention(i, chained, slow=0):
            done = []
            for r in range(0, T, 16):
                o = []
                for half in range(2):
                    for r0 in range(r, r + 16, R):
                        prev = done[-chained] if 0 < chained <= len(done) else None
                        if prev is not None and slow:
                            prev = jnp.concatenate([delayed(prev[0:1], slow), prev[1:]], axis=0)
                        done.append(attend(i * TM + half * T + r0, prev))
                    o.append(jnp.concatenate(done[-(16 // R):], axis=1))
                for n, tiles in enumerate(_right_operands(lambda j: o[0][j], lambda j: o[1][j], lo)):
                    for j, v in enumerate(tiles()):
                        c0 = KO[n] + j * 128
                        o17[r // 2:r // 2 + 8, c0:c0 + 128] = _pack(v.astype(BF))

        def wo_proj(i):
            s0 = i * TM
            m = {}
            for n in ORDER:
                cols = slice(KO[n], KO[n] + KS[n])
                m[n] = _dot_nt(_unpack(wo17[:, cols]), _unpack(o17[:, cols]))
            for n, v in enumerate(_quadrants(m)):
                rows = slice((n // 2) * DHALF, (n // 2 + 1) * DHALF)
                for t in range(T // 128):
                    c0 = (n % 2) * T + t * 128
                    x1[i % 2, rows, c0:c0 + 128] = (xT[rows, s0 + c0:s0 + c0 + 128].astype(F32)
                                                    + gateT[0, rows, :] * v[:, t * 128:(t + 1) * 128])

        def gate_up(i, p):
            fc = 2 * FC // 3
            cs = []
            for w, w24 in ((wg, wg24), (wu, wu24)):
                m = {}
                for n in order3:
                    where = (slice(KO3[n] // 2, (KO3[n] + KS3[n]) // 2), slice(p * fc, (p + 1) * fc))
                    if i > 0:
                        rhs = _unpack(w24[where])
                    else:
                        terms = [[(c, w[r:r + k, (3 * p + j) * fc:(3 * p + j + 1) * fc]) for c, (r, k, j) in right]
                                 for _, right in _parts3(n)]
                        if all(len(t) == 1 for t in terms):
                            rhs = jnp.concatenate([t[0][1] for t in terms], axis=0)
                        else:
                            rhs = jnp.concatenate([_signed_sum([(c, v.astype(F32)) for c, v in t]) for t in terms],
                                                  axis=0).astype(BF)
                        w24[where] = _pack(rhs)
                    m[n] = _dot(_unpack(a24[i % 2, :, KO3[n]:KO3[n] + KS3[n]]), rhs)
                cs.append(_outputs3(m))
            h = [g * u for g, u in zip(*cs)]
            h = [jnp.concatenate(h[3 * half:3 * half + 3], axis=1) for half in range(2)]
            return [v[:, k * FC:(k + 1) * FC] for v in h for k in range(2)]

        h49 = {}

        def stage_hidden(q, h0, h1):
            blocks = [[h[2 * j1 + k2][j2 * 128:(j2 + 1) * 128] for k2 in range(2) for j2 in range(2)]
                      for h in (h0, h1) for j1 in range(2)]
            for n, v in enumerate(_two_levels(_rights, blocks)):
                h49.setdefault(n, []).append(v)

        done = []

        def prep_down(q, dist, slow, fresh=1):
            if fresh:
                done.clear()
            for c in range(0, FC, 128):
                for r in range(0, DQ, 16):
                    outer = [_lefts(*(wdT[i1 * DHALF + i2 * DQ + r:i1 * DHALF + i2 * DQ + r + 16,
                                          (4 * q + 2 * k1 + k2) * FC + c:(4 * q + 2 * k1 + k2) * FC + c + 128].astype(F32)
                                      for i1 in range(2) for k1 in range(2)))
                             for i2 in range(2) for k2 in range(2)]
                    for n in range(7):
                        blocks = [o[n] for o in outer]
                        if len(done) >= dist:
                            blocks[0] = after(blocks[0], done[-dist])
                        where = (slice(r // 2, r // 2 + 8), slice(q * FC + c, q * FC + c + 128))
                        for k, v in enumerate(_lefts(*blocks)):
                            wd49.at[7 * n + k][where] = _pack(v.astype(BF))
                        stored = wd49[(slice(7 * n, 7 * n + 7),) + where]
                        link = functools.reduce(jnp.bitwise_or, [stored[k] for k in range(7)])
                        if slow:
                            link = pltpu.roll(link, 1, 1)
                        link = pltpu.bitcast(link, F32)
                        done.append(jnp.concatenate([link, link], axis=0))

        out_cps = []

        def write_out(i, rows, c0, v):
            s0 = i * TM
            xT[rows, s0 + c0:s0 + c0 + 128] = (x1[i % 2, rows, c0:c0 + 128] + gateT[1, rows, :] * v).astype(BF)

        def hidden_one_level(h):
            return [v.astype(BF) for v in _rights(h[0], h[2], h[1], h[3])]

        def down_one_level(i, p, rights):
            lefts = _lefts(*(wdT[i1 * DHALF:(i1 + 1) * DHALF, (2 * p + k) * FC:(2 * p + k + 1) * FC].astype(F32)
                             for i1 in range(2) for k in range(2)))
            prods = {}
            for products, e in PROGRESSIVE:
                for n in products:
                    part = _dot_nt(lefts[n].astype(BF), rights[n])
                    prods[n] = part if p == 0 else acc7[n] + part
                    if p < nP - 1:
                        acc7[n] = prods[n]
                if p == nP - 1:
                    v = _quadrant(prods, e)
                    for t in range(T // 128):
                        write_out(i, slice((e // 2) * DHALF, (e // 2 + 1) * DHALF), (e % 2) * T + t * 128,
                                  v[:, t * 128:(t + 1) * 128])
            if p == nP - 1:
                out_cps.append([copy_cols(i, xT, outT_hbm, i * TM, TM)])

        def down(i):
            inner = {}
            for products, e1 in PROGRESSIVE:
                for n in products:
                    inner[n] = _quadrants({k: _dot_nt(_unpack(wd49[7 * n + k]), jnp.concatenate(h49.pop(7 * n + k), axis=1).astype(BF))
                                           for k in inner_order})
                r0, c0 = (e1 // 2) * DHALF, (e1 % 2) * T
                for e2 in range(4):
                    v = _quadrant({n: q[e2] for n, q in inner.items()}, e1)
                    write_out(i, slice(r0 + (e2 // 2) * DQ, r0 + (e2 // 2 + 1) * DQ), c0 + (e2 % 2) * 128, v)
                if i == nb - 1:
                    out_cps.append([start_copy(*(a.at[pl.ds(r0, DHALF), pl.ds(i * TM + c0, T)] for a in (xT, outT_hbm)), i)])
            if i < nb - 1:
                out_cps.append([copy_cols(i, xT, outT_hbm, i * TM, TM)])

        hidden = {}
        scope = None
        for step in sched + ["scope"]:
            op, *a = step.split()
            if op == "scope":
                if scope is not None:
                    scope.__exit__(None, None, None)
                scope = jax.named_scope(a[0]) if a else None
                if scope is not None:
                    scope.__enter__()
                continue
            if op == "wait":
                for n in a:
                    for cp in pending.pop(n):
                        cp.wait()
                continue
            if op == "waitout":
                for cp in out_cps.pop(0):
                    cp.wait()
                continue
            a = [int(v) for v in a]
            if op == "gu":
                hidden[tuple(a)] = gate_up(*a)
                if a[0] == 0:
                    hidden[tuple(a)] = hidden_one_level(hidden[tuple(a)])
                elif a[1] % 2:
                    stage_hidden(a[1] // 2, hidden.pop((a[0], a[1] - 1)), hidden.pop(tuple(a)))
            elif op == "down1":
                down_one_level(*a, hidden.pop(tuple(a)))
            else:
                {"mod0": prep_mod0, "mod1": prep_mod1, "mod2": prep_mod2, "prep": prep_wqkv, "prepwo": prep_wo,
                 "ln1": ln1, "ln2": ln2, "qkv": qkv, "att": attention, "wo": wo_proj, "down": down, "prepd": prep_down}[op](*a)
        assert not pending
        for cp in sum(out_cps, []):
            cp.wait()

    n_sems = len(dma)
    hbm = pl.BlockSpec(memory_space=pltpu.HBM)

    def fn(A_x, A_wqkv, A_wo, B_x, B_w_gate, B_w_up, B_w_down, c, w_mod):
        del B_x
        outT = pl.pallas_call(
            kernel,
            in_specs=[hbm] * 8,
            out_specs=hbm,
            out_shape=jax.ShapeDtypeStruct((D, S), BF),
            scratch_shapes=[
                pltpu.VMEM((1, D), BF), pltpu.VMEM((D, S), BF), pltpu.VMEM((D, 3 * D), BF), pltpu.VMEM((D, D), BF),
                pltpu.VMEM((D, F), BF), pltpu.VMEM((D, F), BF), pltpu.VMEM((D, F), BF),
                pltpu.VMEM((D, 6 * D), BF),
                pltpu.VMEM((NT, 1792, 128), F32), pltpu.VMEM((NT, D, 128), F32), pltpu.VMEM((NT, D, 128), F32),
                pltpu.VMEM((448, KT), I32), pltpu.VMEM((DHALF // 2, KT), I32),
                pltpu.VMEM((4, 8, NT * 128), F32), pltpu.VMEM((2, D, 128), F32),
                pltpu.VMEM((KT3 // 2, F // 3), I32), pltpu.VMEM((KT3 // 2, F // 3), I32),
                pltpu.VMEM((49, DQ // 2, F // 4), I32),
                pltpu.VMEM((NT, S, 128), F32), pltpu.VMEM((NT, HALO + S, 128), F32),
                pltpu.VMEM((NT, HALO + S, 128), F32),
                pltpu.VMEM((2, T // 2, KT), I32), pltpu.VMEM((T // 2, KT), I32),
                pltpu.VMEM((2, D, TM), F32),
                pltpu.VMEM((2, T // 2, KT3), I32),
                pltpu.VMEM((7, DHALF, T), F32),
                pltpu.SemaphoreType.DMA((n_sems,)),
            ],
            compiler_params=pltpu.CompilerParams(vmem_limit_bytes=126 * 2**20, flags=flags, disable_semaphore_checks=nocheck),
            name=name,
        )(c, A_x[0].T, A_wqkv, A_wo, B_w_gate, B_w_up, B_w_down.T, w_mod)
        return outT.T[None]

    return fn


SCHEDULE = (
    "wait m0; mod0; wait x0; ln1 0 0; wait qa; prep 0 3; wait qb; prep 3 5; qkv 0 0 0 4; wait k; prep 5 9; "
    "qkv 0 0 4 7; qkv 0 1 0 2; wait v; prep 9 14; qkv 0 1 2 7; wait x12; qkv 0 2; ln1 1 0; qkv 1 0; "
    "qkv 1 1; qkv 1 2; ln1 2 1; qkv 2 0; qkv 2 1; att 0 4 1; wait f01; mod1; prepwo; wo 0; mod2; qkv 2 2; "
    "ln2 0 0; gu 0 0; gu 0 1; down1 0 0; wait f25; gu 0 2; down1 0 1; gu 0 3; down1 0 2; gu 0 4; "
    "down1 0 3; att 1 2 1; wo 1; gu 0 5; down1 0 4; down1 0 5; ln2 1 1; wait x3; gu 1 0; gu 1 1; gu 1 2; "
    "gu 1 3; gu 1 4; att 2 1; wo 2; gu 1 5; prepd 0 3 1; prepd 1 3 1 0; prepd 2 3 1 0; down 1; ln2 2 1; "
    "waitout; gu 2 0; ln1 3 1; qkv 3 0; qkv 3 1; qkv 3 2; gu 2 1; gu 2 2; gu 2 3; gu 2 4; att 3 1; wo 3; "
    "gu 2 5; down 2; ln2 3 1; gu 3 0; gu 3 1; gu 3 2; gu 3 3; gu 3 4; gu 3 5; down 3; "
)
DMA = "m0 x0 qa qb k v x12 f01 f25 x3"


@jax.jit
def pallas_adaLN_cond__sliding_local_dilated__glu_gated_bilinear__prompt_kernel(
    A_x: jax.Array,
    A_wqkv: jax.Array,
    A_wo: jax.Array,
    B_x: jax.Array,
    B_w_gate: jax.Array,
    B_w_up: jax.Array,
    B_w_down: jax.Array,
    c: jax.Array,
    w_mod: jax.Array,
):
    return make(sched=SCHEDULE, dma=DMA)(A_x, A_wqkv, A_wo, B_x, B_w_gate, B_w_up, B_w_down, c, w_mod)
```

```python
import functools

import jax
import jax.numpy as jnp
from jax import lax
import jax.experimental.pallas as pl
import jax.experimental.pallas.tpu as pltpu

S, D, F = 2048, 576, 4608
H, DH, W, DIL = 32, 18, 8, 2
EPS = 1e-5
LOG2E = 1.4426950408889634
QSCALE = DH ** -0.5 * LOG2E
MASKED = -1e9 * LOG2E

TM = 512
T = TM // 2
NB = S // TM
FC = 384
NP = F // (2 * FC)
NT = 5
D2, D4 = D // 2, D // 4
HALO = 16

BF, F32, I32 = jnp.bfloat16, jnp.float32, jnp.int32


def _dot(a, b):
    return jnp.dot(a, b, preferred_element_type=F32)


def _dot_nt(a, b):
    return lax.dot_general(a, b, (((1,), (1,)), ((), ())), preferred_element_type=F32)


def _pack(v):
    return pltpu.bitcast(v.astype(BF), I32)


def _unpack(v):
    return pltpu.bitcast(v, BF)


def _width(j):
    return min(128, D - 128 * j)


def _feature_tiles(y):
    return [y[j * 128:(j + 1) * 128] for j in range(4)] + [jnp.concatenate([y[512:D], y[512:D]], axis=0)]


def _normalize(x):
    colsum = lambda v: jnp.sum(jnp.sum(v.reshape(D // 32, 32, 128), axis=0), axis=0, keepdims=True)
    xc = x - colsum(x) * (1.0 / D)
    return xc * lax.rsqrt(colsum(xc * xc) * (1.0 / D) + EPS)


def _lefts(a11, a12, a21, a22):
    return a11 + a22, a21 + a22, a11, a22, a11 + a12, a21 - a11, a22 - a12


def _rights(b11, b12, b21, b22):
    return b11 + b22, b11, b12 - b22, b21 - b11, b22, b11 + b12, b21 + b22


def _quadrant(m, e):
    return (lambda: m[0] - m[4] + m[3] - m[6], lambda: m[4] + m[2],
            lambda: m[1] + m[3], lambda: m[0] - m[1] + m[2] + m[5])[e]()


def _quadrants(m):
    return [_quadrant(m, e) for e in range(4)]


ORDER2 = (1, 4, 0, 2, 3, 5, 6)
PROGRESSIVE = (((4, 2), 1), ((1, 3), 2), ((0, 5), 3), ((6,), 0))

KS2 = (256, 256, 384, 384, 192, 384, 256)
KO2 = (0, 256, 512, 896, 1280, 1536, 1920)
KT2 = 2176


def _left_tiles(p, q, lo):
    d = [y - x for x, y in zip(p, q)]
    w = lambda a, b: jnp.where(lo, a, b)
    return (
        (p[0] + q[1], w(p[2] + q[3], p[2] - q[2])),
        (q[0] + q[1], w(q[2] + q[3], d[3])),
        (p[0], p[2], w(p[4], p[3])),
        (q[1], w(q[3], p[3]), w(q[4], q[2])),
        (p[0] + p[1], p[2] + p[3]),
        (d[0], d[2], w(d[4], d[3])),
        (d[1], w(d[3], d[4])),
    )


def _right_tiles(n, a, b, lo):
    w = lambda x, y: jnp.where(lo, x, y)
    return (
        lambda: (a(0) + b(1), w(a(2) + b(3), a(2))),
        lambda: (a(0), w(a(2), a(3))),
        lambda: (b(0) - b(1), w(b(2) - b(3), b(2)), w(b(4), b(3))),
        lambda: (a(1) - a(0), w(a(3) - a(2), a(3)), w(a(4), a(2))),
        lambda: (b(1), b(3)),
        lambda: (a(0) + b(0), a(2) + b(2), w(b(4), a(3) + b(3))),
        lambda: (a(1) + b(1), w(a(3) + b(3), a(4))),
    )[n]()


def _slabs(part, start, stop):
    return [(part, d) for d in range(start, stop)]


QKV_GROUPS = (
    (_slabs(0, 0, 8), _slabs(0, 8, 16)),
    (_slabs(1, 0, 8), _slabs(1, 8, 16)),
    (_slabs(2, 0, 8) + _slabs(0, 16, 18) + _slabs(1, 16, 18), _slabs(2, 8, 16) + _slabs(2, 16, 18) * 2),
)

LEFT3 = (
    ((0, 1, 0), (0, 0, 0)), ((0, 0, -1), (0, 0, 0)), ((-1, 0, 1), (0, 0, 0)), ((-1, 1, 0), (0, 0, 0)),
    ((0, -1, 0), (0, 1, 0)), ((0, 0, 0), (0, 0, -1)), ((0, -1, 1), (0, 1, -1)), ((0, -1, 0), (0, 1, -1)),
    ((0, 0, 0), (0, 1, -1)), ((1, 0, -1), (-1, 0, 1)), ((1, 0, 0), (-1, 0, 0)), ((1, 0, -1), (-1, 0, 0)),
    ((0, 0, 0), (-1, 0, 0)), ((0, 1, 0), (-1, 0, 0)), ((0, 0, 0), (-1, 1, 0)))
RIGHT3 = (
    ((0, -1, 0), (0, -1, 1), (0, 0, 0)), ((0, 0, -1), (0, 0, 0), (0, 1, -1)), ((0, 0, -1), (0, 0, 0), (0, 0, 0)),
    ((0, 1, 0), (0, 0, 0), (0, 0, 0)), ((0, 0, 0), (1, -1, 0), (0, -1, 0)), ((0, 0, 0), (0, 0, 1), (1, 0, 1)),
    ((0, 0, 0), (0, 0, 0), (0, 1, 0)), ((0, 0, 0), (0, 0, 1), (0, 1, 0)), ((0, 0, 0), (0, 0, 1), (0, 0, 0)),
    ((0, 0, 0), (0, 0, 0), (1, 0, 0)), ((1, -1, 0), (0, 0, 0), (1, 0, 0)), ((0, 0, -1), (0, 0, 0), (1, 0, 0)),
    ((-1, 0, -1), (-1, 0, 0), (0, 0, 0)), ((0, -1, 0), (-1, 0, 0), (0, 0, 0)), ((0, 0, 0), (-1, 0, 0), (0, 0, 0)))
EXTRA3 = (
    {1: ((1, 0), (0, 0, 1)), 3: ((1, 0), (0, -1, 0)), 4: ((1, -1), (-1, 1, 0)),
     5: ((0, 1), (0, 0, -1)), 13: ((1, 0), (-1, 1, 0)), 14: ((0, 1), (-1, 0, 0))},
    {1: ((1, 0), (0, -1, 1)), 4: ((0, 1), (0, -1, 0)), 5: ((0, 1), (-1, 0, -1)),
     6: ((1, 0), (0, 1, 0)), 9: ((0, 1), (1, 0, 0)), 10: ((1, 0), (1, 0, 0))},
    {3: ((1, 0), (0, -1, 1)), 6: ((1, 0), (0, 0, 1)), 9: ((0, 1), (0, 0, -1)),
     10: ((1, -1), (1, -1, 1)), 13: ((0, 1), (-1, 1, -1)), 14: ((0, 1), (-1, 0, -1))})
SLICES3 = tuple(
    {(1, 2): (2, 1)}.get(s, s) for s in (tuple(k for k in range(3) if n in EXTRA3[k]) for n in range(15)))
KS3 = tuple(128 + 64 * len(s) for s in SLICES3)
KO3 = tuple(sum(KS3[:n]) for n in range(15))
KT3 = sum(KS3)
ORDER3 = (2, 11, 9, 12, 14, 8, 5, 7, 0, 3, 6, 1, 13, 10, 4)


def _outputs3(m):
    a, b = m[2] + m[11], m[7] - m[8]
    c, d = m[0] + b, m[9] - a
    return (m[12] - a - m[3] - m[13] + m[10], m[6] - (c + m[3]), m[2] - b + m[6] + m[1],
            m[12] + d - m[14], m[13] - (m[14] + c) - m[4], m[8] - d - m[5])


def _terms3(n):
    parts = [([(c, (i, k)) for i in range(2) for k, c in enumerate(LEFT3[n][i]) if c],
              [(c, (128 * k, 128, j)) for k in range(3) for j, c in enumerate(RIGHT3[n][k]) if c])]
    for s in SLICES3[n]:
        left, right = EXTRA3[s][n]
        parts.append(([(c, (i, 4 if s == 2 else 3)) for i, c in enumerate(left) if c],
                      [(c, (384 + 64 * s, 64, j)) for j, c in enumerate(right) if c]))
    return [([(c * r[0][0], x) for c, x in l], [(c * r[0][0], x) for c, x in r]) for l, r in parts]


def _signed_sum(terms):
    terms = sorted(terms, key=lambda t: -t[0])
    total = terms[0][1] if terms[0][0] > 0 else -terms[0][1]
    for c, v in terms[1:]:
        total = total + v if c > 0 else total - v
    return total


def _kernel(c_hbm, x_hbm, wqkv_hbm, wo_hbm, wg_hbm, wu_hbm, wd_hbm, wmod_hbm, out_hbm,
            c_ref, xt, wqkv, wo, wg, wu, wd, wmod, wqkv_t, wo_rows, wo_t, qkv_rhs, wo_lhs,
            mod_rows, gate_cols, wg_rhs, wu_rhs, wd_lhs, qbuf, kbuf, vbuf, qkv_lhs, wo_rhs, x1, ffn_lhs,
            acc7, sems):
    lo = lax.broadcasted_iota(I32, (1, 128), 1) < 64

    def start(src, dst, sem):
        copy = pltpu.make_async_copy(src, dst, sems.at[sem])
        copy.start()
        return copy

    def start_cols(sem, *pieces):
        return [start(src.at[:, pl.ds(c0, n)], dst.at[:, pl.ds(c0, n)], sem) for src, dst, c0, n in pieces]

    def wait(copies):
        for copy in copies:
            copy.wait()

    ffn = ((wg_hbm, wg), (wu_hbm, wu), (wd_hbm, wd))
    in_mod = start_cols(0, (c_hbm, c_ref, 0, D), (wmod_hbm, wmod, 0, 2 * D))
    in_x0 = start_cols(1, (x_hbm, xt, 0, TM))
    in_qa = start_cols(2, (wqkv_hbm, wqkv, 0, 384))
    in_qb = start_cols(3, (wqkv_hbm, wqkv, 384, 256))
    in_k = start_cols(4, (wqkv_hbm, wqkv, 640, 512))
    in_v = start_cols(5, (wqkv_hbm, wqkv, 1152, D))
    in_x12 = start_cols(6, (x_hbm, xt, TM, 2 * TM))
    in_ffn0 = start_cols(7, (wo_hbm, wo, 0, D), (wmod_hbm, wmod, 2 * D, 4 * D), *((a, b, 0, 4 * FC) for a, b in ffn))
    in_ffn1 = start_cols(8, *((a, b, 4 * FC, F - 4 * FC) for a, b in ffn))
    in_x3 = start_cols(9, (x_hbm, xt, 3 * TM, TM))

    always = []

    def after(x, prev):
        if not always:
            bits = pltpu.bitcast(jnp.broadcast_to(c_ref[:, 0:128].astype(F32), (8, 128)), I32)
            always.append(((bits * bits) & 2) == 0)
        return jnp.where(jnp.broadcast_to(always[0][0:1], x.shape[-2:]), x, prev)

    def modulation(c0, n):
        cf = c_ref[...].astype(F32)
        s = (cf * jax.nn.sigmoid(cf)).astype(BF)
        return _dot(jnp.broadcast_to(s, (16, D)), wmod[:, c0:c0 + n])[0:8]

    def set_shift_scale(n, shift, scale):
        mod_rows[2 * n] = jnp.concatenate([shift, shift[:, 512:D]], axis=1)
        scale = 1.0 + scale
        mod_rows[2 * n + 1] = jnp.concatenate([scale, scale[:, 512:D]], axis=1)

    def set_gate(n, row):
        for j in range(NT):
            r = row[0:1, j * 128:j * 128 + _width(j)]
            gate_cols[n, j * 128:j * 128 + _width(j), :] = jnp.broadcast_to(r, (128, _width(j))).T

    def store_left2(dst, rows, p, q):
        for n, tiles in enumerate(_left_tiles(p, q, lo)):
            for j, v in enumerate(tiles):
                dst[rows, KO2[n] + j * 128:KO2[n] + (j + 1) * 128] = _pack(v)

    def store_left3(dst, rows, *groups):
        for n in range(15):
            parts = [_signed_sum([(c, groups[i][k]) for c, (i, k) in left]) for left, _ in _terms3(n)]
            tiles = parts[:1] + ([jnp.where(lo, *parts[1:])] if len(parts) > 1 else [])
            for j, v in enumerate(tiles):
                dst[rows, KO3[n] + j * 128:KO3[n] + (j + 1) * 128] = _pack(v)

    def ada_norm(store, load, n, spread):
        prev = None
        for t in range(T // 128):
            halves = []
            for half in range(2):
                x = load(half * T + t * 128)
                if prev is not None:
                    x = jnp.concatenate([after(x[0:128], prev), x[128:D]], axis=0)
                tiles = []
                for j, y in enumerate(_feature_tiles(_normalize(x))):
                    if spread and j > 0:
                        y = after(y, prev)
                    cols = slice(j * 128, (j + 1) * 128)
                    tiles.append(y.T * mod_rows[2 * n + 1, 0:1, cols] + mod_rows[2 * n, 0:1, cols])
                    prev = tiles[-1] if spread else None
                halves.append(tiles)
            store(slice(t * 64, (t + 1) * 64), *halves)

    def norm1(i, spread):
        ada_norm(functools.partial(store_left2, qkv_lhs.at[i % 2]),
                 lambda r: xt[:, i * TM + r:i * TM + r + 128].astype(F32), 0, spread)

    def norm2(i, spread):
        ada_norm(functools.partial(store_left3, ffn_lhs.at[i % 2]), lambda r: x1[i % 2, :, r:r + 128], 1, spread)

    def transpose_wqkv(first, last):
        for cb in range(first, last):
            cw = min(128, 3 * D - cb * 128)
            for j, t in enumerate(_feature_tiles(wqkv[:, cb * 128:cb * 128 + cw].astype(F32))):
                wqkv_t[j, cb * 128:cb * 128 + cw, :] = t.T

    qkv_products = {}

    def qkv(i, g, first=0, last=7):
        rows = slice(g * 128, g * 128 + len(QKV_GROUPS[g][0]) * H // 2)
        gather = [lambda j, slabs=slabs: jnp.concatenate(
            [wqkv_t[j, pl.ds(part * D + d, H, stride=DH), :] for part, d in slabs], axis=0) for slabs in QKV_GROUPS[g]]
        m = qkv_products.setdefault((i, g), {})
        for n in ORDER2[first:last]:
            cols = slice(KO2[n], KO2[n] + KS2[n])
            if i == 0:
                rhs = jnp.concatenate(_right_tiles(n, *gather, lo), axis=1).astype(BF)[:, 0:KS2[n]]
                qkv_rhs[rows, cols] = _pack(rhs)
            else:
                rhs = _unpack(qkv_rhs[rows, cols])
            m[n] = _dot_nt(_unpack(qkv_lhs[i % 2, :, cols]), rhs)
        if last < 7:
            return
        c = _quadrants(m)
        for half in range(2):
            r = i * TM + half * T
            for j in range(4):
                tile = c[2 * half + j // 2][:, (j % 2) * 128:(j % 2 + 1) * 128]
                if g == 0:
                    qbuf[j, r:r + T, :] = tile * QSCALE
                else:
                    (kbuf, vbuf)[g - 1][j, HALO + r:HALO + r + T, :] = tile
            if g == 2:
                qk = c[2 * half][:, 256:384]
                qbuf[4, r:r + T, :] = jnp.where(lo, qk * QSCALE, 0.0)
                kbuf[4, HALO + r:HALO + r + T, :] = jnp.where(lo, pltpu.roll(qk, 64, 1), 0.0)
                vbuf[4, HALO + r:HALO + r + T, :] = c[2 * half + 1][:, 256:384]
        if i == 0 and g == 2:
            for j in range(NT):
                kbuf[j, 0:HALO, :] = jnp.broadcast_to(kbuf[j, HALO:HALO + 1, :], (HALO, 128))
                vbuf[j, 0:HALO, :] = jnp.broadcast_to(vbuf[j, HALO:HALO + 1, :], (HALO, 128))

    def attend(r0, prev):
        q = qbuf[:, r0:r0 + 8, :]
        if prev is not None:
            q = after(q, prev)
        logits = []
        for w in range(W):
            a = HALO + r0 - DIL * w
            p = jnp.sum(q * kbuf[:, a:a + 8, :], axis=0)
            p = p + pltpu.roll(p, 64, 1)
            p = p + pltpu.roll(p, 32, 1)
            if r0 < DIL * w:
                p = jnp.where(lax.broadcasted_iota(I32, (8, 128), 0) + r0 >= DIL * w, p, MASKED)
            logits.append(p)
        m = functools.reduce(jnp.maximum, logits)
        es = [jnp.exp2(l - m) for l in logits]
        den = functools.reduce(jnp.add, es)
        acc = None
        for w in range(W):
            a = HALO + r0 - DIL * w
            t = es[w][None] * vbuf[:, a:a + 8, :]
            acc = t if acc is None else acc + t
        inv = pl.reciprocal(den, approx=True)
        inv = inv * (2.0 - den * inv)
        inv = inv * (2.0 - den * inv)
        return acc * inv[None]

    def attention(i, chains, delay):
        done = []
        for r in range(0, T, 16):
            o = []
            for half in range(2):
                for r0 in (r, r + 8):
                    prev = done[-chains] if len(done) >= chains else None
                    if prev is not None and delay:
                        prev = jnp.concatenate([pltpu.roll(prev[0:1], 1, 2), prev[1:]], axis=0)
                    done.append(attend(i * TM + half * T + r0, prev))
                o.append(jnp.concatenate(done[-2:], axis=1))
            for n in range(7):
                for j, v in enumerate(_right_tiles(n, lambda j: o[0][j], lambda j: o[1][j], lo)):
                    wo_rhs[r // 2:r // 2 + 8, KO2[n] + j * 128:KO2[n] + (j + 1) * 128] = _pack(v)

    def prepare_wo():
        for j in range(NT):
            wo_rows[j, 0:D, 0:_width(j)] = wo[:, j * 128:j * 128 + _width(j)].astype(F32)
        for j in range(NT):
            p = jnp.concatenate([wo_rows[j, pl.ds(d, H, stride=DH), :] for d in range(DH)], axis=0)
            for n, t in enumerate(_feature_tiles(p[:, 0:_width(j)])):
                wo_t[n, j * 128:j * 128 + _width(j), :] = t.T
        store_left2(wo_lhs, slice(None), [wo_t[n, 0:D2, :] for n in range(NT)], [wo_t[n, D2:D, :] for n in range(NT)])

    def out_projection(i):
        m = {}
        for n in ORDER2:
            cols = slice(KO2[n], KO2[n] + KS2[n])
            m[n] = _dot_nt(_unpack(wo_lhs[:, cols]), _unpack(wo_rhs[:, cols]))
        for e, v in enumerate(_quadrants(m)):
            rows = slice((e // 2) * D2, (e // 2 + 1) * D2)
            for t in range(T // 128):
                c0 = (e % 2) * T + t * 128
                x1[i % 2, rows, c0:c0 + 128] = (xt[rows, i * TM + c0:i * TM + c0 + 128].astype(F32)
                                                + gate_cols[0, rows, :] * v[:, t * 128:(t + 1) * 128])

    def gate_up(i, p):
        fc = 2 * FC // 3
        branches = []
        for w, w_rhs in ((wg, wg_rhs), (wu, wu_rhs)):
            m = {}
            for n in ORDER3:
                where = (slice(KO3[n] // 2, (KO3[n] + KS3[n]) // 2), slice(p * fc, (p + 1) * fc))
                if i == 0:
                    terms = [[(c, w[r:r + k, (3 * p + j) * fc:(3 * p + j + 1) * fc]) for c, (r, k, j) in right]
                             for _, right in _terms3(n)]
                    if all(len(t) == 1 for t in terms):
                        rhs = jnp.concatenate([t[0][1] for t in terms], axis=0)
                    else:
                        rhs = jnp.concatenate([_signed_sum([(c, v.astype(F32)) for c, v in t]) for t in terms],
                                              axis=0).astype(BF)
                    w_rhs[where] = _pack(rhs)
                else:
                    rhs = _unpack(w_rhs[where])
                m[n] = _dot(_unpack(ffn_lhs[i % 2, :, KO3[n]:KO3[n] + KS3[n]]), rhs)
            branches.append(_outputs3(m))
        h = [g * u for g, u in zip(*branches)]
        h = [jnp.concatenate(h[3 * half:3 * half + 3], axis=1) for half in range(2)]
        return [v[:, k * FC:(k + 1) * FC] for v in h for k in range(2)]

    def write_out(i, rows, c0, v):
        xt[rows, i * TM + c0:i * TM + c0 + 128] = (x1[i % 2, rows, c0:c0 + 128] + gate_cols[1, rows, :] * v).astype(BF)

    def hidden_one_level(p):
        h = gate_up(0, p)
        return [v.astype(BF) for v in _rights(h[0], h[2], h[1], h[3])]

    def down_one_level(p, rights):
        lefts = _lefts(*(wd[i1 * D2:(i1 + 1) * D2, (2 * p + k) * FC:(2 * p + k + 1) * FC].astype(F32)
                         for i1 in range(2) for k in range(2)))
        m = {}
        for products, e in PROGRESSIVE:
            for n in products:
                part = _dot_nt(lefts[n].astype(BF), rights[n])
                m[n] = part if p == 0 else acc7[n] + part
                if p < NP - 1:
                    acc7[n] = m[n]
            if p == NP - 1:
                v = _quadrant(m, e)
                for t in range(T // 128):
                    write_out(0, slice((e // 2) * D2, (e // 2 + 1) * D2), (e % 2) * T + t * 128,
                              v[:, t * 128:(t + 1) * 128])

    hidden = {}

    def hidden_two_levels(h0, h1):
        outer = [_rights(*(h[2 * j1 + k2][j2 * 128:(j2 + 1) * 128] for h in (h0, h1) for j1 in range(2)))
                 for k2 in range(2) for j2 in range(2)]
        for n in range(7):
            for k, v in enumerate(_rights(*(o[n] for o in outer))):
                hidden.setdefault(7 * n + k, []).append(v)

    def prepare_wd(chains):
        done = []
        for q in range(NP // 2):
            for c in range(0, FC, 128):
                for r in range(0, D4, 16):
                    outer = [_lefts(*(wd[i1 * D2 + i2 * D4 + r:i1 * D2 + i2 * D4 + r + 16,
                                         (4 * q + 2 * k1 + k2) * FC + c:(4 * q + 2 * k1 + k2) * FC + c + 128].astype(F32)
                                      for i1 in range(2) for k1 in range(2)))
                             for i2 in range(2) for k2 in range(2)]
                    where = (slice(r // 2, r // 2 + 8), slice(q * FC + c, q * FC + c + 128))
                    for n in range(7):
                        blocks = [o[n] for o in outer]
                        if len(done) >= chains:
                            blocks[0] = after(blocks[0], done[-chains])
                        for k, v in enumerate(_lefts(*blocks)):
                            wd_lhs.at[7 * n + k][where] = _pack(v)
                        stored = wd_lhs[(slice(7 * n, 7 * n + 7),) + where]
                        link = functools.reduce(jnp.bitwise_or, [stored[k] for k in range(7)])
                        link = pltpu.bitcast(pltpu.roll(link, 1, 1), F32)
                        done.append(jnp.concatenate([link, link], axis=0))

    def down(i):
        copies, inner = [], {}
        for products, e1 in PROGRESSIVE:
            for n in products:
                inner[n] = _quadrants({
                    k: _dot_nt(_unpack(wd_lhs[7 * n + k]), jnp.concatenate(hidden.pop(7 * n + k), axis=1).astype(BF))
                    for group, _ in PROGRESSIVE for k in group})
            r0, c0 = (e1 // 2) * D2, (e1 % 2) * T
            for e2 in range(4):
                write_out(i, slice(r0 + (e2 // 2) * D4, r0 + (e2 // 2 + 1) * D4), c0 + (e2 % 2) * 128,
                          _quadrant({n: quads[e2] for n, quads in inner.items()}, e1))
            if i == NB - 1:
                copies.append(start(*(a.at[pl.ds(r0, D2), pl.ds(i * TM + c0, T)] for a in (xt, out_hbm)), i))
        return copies if i == NB - 1 else start_cols(i, (xt, out_hbm, i * TM, TM))

    wait(in_mod)
    m = modulation(0, 2 * D)
    set_shift_scale(0, m[:, 0:D], m[:, D:2 * D])
    wait(in_x0)
    norm1(0, False)
    wait(in_qa)
    transpose_wqkv(0, 3)
    wait(in_qb)
    transpose_wqkv(3, 5)
    qkv(0, 0, 0, 4)
    wait(in_k)
    transpose_wqkv(5, 9)
    qkv(0, 0, 4, 7)
    qkv(0, 1, 0, 2)
    wait(in_v)
    transpose_wqkv(9, 14)
    qkv(0, 1, 2, 7)
    wait(in_x12)
    qkv(0, 2)
    norm1(1, False)
    for g in range(3):
        qkv(1, g)
    norm1(2, True)
    qkv(2, 0)
    qkv(2, 1)
    attention(0, 4, True)
    wait(in_ffn0)
    set_gate(0, modulation(2 * D, 640)[:, 0:D])
    prepare_wo()
    out_projection(0)
    m = modulation(3 * D - 64, 3 * D + 64)
    set_shift_scale(1, m[:, 64:64 + D], m[:, 64 + D:64 + 2 * D])
    set_gate(1, m[:, 64 + 2 * D:64 + 3 * D])
    qkv(2, 2)
    norm2(0, False)

    pending = None
    for p in range(NP):
        if p == 2:
            wait(in_ffn1)
        if p == NP - 1:
            attention(1, 2, True)
            out_projection(1)
        rights = hidden_one_level(p)
        if p > 0:
            down_one_level(p - 1, pending)
        pending = rights
    down_one_level(NP - 1, pending)
    outputs = [start_cols(0, (xt, out_hbm, 0, TM))]
    norm2(1, True)
    wait(in_x3)

    for i in range(1, NB):
        for p in range(NP):
            if (i, p) == (2, 1):
                norm1(3, True)
                for g in range(3):
                    qkv(3, g)
            if p == NP - 1 and i + 1 < NB:
                attention(i + 1, 1, False)
                out_projection(i + 1)
            h = gate_up(i, p)
            if p % 2:
                hidden_two_levels(pending, h)
            pending = h
        if i == 1:
            prepare_wd(3)
        outputs.append(down(i))
        if i + 1 < NB:
            norm2(i + 1, True)
        if i == 1:
            wait(outputs.pop(0))
    for copies in outputs:
        wait(copies)


@jax.jit
def pallas_adaLN_cond__sliding_local_dilated__glu_gated_bilinear__prompt_kernel(
    A_x: jax.Array,
    A_wqkv: jax.Array,
    A_wo: jax.Array,
    B_x: jax.Array,
    B_w_gate: jax.Array,
    B_w_up: jax.Array,
    B_w_down: jax.Array,
    c: jax.Array,
    w_mod: jax.Array,
):
    del B_x
    hbm = pl.BlockSpec(memory_space=pltpu.HBM)
    vmem = pltpu.VMEM
    out_t = pl.pallas_call(
        _kernel,
        in_specs=[hbm] * 8,
        out_specs=hbm,
        out_shape=jax.ShapeDtypeStruct((D, S), BF),
        scratch_shapes=[
            vmem((1, D), BF),
            vmem((D, S), BF),
            vmem((D, 3 * D), BF),
            vmem((D, D), BF),
            vmem((D, F), BF),
            vmem((D, F), BF),
            vmem((D, F), BF),
            vmem((D, 6 * D), BF),
            vmem((NT, 1792, 128), F32),
            vmem((NT, D + 24, 128), F32),
            vmem((NT, D, 128), F32),
            vmem((448, KT2), I32),
            vmem((D2 // 2, KT2), I32),
            vmem((4, 8, NT * 128), F32),
            vmem((2, D, 128), F32),
            vmem((KT3 // 2, F // 3), I32),
            vmem((KT3 // 2, F // 3), I32),
            vmem((49, D4 // 2, F // 4), I32),
            vmem((NT, S, 128), F32),
            vmem((NT, HALO + S, 128), F32),
            vmem((NT, HALO + S, 128), F32),
            vmem((2, T // 2, KT2), I32),
            vmem((T // 2, KT2), I32),
            vmem((2, D, TM), F32),
            vmem((2, T // 2, KT3), I32),
            vmem((7, D2, T), F32),
            pltpu.SemaphoreType.DMA((10,)),
        ],
        compiler_params=pltpu.CompilerParams(vmem_limit_bytes=126 * 2**20),
        name="adaln_local_attention_bilinear_glu",
    )(c, A_x.reshape(S, D).T, A_wqkv, A_wo, B_w_gate, B_w_up, B_w_down.T, w_mod)
    return out_t.T.reshape(1, S, D)
```

```python
import functools

import jax
import jax.numpy as jnp
from jax import lax
import jax.experimental.pallas as pl
import jax.experimental.pallas.tpu as pltpu

S, D, F = 2048, 576, 4608
H, DH, W, DIL = 32, 18, 8, 2
EPS = 1e-5
LOG2E = 1.4426950408889634
QSCALE = DH ** -0.5 * LOG2E
MASKED = -1e9 * LOG2E

TM = 512
T = TM // 2
NB = S // TM
FC = 384
NP = F // (2 * FC)
NT = 5
D2, D4 = D // 2, D // 4
HALO = 16

BF, F32, I32 = jnp.bfloat16, jnp.float32, jnp.int32


def _dot(a, b):
    return jnp.dot(a, b, preferred_element_type=F32)


def _dot_nt(a, b):
    return lax.dot_general(a, b, (((1,), (1,)), ((), ())), preferred_element_type=F32)


def _pack(v):
    return pltpu.bitcast(v.astype(BF), I32)


def _unpack(v):
    return pltpu.bitcast(v, BF)


def _width(j):
    return min(128, D - 128 * j)


def _feature_tiles(y):
    return [y[j * 128:(j + 1) * 128] for j in range(4)] + [jnp.concatenate([y[512:D], y[512:D]], axis=0)]


def _normalize(x):
    colsum = lambda v: jnp.sum(jnp.sum(v.reshape(D // 32, 32, 128), axis=0), axis=0, keepdims=True)
    xc = x - colsum(x) * (1.0 / D)
    return xc * lax.rsqrt(colsum(xc * xc) * (1.0 / D) + EPS)


def _lefts(a11, a12, a21, a22):
    return a11 + a22, a21 + a22, a11, a22, a11 + a12, a21 - a11, a22 - a12


def _rights(b11, b12, b21, b22):
    return b11 + b22, b11, b12 - b22, b21 - b11, b22, b11 + b12, b21 + b22


def _quadrant(m, e):
    return (lambda: m[0] - m[4] + m[3] - m[6], lambda: m[4] + m[2],
            lambda: m[1] + m[3], lambda: m[0] - m[1] + m[2] + m[5])[e]()


def _quadrants(m):
    return [_quadrant(m, e) for e in range(4)]


ORDER2 = (1, 4, 0, 2, 3, 5, 6)
PROGRESSIVE = (((4, 2), 1), ((1, 3), 2), ((0, 5), 3), ((6,), 0))

KS2 = (256, 256, 384, 384, 192, 384, 256)
KO2 = (0, 256, 512, 896, 1280, 1536, 1920)
KT2 = 2176


def _left_tiles(p, q, lo):
    d = [y - x for x, y in zip(p, q)]
    w = lambda a, b: jnp.where(lo, a, b)
    return (
        (p[0] + q[1], w(p[2] + q[3], p[2] - q[2])),
        (q[0] + q[1], w(q[2] + q[3], d[3])),
        (p[0], p[2], w(p[4], p[3])),
        (q[1], w(q[3], p[3]), w(q[4], q[2])),
        (p[0] + p[1], p[2] + p[3]),
        (d[0], d[2], w(d[4], d[3])),
        (d[1], w(d[3], d[4])),
    )


def _right_tiles(n, a, b, lo):
    w = lambda x, y: jnp.where(lo, x, y)
    return (
        lambda: (a(0) + b(1), w(a(2) + b(3), a(2))),
        lambda: (a(0), w(a(2), a(3))),
        lambda: (b(0) - b(1), w(b(2) - b(3), b(2)), w(b(4), b(3))),
        lambda: (a(1) - a(0), w(a(3) - a(2), a(3)), w(a(4), a(2))),
        lambda: (b(1), b(3)),
        lambda: (a(0) + b(0), a(2) + b(2), w(b(4), a(3) + b(3))),
        lambda: (a(1) + b(1), w(a(3) + b(3), a(4))),
    )[n]()


def _slabs(part, start, stop):
    return [(part, d) for d in range(start, stop)]


QKV_GROUPS = (
    (_slabs(0, 0, 8), _slabs(0, 8, 16)),
    (_slabs(1, 0, 8), _slabs(1, 8, 16)),
    (_slabs(2, 0, 8) + _slabs(0, 16, 18) + _slabs(1, 16, 18), _slabs(2, 8, 16) + _slabs(2, 16, 18) * 2),
)

LEFT3 = (
    ((0, 1, 0), (0, 0, 0)), ((0, 0, -1), (0, 0, 0)), ((-1, 0, 1), (0, 0, 0)), ((-1, 1, 0), (0, 0, 0)),
    ((0, -1, 0), (0, 1, 0)), ((0, 0, 0), (0, 0, -1)), ((0, -1, 1), (0, 1, -1)), ((0, -1, 0), (0, 1, -1)),
    ((0, 0, 0), (0, 1, -1)), ((1, 0, -1), (-1, 0, 1)), ((1, 0, 0), (-1, 0, 0)), ((1, 0, -1), (-1, 0, 0)),
    ((0, 0, 0), (-1, 0, 0)), ((0, 1, 0), (-1, 0, 0)), ((0, 0, 0), (-1, 1, 0)))
RIGHT3 = (
    ((0, -1, 0), (0, -1, 1), (0, 0, 0)), ((0, 0, -1), (0, 0, 0), (0, 1, -1)), ((0, 0, -1), (0, 0, 0), (0, 0, 0)),
    ((0, 1, 0), (0, 0, 0), (0, 0, 0)), ((0, 0, 0), (1, -1, 0), (0, -1, 0)), ((0, 0, 0), (0, 0, 1), (1, 0, 1)),
    ((0, 0, 0), (0, 0, 0), (0, 1, 0)), ((0, 0, 0), (0, 0, 1), (0, 1, 0)), ((0, 0, 0), (0, 0, 1), (0, 0, 0)),
    ((0, 0, 0), (0, 0, 0), (1, 0, 0)), ((1, -1, 0), (0, 0, 0), (1, 0, 0)), ((0, 0, -1), (0, 0, 0), (1, 0, 0)),
    ((-1, 0, -1), (-1, 0, 0), (0, 0, 0)), ((0, -1, 0), (-1, 0, 0), (0, 0, 0)), ((0, 0, 0), (-1, 0, 0), (0, 0, 0)))
EXTRA3 = (
    {1: ((1, 0), (0, 0, 1)), 3: ((1, 0), (0, -1, 0)), 4: ((1, -1), (-1, 1, 0)),
     5: ((0, 1), (0, 0, -1)), 13: ((1, 0), (-1, 1, 0)), 14: ((0, 1), (-1, 0, 0))},
    {1: ((1, 0), (0, -1, 1)), 4: ((0, 1), (0, -1, 0)), 5: ((0, 1), (-1, 0, -1)),
     6: ((1, 0), (0, 1, 0)), 9: ((0, 1), (1, 0, 0)), 10: ((1, 0), (1, 0, 0))},
    {3: ((1, 0), (0, -1, 1)), 6: ((1, 0), (0, 0, 1)), 9: ((0, 1), (0, 0, -1)),
     10: ((1, -1), (1, -1, 1)), 13: ((0, 1), (-1, 1, -1)), 14: ((0, 1), (-1, 0, -1))})
SLICES3 = tuple(
    {(1, 2): (2, 1)}.get(s, s) for s in (tuple(k for k in range(3) if n in EXTRA3[k]) for n in range(15)))
KS3 = tuple(128 + 64 * len(s) for s in SLICES3)
KO3 = tuple(sum(KS3[:n]) for n in range(15))
KT3 = sum(KS3)
ORDER3 = (2, 11, 9, 12, 14, 8, 5, 7, 0, 3, 6, 1, 13, 10, 4)


def _outputs3(m):
    a, b = m[2] + m[11], m[7] - m[8]
    c, d = m[0] + b, m[9] - a
    return (m[12] - a - m[3] - m[13] + m[10], m[6] - (c + m[3]), m[2] - b + m[6] + m[1],
            m[12] + d - m[14], m[13] - (m[14] + c) - m[4], m[8] - d - m[5])


def _terms3(n):
    parts = [([(c, (i, k)) for i in range(2) for k, c in enumerate(LEFT3[n][i]) if c],
              [(c, (128 * k, 128, j)) for k in range(3) for j, c in enumerate(RIGHT3[n][k]) if c])]
    for s in SLICES3[n]:
        left, right = EXTRA3[s][n]
        parts.append(([(c, (i, 4 if s == 2 else 3)) for i, c in enumerate(left) if c],
                      [(c, (384 + 64 * s, 64, j)) for j, c in enumerate(right) if c]))
    return [([(c * r[0][0], x) for c, x in l], [(c * r[0][0], x) for c, x in r]) for l, r in parts]


def _terms3_sign(n):
    return max(c for row in RIGHT3[n] for c in row if c)


def _signed_sum(terms):
    terms = sorted(terms, key=lambda t: -t[0])
    total = terms[0][1] if terms[0][0] > 0 else -terms[0][1]
    for c, v in terms[1:]:
        total = total + v if c > 0 else total - v
    return total


def _kernel(c_hbm, x_hbm, wqkv_hbm, wo_hbm, wg_hbm, wu_hbm, wd_hbm, wmod_hbm, out_hbm,
            c_ref, xt, wqkv, wo, wg, wu, wd, wmod, wqkv_t, wo_rows, wo_t, qkv_rhs, wo_lhs,
            mod_rows, gate_cols, wg_rhs, wu_rhs, wd_lhs, qbuf, kbuf, vbuf, qkv_lhs, wo_rhs, x1, ffn_lhs,
            acc, sems):
    lo = lax.broadcasted_iota(I32, (1, 128), 1) < 64

    def start(src, dst, sem):
        copy = pltpu.make_async_copy(src, dst, sems.at[sem])
        copy.start()
        return copy

    def start_cols(sem, *pieces):
        return [start(src.at[:, pl.ds(c0, n)], dst.at[:, pl.ds(c0, n)], sem) for src, dst, c0, n in pieces]

    def wait(copies):
        for copy in copies:
            copy.wait()

    ffn = ((wg_hbm, wg), (wu_hbm, wu), (wd_hbm, wd))
    in_mod = start_cols(0, (c_hbm, c_ref, 0, D), (wmod_hbm, wmod, 0, 2 * D))
    in_x0 = start_cols(1, (x_hbm, xt, 0, TM))
    in_qa = start_cols(2, (wqkv_hbm, wqkv, 0, 384))
    in_qb = start_cols(3, (wqkv_hbm, wqkv, 384, 256))
    in_k = start_cols(4, (wqkv_hbm, wqkv, 640, 512))
    in_v = start_cols(5, (wqkv_hbm, wqkv, 1152, D))
    in_x12 = start_cols(6, (x_hbm, xt, TM, 2 * TM))
    in_ffn0 = start_cols(7, (wo_hbm, wo, 0, D), (wmod_hbm, wmod, 2 * D, 4 * D), *((a, b, 0, 4 * FC) for a, b in ffn))
    in_ffn1 = start_cols(8, *((a, b, 4 * FC, F - 4 * FC) for a, b in ffn))
    in_x3 = start_cols(9, (x_hbm, xt, 3 * TM, TM))

    always = []

    def after(x, prev):
        if not always:
            bits = pltpu.bitcast(jnp.broadcast_to(c_ref[:, 0:128].astype(F32), (8, 128)), I32)
            always.append(((bits * bits) & 2) == 0)
        return jnp.where(jnp.broadcast_to(always[0][0:1], x.shape[-2:]), x, prev)

    def modulation(c0, n):
        cf = c_ref[...].astype(F32)
        s = (cf * jax.nn.sigmoid(cf)).astype(BF)
        return _dot(jnp.broadcast_to(s, (16, D)), wmod[:, c0:c0 + n])[0:8]

    def set_shift_scale(n, shift, scale):
        mod_rows[2 * n] = jnp.concatenate([shift, shift[:, 512:D]], axis=1)
        scale = 1.0 + scale
        mod_rows[2 * n + 1] = jnp.concatenate([scale, scale[:, 512:D]], axis=1)

    def set_gate(n, row):
        for j in range(NT):
            r = row[0:1, j * 128:j * 128 + _width(j)]
            gate_cols[n, j * 128:j * 128 + _width(j), :] = jnp.broadcast_to(r, (128, _width(j))).T

    def store_left2(dst, rows, p, q):
        for n, tiles in enumerate(_left_tiles(p, q, lo)):
            for j, v in enumerate(tiles):
                dst[rows, KO2[n] + j * 128:KO2[n] + (j + 1) * 128] = _pack(v)

    def store_left3(dst, rows, *groups):
        for n in range(15):
            parts = [_signed_sum([(c, groups[i][k]) for c, (i, k) in left]) for left, _ in _terms3(n)]
            tiles = parts[:1] + ([jnp.where(lo, *parts[1:])] if len(parts) > 1 else [])
            for j, v in enumerate(tiles):
                dst[rows, KO3[n] + j * 128:KO3[n] + (j + 1) * 128] = _pack(v)

    def ada_norm(store, load, n, spread):
        prev = None
        for t in range(T // 128):
            halves = []
            for half in range(2):
                x = load(half * T + t * 128)
                if prev is not None:
                    x = jnp.concatenate([after(x[0:128], prev), x[128:D]], axis=0)
                tiles = []
                for j, y in enumerate(_feature_tiles(_normalize(x))):
                    if spread and j > 0:
                        y = after(y, prev)
                    cols = slice(j * 128, (j + 1) * 128)
                    tiles.append(y.T * mod_rows[2 * n + 1, 0:1, cols] + mod_rows[2 * n, 0:1, cols])
                    prev = tiles[-1] if spread else None
                halves.append(tiles)
            store(slice(t * 64, (t + 1) * 64), *halves)

    def norm1(i, spread):
        ada_norm(functools.partial(store_left2, qkv_lhs.at[i % 2]),
                 lambda r: xt[:, i * TM + r:i * TM + r + 128].astype(F32), 0, spread)

    def norm2(i, spread):
        ada_norm(functools.partial(store_left3, ffn_lhs.at[i % 2]), lambda r: x1[i % 2, :, r:r + 128], 1, spread)

    def transpose_wqkv(first, last):
        for cb in range(first, last):
            cw = min(128, 3 * D - cb * 128)
            for j, t in enumerate(_feature_tiles(wqkv[:, cb * 128:cb * 128 + cw].astype(F32))):
                wqkv_t[j, cb * 128:cb * 128 + cw, :] = t.T

    qkv_products = {}

    def qkv(i, g, first=0, last=7):
        rows = slice(g * 128, g * 128 + len(QKV_GROUPS[g][0]) * H // 2)
        gather = [lambda j, slabs=slabs: jnp.concatenate(
            [wqkv_t[j, pl.ds(part * D + d, H, stride=DH), :] for part, d in slabs], axis=0) for slabs in QKV_GROUPS[g]]
        m = qkv_products.setdefault((i, g), {})
        for n in ORDER2[first:last]:
            cols = slice(KO2[n], KO2[n] + KS2[n])
            if i == 0:
                rhs = jnp.concatenate(_right_tiles(n, *gather, lo), axis=1).astype(BF)[:, 0:KS2[n]]
                qkv_rhs[rows, cols] = _pack(rhs)
            else:
                rhs = _unpack(qkv_rhs[rows, cols])
            m[n] = _dot_nt(_unpack(qkv_lhs[i % 2, :, cols]), rhs)
        if last < 7:
            return
        c = _quadrants(m)
        for half in range(2):
            r = i * TM + half * T
            for j in range(4):
                tile = c[2 * half + j // 2][:, (j % 2) * 128:(j % 2 + 1) * 128]
                if g == 0:
                    qbuf[j, r:r + T, :] = tile * QSCALE
                else:
                    (kbuf, vbuf)[g - 1][j, HALO + r:HALO + r + T, :] = tile
            if g == 2:
                qk = c[2 * half][:, 256:384]
                qbuf[4, r:r + T, :] = jnp.where(lo, qk * QSCALE, 0.0)
                kbuf[4, HALO + r:HALO + r + T, :] = jnp.where(lo, pltpu.roll(qk, 64, 1), 0.0)
                vbuf[4, HALO + r:HALO + r + T, :] = c[2 * half + 1][:, 256:384]
        if i == 0 and g == 2:
            for j in range(NT):
                kbuf[j, 0:HALO, :] = jnp.broadcast_to(kbuf[j, HALO:HALO + 1, :], (HALO, 128))
                vbuf[j, 0:HALO, :] = jnp.broadcast_to(vbuf[j, HALO:HALO + 1, :], (HALO, 128))

    def attend(r0, prev):
        q = qbuf[:, r0:r0 + 8, :]
        if prev is not None:
            q = after(q, prev)
        logits = []
        for w in range(W):
            a = HALO + r0 - DIL * w
            p = jnp.sum(q * kbuf[:, a:a + 8, :], axis=0)
            p = p + pltpu.roll(p, 64, 1)
            p = p + pltpu.roll(p, 32, 1)
            if r0 < DIL * w:
                p = jnp.where(lax.broadcasted_iota(I32, (8, 128), 0) + r0 >= DIL * w, p, MASKED)
            logits.append(p)
        m = functools.reduce(jnp.maximum, logits)
        es = [jnp.exp2(l - m) for l in logits]
        den = functools.reduce(jnp.add, es)
        acc = None
        for w in range(W):
            a = HALO + r0 - DIL * w
            t = es[w][None] * vbuf[:, a:a + 8, :]
            acc = t if acc is None else acc + t
        inv = pl.reciprocal(den, approx=True)
        inv = inv * (2.0 - den * inv)
        inv = inv * (2.0 - den * inv)
        return acc * inv[None]

    def attention(i, chains, delay):
        done = []
        for r in range(0, T, 16):
            o = []
            for half in range(2):
                for r0 in (r, r + 8):
                    prev = done[-chains] if len(done) >= chains else None
                    if prev is not None and delay:
                        prev = jnp.concatenate([pltpu.roll(prev[0:1], 1, 2), prev[1:]], axis=0)
                    done.append(attend(i * TM + half * T + r0, prev))
                o.append(jnp.concatenate(done[-2:], axis=1))
            for n in range(7):
                for j, v in enumerate(_right_tiles(n, lambda j: o[0][j], lambda j: o[1][j], lo)):
                    wo_rhs[r // 2:r // 2 + 8, KO2[n] + j * 128:KO2[n] + (j + 1) * 128] = _pack(v)

    def prepare_wo():
        for j in range(NT):
            wo_rows[j, 0:D, 0:_width(j)] = wo[:, j * 128:j * 128 + _width(j)].astype(F32)
        for j in range(NT):
            p = jnp.concatenate([wo_rows[j, pl.ds(d, H, stride=DH), :] for d in range(DH)], axis=0)
            for n, t in enumerate(_feature_tiles(p[:, 0:_width(j)])):
                wo_t[n, j * 128:j * 128 + _width(j), :] = t.T
        store_left2(wo_lhs, slice(None), [wo_t[n, 0:D2, :] for n in range(NT)], [wo_t[n, D2:D, :] for n in range(NT)])

    def out_projection(i):
        m = {}
        for n in ORDER2:
            cols = slice(KO2[n], KO2[n] + KS2[n])
            m[n] = _dot_nt(_unpack(wo_lhs[:, cols]), _unpack(wo_rhs[:, cols]))
        for e, v in enumerate(_quadrants(m)):
            rows = slice((e // 2) * D2, (e // 2 + 1) * D2)
            for t in range(T // 128):
                c0 = (e % 2) * T + t * 128
                x1[i % 2, rows, c0:c0 + 128] = (xt[rows, i * TM + c0:i * TM + c0 + 128].astype(F32)
                                                + gate_cols[0, rows, :] * v[:, t * 128:(t + 1) * 128])

    def gate_up(i, p):
        fc = 2 * FC // 3
        branches = []
        for w, w_rhs in ((wg, wg_rhs), (wu, wu_rhs)):
            m = {}
            for n in ORDER3:
                where = (slice(KO3[n] // 2, (KO3[n] + KS3[n]) // 2), slice(p * fc, (p + 1) * fc))
                if i == 0:
                    terms = [[(c, w[r:r + k, (3 * p + j) * fc:(3 * p + j + 1) * fc]) for c, (r, k, j) in right]
                             for _, right in _terms3(n)]
                    if all(len(t) == 1 for t in terms):
                        rhs = jnp.concatenate([t[0][1] for t in terms], axis=0)
                    else:
                        rhs = jnp.concatenate([_signed_sum([(c, v.astype(F32)) for c, v in t]) for t in terms],
                                              axis=0).astype(BF)
                    w_rhs[where] = _pack(rhs)
                else:
                    rhs = _unpack(w_rhs[where])
                m[n] = _dot(_unpack(ffn_lhs[i % 2, :, KO3[n]:KO3[n] + KS3[n]]), rhs)
            branches.append(_outputs3(m))
        return [g * u for g, u in zip(*branches)]

    def write_out(i, rows, c0, v):
        xt[rows, i * TM + c0:i * TM + c0 + 128] = (x1[i % 2, rows, c0:c0 + 128] + gate_cols[1, rows, :] * v).astype(BF)

    def hidden_one_level(p):
        h = gate_up(0, p)
        return [_signed_sum([(c * _terms3_sign(n), h[3 * i + k]) for i in range(2) for k, c in enumerate(LEFT3[n][i]) if c]).astype(BF)
                for n in range(15)]

    def down_one_level(p, rights):
        fc, d3 = 2 * FC // 3, D // 3
        m = {}
        for n in ORDER3:
            left = _signed_sum([(c * _terms3_sign(n), wd[j * d3:(j + 1) * d3, (3 * p + k) * fc:(3 * p + k + 1) * fc].astype(F32))
                                for k in range(3) for j, c in enumerate(RIGHT3[n][k]) if c])
            part = _dot_nt(left.astype(BF), rights[n])
            m[n] = part if p == 0 else acc[n] + part
            if p < NP - 1:
                acc[n] = m[n]
        if p == NP - 1:
            for e, v in enumerate(_outputs3(m)):
                for t in range(T // 128):
                    write_out(0, slice((e % 3) * d3, (e % 3 + 1) * d3), (e // 3) * T + t * 128,
                              v[:, t * 128:(t + 1) * 128])

    hidden = {}

    def hidden_two_levels(h0, h1):
        wide = [jnp.concatenate(h[3 * j1:3 * j1 + 3], axis=1) for h in (h0, h1) for j1 in range(2)]
        outer = [_rights(*(v[j2 * 128:(j2 + 1) * 128, k2 * FC:(k2 + 1) * FC] for v in wide))
                 for k2 in range(2) for j2 in range(2)]
        for n in range(7):
            for k, v in enumerate(_rights(*(o[n] for o in outer))):
                hidden.setdefault(7 * n + k, []).append(v)

    def prepare_wd(chains):
        done = []
        for q in range(NP // 2):
            for c in range(0, FC, 128):
                for r in range(0, D4, 16):
                    outer = [_lefts(*(wd[i1 * D2 + i2 * D4 + r:i1 * D2 + i2 * D4 + r + 16,
                                         (4 * q + 2 * k1 + k2) * FC + c:(4 * q + 2 * k1 + k2) * FC + c + 128].astype(F32)
                                      for i1 in range(2) for k1 in range(2)))
                             for i2 in range(2) for k2 in range(2)]
                    where = (slice(r // 2, r // 2 + 8), slice(q * FC + c, q * FC + c + 128))
                    for n in range(7):
                        blocks = [o[n] for o in outer]
                        if len(done) >= chains:
                            blocks[0] = after(blocks[0], done[-chains])
                        for k, v in enumerate(_lefts(*blocks)):
                            wd_lhs.at[7 * n + k][where] = _pack(v)
                        stored = wd_lhs[(slice(7 * n, 7 * n + 7),) + where]
                        link = functools.reduce(jnp.bitwise_or, [stored[k] for k in range(7)])
                        link = pltpu.bitcast(pltpu.roll(link, 1, 1), F32)
                        done.append(jnp.concatenate([link, link], axis=0))

    def down(i):
        copies, inner = [], {}
        for products, e1 in PROGRESSIVE:
            for n in products:
                inner[n] = _quadrants({
                    k: _dot_nt(_unpack(wd_lhs[7 * n + k]), jnp.concatenate(hidden.pop(7 * n + k), axis=1).astype(BF))
                    for group, _ in PROGRESSIVE for k in group})
            r0, c0 = (e1 // 2) * D2, (e1 % 2) * T
            for e2 in range(4):
                write_out(i, slice(r0 + (e2 // 2) * D4, r0 + (e2 // 2 + 1) * D4), c0 + (e2 % 2) * 128,
                          _quadrant({n: quads[e2] for n, quads in inner.items()}, e1))
            if i == NB - 1:
                copies.append(start(*(a.at[pl.ds(r0, D2), pl.ds(i * TM + c0, T)] for a in (xt, out_hbm)), i))
        return copies if i == NB - 1 else start_cols(i, (xt, out_hbm, i * TM, TM))

    wait(in_mod)
    m = modulation(0, 2 * D)
    set_shift_scale(0, m[:, 0:D], m[:, D:2 * D])
    wait(in_x0)
    norm1(0, False)
    wait(in_qa)
    transpose_wqkv(0, 3)
    wait(in_qb)
    transpose_wqkv(3, 5)
    qkv(0, 0, 0, 4)
    wait(in_k)
    transpose_wqkv(5, 9)
    qkv(0, 0, 4, 7)
    qkv(0, 1, 0, 2)
    wait(in_v)
    transpose_wqkv(9, 14)
    qkv(0, 1, 2, 7)
    wait(in_x12)
    qkv(0, 2)
    norm1(1, False)
    for g in range(3):
        qkv(1, g)
    norm1(2, True)
    qkv(2, 0)
    qkv(2, 1)
    attention(0, 4, True)
    wait(in_ffn0)
    set_gate(0, modulation(2 * D, 640)[:, 0:D])
    prepare_wo()
    out_projection(0)
    m = modulation(3 * D - 64, 3 * D + 64)
    set_shift_scale(1, m[:, 64:64 + D], m[:, 64 + D:64 + 2 * D])
    set_gate(1, m[:, 64 + 2 * D:64 + 3 * D])
    qkv(2, 2)
    norm2(0, False)

    pending = None
    for p in range(NP):
        if p == 2:
            wait(in_ffn1)
        if p == NP - 1:
            attention(1, 2, True)
            out_projection(1)
        rights = hidden_one_level(p)
        if p > 0:
            down_one_level(p - 1, pending)
        pending = rights
    down_one_level(NP - 1, pending)
    outputs = [start_cols(0, (xt, out_hbm, 0, TM))]
    norm2(1, True)
    wait(in_x3)

    for i in range(1, NB):
        for p in range(NP):
            if (i, p) == (2, 1):
                norm1(3, True)
                for g in range(3):
                    qkv(3, g)
            if p == NP - 1 and i + 1 < NB:
                attention(i + 1, 1, False)
                out_projection(i + 1)
            h = gate_up(i, p)
            if p % 2:
                hidden_two_levels(pending, h)
            pending = h
        if i == 1:
            prepare_wd(3)
        outputs.append(down(i))
        if i + 1 < NB:
            norm2(i + 1, True)
        if i == 1:
            wait(outputs.pop(0))
    for copies in outputs:
        wait(copies)


@jax.jit
def pallas_adaLN_cond__sliding_local_dilated__glu_gated_bilinear__prompt_kernel(
    A_x: jax.Array,
    A_wqkv: jax.Array,
    A_wo: jax.Array,
    B_x: jax.Array,
    B_w_gate: jax.Array,
    B_w_up: jax.Array,
    B_w_down: jax.Array,
    c: jax.Array,
    w_mod: jax.Array,
):
    del B_x
    hbm = pl.BlockSpec(memory_space=pltpu.HBM)
    vmem = pltpu.VMEM
    out_t = pl.pallas_call(
        _kernel,
        in_specs=[hbm] * 8,
        out_specs=hbm,
        out_shape=jax.ShapeDtypeStruct((D, S), BF),
        scratch_shapes=[
            vmem((1, D), BF),
            vmem((D, S), BF),
            vmem((D, 3 * D), BF),
            vmem((D, D), BF),
            vmem((D, F), BF),
            vmem((D, F), BF),
            vmem((D, F), BF),
            vmem((D, 6 * D), BF),
            vmem((NT, 1792, 128), F32),
            vmem((NT, D + 24, 128), F32),
            vmem((NT, D, 128), F32),
            vmem((448, KT2), I32),
            vmem((D2 // 2, KT2), I32),
            vmem((4, 8, NT * 128), F32),
            vmem((2, D, 128), F32),
            vmem((KT3 // 2, F // 3), I32),
            vmem((KT3 // 2, F // 3), I32),
            vmem((49, D4 // 2, F // 4), I32),
            vmem((NT, S, 128), F32),
            vmem((NT, HALO + S, 128), F32),
            vmem((NT, HALO + S, 128), F32),
            vmem((2, T // 2, KT2), I32),
            vmem((T // 2, KT2), I32),
            vmem((2, D, TM), F32),
            vmem((2, T // 2, KT3), I32),
            vmem((15, D // 3, T), F32),
            pltpu.SemaphoreType.DMA((10,)),
        ],
        compiler_params=pltpu.CompilerParams(vmem_limit_bytes=126 * 2**20),
        name="adaln_local_attention_bilinear_glu",
    )(c, A_x.reshape(S, D).T, A_wqkv, A_wo, B_w_gate, B_w_up, B_w_down.T, w_mod)
    return out_t.T.reshape(1, S, D)
```
